```python
import jax
import jax.numpy as jnp

def _softmax(x, axis=-1):
    return jax.nn.softmax(x, axis=axis)
def _gelu(x):
    return jax.nn.gelu(x, approximate=True)
def _silu(x):
    return jax.nn.silu(x)
def _sigmoid(x):
    return jax.nn.sigmoid(x)
def _layernorm(x, axis=-1, eps=1e-5):
    m = jnp.mean(x, axis=axis, keepdims=True)
    v = jnp.var(x, axis=axis, keepdims=True)
    return (x - m) / jnp.sqrt(v + eps)
def _scatter_add(tgt, idx, src, axis=0):
    return tgt.at[idx].add(src)
def _segment_sum(src, seg, n):
    return jax.ops.segment_sum(src, seg, n)
class _Rng:
    def __init__(self, key):
        self._k = key
    def _next(self):
        self._k, sub = jax.random.split(self._k)
        return sub
    def normal(self, shape):
        return jax.random.normal(self._next(), shape, dtype=jnp.bfloat16)
    def randint(self, lo, hi, shape):
        return jax.random.randint(self._next(), shape, lo, hi, dtype=jnp.int32)
    def uniform(self, shape, lo=0.0, hi=1.0):
        return jax.random.uniform(self._next(), shape, jnp.bfloat16, lo, hi)
    def permutation(self, n):
        return jax.random.permutation(self._next(), n)


kernel_name = 'sequential_preLN__sliding_local_dilated__glu_gated_geglu__prompt'

def setup_inputs():
    _rng = _Rng(jax.random.key(int.from_bytes(__import__("os").urandom(4), "little")))
    _w = (lambda a: (lambda t: t.astype(jnp.bfloat16) if jnp.issubdtype(t.dtype, jnp.floating) else t)(jnp.asarray(a)))
    def _A_setup():
        B, S, D = 1, 2048, 1024
        return {
            "x": _w((lambda *s: _rng.normal(s) * 0.05)(B, S, D)),
            "wqkv": _w((lambda *s: _rng.normal(s) * 0.05)(D, 3 * D)),
            "wo": _w((lambda *s: _rng.normal(s) * 0.05)(D, D)),
        }
    _A_in = _A_setup()

    def _B_setup():
        B, S, Dm, Df = 1, 2048, 1024, 3584
        return {
            "x": _w((lambda *s: _rng.normal(s) * 0.05)(B, S, Dm)),
            "w_gate": _w((lambda *s: _rng.normal(s) * 0.05)(Dm, Df) * (Dm ** -0.5)),
            "w_up": _w((lambda *s: _rng.normal(s) * 0.05)(Dm, Df) * (Dm ** -0.5)),
            "w_down": _w((lambda *s: _rng.normal(s) * 0.05)(Df, Dm) * (Df ** -0.5)),
        }
    _B_in = _B_setup()

    return {
        "A_x": _A_in["x"],
        "A_wqkv": _A_in["wqkv"],
        "A_wo": _A_in["wo"],
        "B_x": _B_in["x"],
        "B_w_gate": _B_in["w_gate"],
        "B_w_up": _B_in["w_up"],
        "B_w_down": _B_in["w_down"],
    }

def reference(A_x, A_wqkv, A_wo, B_x, B_w_gate, B_w_up, B_w_down):
    def _A_ref(x, wqkv, wo):
        B, S, D = x.shape
        H = 32; Dh = D // H
        W, dil = 8, 2
        qkv = (lambda x, *d: x.transpose(*d))((x @ wqkv).reshape(B, S, 3, H, Dh), 2, 0, 3, 1, 4)
        q, k, v = qkv[0], qkv[1], qkv[2]
        scale = Dh ** -0.5
        pos = jnp.arange(S)
        off = jnp.arange(W) * dil
        idx = pos[:, None] - off[None, :]
        mask = idx >= 0
        idx_c = jnp.where(mask, idx, 0).reshape(-1)
        kg = k[:, :, idx_c, :].reshape(B, H, S, W, Dh)
        vg = v[:, :, idx_c, :].reshape(B, H, S, W, Dh)
        logits = jnp.einsum("bhsd,bhswd->bhsw", q, kg) * scale
        logits = jnp.where(mask[None, None, :, :], logits, -1e9)
        attn = _softmax(logits, axis=-1)
        o = jnp.einsum("bhsw,bhswd->bhsd", attn, vg)
        return (lambda x, *d: x.transpose(*d))(o, 0, 2, 1, 3).reshape(B, S, D) @ wo

    def _B_ref(x, w_gate, w_up, w_down):
        g = jnp.einsum("bsd,df->bsf", x, w_gate)
        u = jnp.einsum("bsd,df->bsf", x, w_up)
        h = _gelu(g) * u
        return jnp.einsum("bsf,fd->bsd", h, w_down)

    x = A_x
    h = x + _A_ref(_layernorm(x, axis=-1), A_wqkv, A_wo)
    h2 = h + _B_ref(_layernorm(h, axis=-1), B_w_gate, B_w_up, B_w_down)
    return h2
```

```python
import functools
import numpy as np
import jax
import jax.numpy as jnp
import jax.experimental.pallas as pl
import jax.experimental.pallas.tpu as pltpu

CFG = dict(T1=256, T2=256, FC=512, R=16, PR=64, bigdown=False, flags=None)

_H, _DH, _W, _DIL = 32, 32, 8, 2
_HALO = 16
_EPS = 1e-5
_F32, _BF16 = jnp.float32, jnp.bfloat16


def _dot(a, b):
    return jnp.dot(a, b, preferred_element_type=_F32)


def _layernorm(x):
    m = jnp.mean(x, axis=-1, keepdims=True)
    xc = x - m
    v = jnp.mean(xc * xc, axis=-1, keepdims=True)
    return xc * jax.lax.rsqrt(v + _EPS)


def _geglu(g, u):
    c1 = float(np.sqrt(2.0 / np.pi))
    c2 = c1 * 0.044715
    th = jnp.tanh(g * (c1 + c2 * (g * g)))
    hu = (0.5 * g) * u
    return hu * th + hu


def _permute_cols(w_ref, col0, r0, rows):
    shape = (rows // 2, 128)
    lane = jax.lax.broadcasted_iota(jnp.int32, shape, 1)
    h_lo, beta, d_lo = lane & 3, (lane >> 2) & 7, lane >> 5
    vs = []
    for g in range(8):
        x = pltpu.bitcast(w_ref[pl.ds(r0, rows), pl.ds(col0 + g * 128, 128)], jnp.int32)
        idx = h_lo * 32 + (beta ^ g) * 4 + d_lo
        vs.append(jnp.take_along_axis(x, idx, axis=1, mode="promise_in_bounds"))
    for b in range(3):
        m = (lane & (4 << b)) != 0
        vs = [jnp.where(m, vs[j ^ (1 << b)], vs[j]) for j in range(8)]
    for j in range(8):
        y = vs[j]
        if j:
            y = jnp.take_along_axis(y, lane ^ (j << 2), axis=1, mode="promise_in_bounds")
        w_ref[pl.ds(r0, rows), pl.ds(col0 + j * 128, 128)] = pltpu.bitcast(y, _BF16)


def _attention(q_s, k_s, v_s, o_s, r0, rows, pos0):
    scale = _DH ** -0.5
    q = [q_s[c, pl.ds(r0, rows), :] for c in range(8)]
    ls = []
    for w in range(_W):
        s = _HALO + r0 - _DIL * w
        acc = q[0] * k_s[0, pl.ds(s, rows), :]
        for c in range(1, 8):
            acc = acc + q[c] * k_s[c, pl.ds(s, rows), :]
        acc = acc + pltpu.roll(acc, 64, 1)
        acc = acc + pltpu.roll(acc, 32, 1)
        l = acc * scale
        if pos0 is not None and w > 0:
            pos = pos0 + r0 + jax.lax.broadcasted_iota(jnp.int32, l.shape, 0)
            l = jnp.where(pos >= _DIL * w, l, -1e9)
        ls.append(l)
    m = functools.reduce(jnp.maximum, ls)
    ps = [jnp.exp(l - m) for l in ls]
    inv = 1.0 / functools.reduce(jnp.add, ps)
    ps = [p * inv for p in ps]
    for c in range(8):
        acc = ps[0] * v_s[c, pl.ds(_HALO + r0, rows), :]
        for w in range(1, _W):
            acc = acc + ps[w] * v_s[c, pl.ds(_HALO + r0 - _DIL * w, rows), :]
        o_s[pl.ds(r0, rows), pl.ds(c * 128, 128)] = acc.astype(_BF16)


@jax.jit
def pallas_sequential_preLN__sliding_local_dilated__glu_gated_geglu__prompt_kernel(
    A_x, A_wqkv, A_wo, B_x, B_w_gate, B_w_up, B_w_down,
):
    del B_x
    B, S, D = A_x.shape
    F = B_w_gate.shape[1]
    T1, T2, FC, R, PR = CFG["T1"], CFG["T2"], CFG["FC"], CFG["R"], CFG["PR"]
    n1, n2 = S // T1, S // T2

    def kernel(x_hbm, wqkv_hbm, wo_hbm, wg_hbm, wu_hbm, wd_hbm, out_hbm,
               x_s, wqkv, wo, wg, wu, wd, wo32, q_s, k_s, v_s, o_s, h_s, hn_s, a_s, out_s, sem, osem):
        xcp = [pltpu.make_async_copy(x_hbm.at[pl.ds(i * T1, T1)], x_s.at[pl.ds(i * T1, T1)], sem.at[i]) for i in range(n1)]
        wcp = [pltpu.make_async_copy(wqkv_hbm.at[:, pl.ds(j * D, D)], wqkv.at[:, pl.ds(j * D, D)], sem.at[n1 + j]) for j in range(3)]
        ocp = pltpu.make_async_copy(wo_hbm, wo, sem.at[n1 + 3])
        fcp = [pltpu.make_async_copy(a, b, sem.at[n1 + 4 + j]) for j, (a, b) in enumerate(((wg_hbm, wg), (wu_hbm, wu), (wd_hbm, wd)))]
        for c in wcp + [xcp[0], ocp] + xcp[1:] + fcp:
            c.start()

        with jax.named_scope("sc_prep"):
            for j in range(3):
                wcp[j].wait()

                def pbody(i, _):
                    _permute_cols(wqkv, j * D, pl.multiple_of(i * PR, PR), PR)
                jax.lax.fori_loop(0, D // PR, pbody, None)
            ocp.wait()
            for c in range(8):
                wo32[c] = wo[:, pl.ds(c * 128, 128)].astype(_F32)
            for c in range(8):
                for d in range(_DH):
                    wo[pl.ds(d * _H, _H), pl.ds(c * 128, 128)] = wo32[c, pl.ds(d, _H, stride=_DH), :].astype(_BF16)
            for c in xcp:
                c.wait()
            k_s[:, pl.ds(T1, _HALO), :] = jnp.zeros((8, _HALO, 128), _F32)
            v_s[:, pl.ds(T1, _HALO), :] = jnp.zeros((8, _HALO, 128), _F32)

        def p1(i, _):
            r = pl.multiple_of(i * T1, T1)
            x = x_s[pl.ds(r, T1), :].astype(_F32)
            xn = _layernorm(x).astype(_BF16)
            k_s[:, pl.ds(0, _HALO), :] = k_s[:, pl.ds(T1, _HALO), :]
            v_s[:, pl.ds(0, _HALO), :] = v_s[:, pl.ds(T1, _HALO), :]
            for j, (dst, off) in enumerate(((q_s, 0), (k_s, _HALO), (v_s, _HALO))):
                y = _dot(xn, wqkv[:, pl.ds(j * D, D)])
                for c in range(8):
                    dst[c, pl.ds(off, T1), :] = y[:, c * 128:(c + 1) * 128]
            for r0 in range(0, T1, R):
                _attention(q_s, k_s, v_s, o_s, r0, R, r if r0 < _HALO else None)
            h = x_s[pl.ds(r, T1), :].astype(_F32) + _dot(o_s[...], wo[...])
            h_s[pl.ds(r, T1), :] = h
            hn_s[pl.ds(r, T1), :] = _layernorm(h).astype(_BF16)

        with jax.named_scope("sc_p1"):
            jax.lax.fori_loop(0, n1, p1, None)
            for c in fcp:
                c.wait()

        def ocopy(i):
            return pltpu.make_async_copy(out_s.at[pl.ds(i * T2, T2)], out_hbm.at[pl.ds(i * T2, T2)], osem.at[i])

        def p2(i, _):
            r = pl.multiple_of(i * T2, T2)
            hn = hn_s[pl.ds(r, T2), :]
            acc = h_s[pl.ds(r, T2), :]
            for c in range(F // FC):
                g = _dot(hn, wg[:, pl.ds(c * FC, FC)])
                u = _dot(hn, wu[:, pl.ds(c * FC, FC)])
                a = _geglu(g, u).astype(_BF16)
                if CFG["bigdown"]:
                    a_s[:, pl.ds(c * FC, FC)] = a
                else:
                    acc = acc + _dot(a, wd[pl.ds(c * FC, FC), :])
            if CFG["bigdown"]:
                acc = acc + _dot(a_s[...], wd[...])
            out_s[pl.ds(r, T2), :] = acc.astype(_BF16)
            ocopy(i).start()

        with jax.named_scope("sc_p2"):
            jax.lax.fori_loop(0, n2, p2, None)
        with jax.named_scope("sc_tail"):
            for i in range(n2):
                ocopy(i).wait()

    any_spec = pl.BlockSpec(memory_space=pl.ANY)
    out = pl.pallas_call(
        kernel,
        out_shape=jax.ShapeDtypeStruct((S, D), A_x.dtype),
        in_specs=[any_spec] * 6,
        out_specs=any_spec,
        scratch_shapes=[
            pltpu.VMEM((S, D), _BF16), pltpu.VMEM((D, 3 * D), _BF16), pltpu.VMEM((D, D), _BF16),
            pltpu.VMEM((D, F), _BF16), pltpu.VMEM((D, F), _BF16), pltpu.VMEM((F, D), _BF16),
            pltpu.VMEM((8, D, 128), _F32),
            pltpu.VMEM((8, T1, 128), _F32), pltpu.VMEM((8, T1 + _HALO, 128), _F32), pltpu.VMEM((8, T1 + _HALO, 128), _F32),
            pltpu.VMEM((T1, D), _BF16), pltpu.VMEM((S, D), _F32), pltpu.VMEM((S, D), _BF16),
            pltpu.VMEM((T2, F), _BF16), pltpu.VMEM((S, D), _BF16),
            pltpu.SemaphoreType.DMA((n1 + 7,)), pltpu.SemaphoreType.DMA((n2,)),
        ],
        compiler_params=pltpu.CompilerParams(vmem_limit_bytes=110 * 1024 * 1024, flags=CFG["flags"]),
    )(A_x.reshape(S, D), A_wqkv, A_wo, B_w_gate, B_w_up, B_w_down)
    return out.reshape(B, S, D)
```

```python
import functools
import numpy as np
import jax
import jax.numpy as jnp
import jax.experimental.pallas as pl
import jax.experimental.pallas.tpu as pltpu

CFG = dict(T1=256, T=256, FC=512, R=16, PR=32, NQ=4, flags=None, OP=4, LR=16, scopes=False, skip=0, PR0=128, F1=5, F2=4, F0=2, unroll=False)

_H, _DH, _W, _DIL = 32, 32, 8, 2
_HALO = 16
_EPS = 1e-5
_F32, _BF16, _I32 = jnp.float32, jnp.bfloat16, jnp.int32


def _dot(a, b):
    return jnp.dot(a, b, preferred_element_type=_F32)


def _pack(x):
    return pltpu.bitcast(x.astype(_BF16), _I32)


def _unpack(x):
    return pltpu.bitcast(x, _BF16)


def _token(parts):
    tiles = [p[r:r + 8, c:c + 128] for p in parts
             for r in range(0, p.shape[0], 8) for c in range(0, p.shape[1], 128)]
    return functools.reduce(jnp.bitwise_or, tiles)


def _dot_paced(a, w, jobs, zero, first=0):
    if jobs:
        nt, nk = w.shape[1] // 128, w.shape[0] // 256
        top = [[w[k * 256:k * 256 + 8, t * 128:(t + 1) * 128] for t in range(nt)] for k in range(nk)]
        for j, job in enumerate(jobs):
            t, k = divmod(first + ((j + 1) * (nt * nk - first) - 1) // len(jobs), nk)
            top[k][t] = top[k][t] | (job() & zero)
        w = jnp.concatenate(
            [p for k in range(nk) for p in (jnp.concatenate(top[k], axis=1), w[k * 256 + 8:(k + 1) * 256])], axis=0)
    return _dot(a, _unpack(w))


def _share(jobs, j, parts):
    return jobs[j * len(jobs) // parts:(j + 1) * len(jobs) // parts]


def _layernorm(x):
    m = jnp.mean(x, axis=-1, keepdims=True)
    xc = x - m
    v = jnp.mean(xc * xc, axis=-1, keepdims=True)
    return xc * jax.lax.rsqrt(v + _EPS)


def _geglu(g, u):
    c1 = float(np.sqrt(2.0 / np.pi))
    c2 = c1 * 0.044715
    th = jnp.tanh(g * (c1 + c2 * (g * g)))
    hu = (0.5 * g) * u
    return hu * th + hu


def _permute_cols(src, dst, r0, rows):
    shape = (rows // 2, 128)
    lane = jax.lax.broadcasted_iota(_I32, shape, 1)
    h_lo, beta, d_lo = lane & 3, (lane >> 2) & 7, lane >> 5
    vs = []
    for g in range(8):
        x = pltpu.bitcast(src[pl.ds(r0, rows), pl.ds(g * 128, 128)], _I32)
        idx = h_lo * 32 + (beta ^ g) * 4 + d_lo
        vs.append(jnp.take_along_axis(x, idx, axis=1, mode="promise_in_bounds"))
    for b in range(3):
        m = (lane & (4 << b)) != 0
        vs = [jnp.where(m, vs[j ^ (1 << b)], vs[j]) for j in range(8)]
    for j in range(8):
        if j:
            vs[j] = jnp.take_along_axis(vs[j], lane ^ (j << 2), axis=1, mode="promise_in_bounds")
        dst[pl.ds(r0 // 2, rows // 2), pl.ds(j * 128, 128)] = vs[j]
    return _token(vs)


def _permute_rows(src, tmp, dst, c):
    cols = pl.ds(c * 128 if isinstance(c, int) else pl.multiple_of(c * 128, 128), 128)
    for h in range(_H):
        tmp[c, pl.ds(h * (_DH + 1), _DH), :] = src[pl.ds(h * _DH, _DH), cols].astype(_F32)
    ys = []
    for d in range(_DH):
        ys.append(_pack(tmp[c, pl.ds(d, _H, stride=_DH + 1), :]))
        dst[pl.ds(d * _H // 2, _H // 2), cols] = ys[-1]
    return _token(ys)


def _attention(q_s, k_s, v_s, o_s, r0, rows, first):
    scale = _DH ** -0.5
    q = [q_s[c, pl.ds(r0, rows), :] for c in range(8)]
    ls = []
    for w in range(_W):
        s = _HALO + r0 - _DIL * w
        acc = q[0] * k_s[0, pl.ds(s, rows), :]
        for c in range(1, 8):
            acc = acc + q[c] * k_s[c, pl.ds(s, rows), :]
        if not CFG["skip"] & 1: acc = acc + pltpu.roll(acc, 64, 1)
        if not CFG["skip"] & 1: acc = acc + pltpu.roll(acc, 32, 1)
        l = acc * scale
        if first and r0 < _DIL * w:
            pos = r0 + jax.lax.broadcasted_iota(_I32, l.shape, 0)
            l = jnp.where(pos >= _DIL * w, l, -1e9)
        ls.append(l)
    m = functools.reduce(jnp.maximum, ls)
    ps = [jnp.exp(l - m) for l in ls]
    inv = 1.0 / functools.reduce(jnp.add, ps)
    ps = [p * inv for p in ps]
    ys = []
    for c in range(8):
        acc = ps[0] * v_s[c, pl.ds(_HALO + r0, rows), :]
        for w in range(1, _W):
            acc = acc + ps[w] * v_s[c, pl.ds(_HALO + r0 - _DIL * w, rows), :]
        ys.append(_pack(acc))
        o_s[pl.ds(r0 // 2, rows // 2), pl.ds(c * 128, 128)] = ys[-1]
    return _token(ys)


def _layernorm_rows(src, dst, r0, rows):
    y = _pack((_layernorm if not CFG["skip"] & 2 else (lambda t: t * 20.0))(src[pl.ds(r0, rows), :].astype(_F32)))
    dst[pl.ds(r0 // 2, rows // 2), :] = y
    return _token([y])


class _NoScope:
    def __init__(self, name):
        pass

    def __enter__(self):
        pass

    def __exit__(self, *a):
        pass


@jax.jit
def pallas_sequential_preLN__sliding_local_dilated__glu_gated_geglu__prompt_kernel(
    A_x, A_wqkv, A_wo, B_x, B_w_gate, B_w_up, B_w_down,
):
    del B_x
    B, S, D = A_x.shape
    F = B_w_gate.shape[1]
    T1, T, FC, R, PR, NQ = (CFG[k] for k in ("T1", "T", "FC", "R", "PR", "NQ"))
    n1, n = S // T1, S // T
    scope = jax.named_scope if CFG["scopes"] else _NoScope

    def kernel(x_hbm, wqkv_hbm, wo_hbm, wg_hbm, wu_hbm, wd_hbm, out_hbm,
               x_s, wq_in, wkv_in, wo_in, wg, wu, wd, wq, wk, wv, wo, wo32,
               xn_s, q_s, k_s, v_s, o_s, ha_s, hb_s, hna_s, hnb_s, out_s, zero_s, sem, xsem, ksem, osem):
        P = functools.partial
        LR = CFG["LR"]
        qr, kr = D // NQ, D // n1

        def rows(i, size, extra=0):
            return pl.ds(i * size if isinstance(i, int) else pl.multiple_of(i * size, size), size + extra)

        def xcp(i):
            return pltpu.make_async_copy(x_hbm.at[rows(i, T1)], x_s.at[rows(i, T1)], xsem.at[i])

        def kcp(i):
            return pltpu.make_async_copy(wqkv_hbm.at[rows(i, kr), pl.ds(D, 2 * D)], wkv_in.at[rows(i, kr)], ksem.at[i])

        def qcp(j):
            return pltpu.make_async_copy(wqkv_hbm.at[rows(j, qr), pl.ds(0, D)], wq_in.at[rows(j, qr)], sem.at[5 + j])

        ocp, *fcp = [pltpu.make_async_copy(a, b, sem.at[j]) for j, (a, b) in enumerate((
            (wo_hbm, wo_in), (wg_hbm, wg), (wu_hbm, wu), (wd_hbm, wd)))]

        def perm(src, dst, i):
            return [P(_permute_cols, src.at[rows(i, kr)], dst.at[rows(i, kr // 2)], r0, PR) for r0 in range(0, kr, PR)]

        def proj(i, t, w, dst, off, jobs, first=0):
            y = _dot_paced(_unpack(xn_s[rows(i, t // 2), :]), w[...], jobs, zero_s[...], first)
            dst = dst.at[:, rows(i, t, off), :]
            for c in range(8):
                dst[c, pl.ds(off, t), :] = y[:, c * 128:(c + 1) * 128]

        with scope("sc_p0"):
            for c in [xcp(0)] + [qcp(j) for j in range(NQ)]:
                c.start()
            zero_s[...] = jnp.zeros((8, 128), _I32)
            k_s[:, pl.ds(0, _HALO), :] = jnp.zeros((8, _HALO, 128), _F32)
            xcp(0).wait()

            def ln_step(j, _):
                _layernorm_rows(x_s.at[rows(j, 256)], xn_s.at[rows(j, 128)], 0, 256)
            jax.lax.fori_loop(0, T1 // 256, ln_step, None)

            def p_step(j, _):
                qcp(j).wait()

                @pl.when(j == NQ - 2)
                def _():
                    xcp(1).start()
                    kcp(0).start()
                for r0 in range(0, qr, CFG["PR0"]):
                    _permute_cols(wq_in.at[rows(j, qr)], wq.at[rows(j, qr // 2)], r0, CFG["PR0"])
            jax.lax.fori_loop(0, NQ, p_step, None)

        def q_step(i, _):
            @pl.when(i + 2 < n1)
            def _():
                xcp(i + 2).start()

            @pl.when(i + 1 < n1)
            def _():
                kcp(i + 1).start()
                xcp(i + 1).wait()

            @pl.when(i == n1 - 2)
            def _():
                ocp.start()
            kcp(i).wait()
            j = jnp.minimum(i + 1, n1 - 1)
            jobs = [P(_layernorm_rows, x_s.at[rows(j, T1)], xn_s.at[rows(j, T1 // 2)], r0, LR) for r0 in range(0, T1, LR)]
            extra = perm(wkv_in.at[:, pl.ds(0, D)], wk, i) + perm(wkv_in.at[:, pl.ds(D, D)], wv, i)
            jobs = sum([_share(jobs, j, len(extra)) + [e] for j, e in enumerate(extra)], [])
            parts = T1 // 256
            for p in range(parts):
                proj(i * parts + p, 256, wq, q_s, 0, _share(jobs, p, parts), 0 if p else CFG['F0'])

        with scope("sc_q"):
            jax.lax.fori_loop(0, n1, q_step, None)

        def attn(i, first):
            q_t = q_s.at[:, rows(i, T), :]
            k_t = k_s.at[:, rows(i, T, _HALO), :]
            v_t = v_s.at[:, rows(i, T, _HALO), :]
            return [P(_attention, q_t, k_t, v_t, o_s, r0, R, first) for r0 in range(0, T, R)]

        def kv_step(i, _):
            proj(i, T, wk, k_s, _HALO, [P(_permute_rows, wo_in, wo32, wo, i)])
            proj(i, T, wv, v_s, _HALO, [])

        with scope("sc_kv"):
            ocp.wait()
            for c in fcp:
                c.start()
            jax.lax.fori_loop(0, n - 1, kv_step, None)
        with scope("sc_kvl"):
            for c in range(8):
                v_s[c, pl.ds(0, _HALO), :] = jnp.broadcast_to(v_s[c, pl.ds(_HALO, 1), :], (_HALO, 128))
            jobs = [P(_permute_rows, wo_in, wo32, wo, n - 1)] + attn(0, True)
            proj(n - 1, T, wk, k_s, _HALO, _share(jobs, 0, 2))
            proj(n - 1, T, wv, v_s, _HALO, _share(jobs, 1, 2))
            for c in fcp:
                c.wait()

        def ocopy(i):
            return pltpu.make_async_copy(out_s.at[rows(i, T)], out_hbm.at[rows(i, T)], osem.at[i])

        def ffn(i, _):
            zero = zero_s[...]
            nc, hf = F // FC, T // 2
            z = i >> 8
            words = lambda w: pltpu.bitcast(w, _I32)
            x_t = x_s.at[rows(i, T)]
            hs, hns = (ha_s, hb_s), (hna_s, hnb_s)
            ln2 = [[P(_layernorm_rows, hs[p].at[rows(z, hf)], hns[p], r0, LR) for r0 in range(0, hf, LR)] for p in range(2)]
            for p in range(2):
                hs[p][...] = x_t[pl.ds(p * hf, hf), :].astype(_F32) + _dot_paced(
                    _unpack(o_s[pl.ds(p * hf // 2, hf // 2), :]), wo[rows(z if p else 0, D // 2), :],
                    ln2[0] if p else [], zero, CFG["F1"])
            g = []
            for p in range(2):
                g.append(_dot_paced(_unpack(hns[p][rows(z, hf // 2), :]), words(wg[rows(z if p else 0, D), pl.ds(0, FC)]),
                                    [] if p else ln2[1], zero, CFG["F2"]))
            hn = _unpack(jnp.concatenate([r[rows(z, hf // 2), :] for r in hns], axis=0))
            a = _geglu(jnp.concatenate(g, axis=0), _dot(hn, wu[:, pl.ds(0, FC)])).astype(_BF16)
            acc = jnp.concatenate([r[rows(z, hf), :] for r in hs], axis=0) + _dot(a, wd[pl.ds(0, FC), :])
            att = attn(jnp.minimum(i + 1, n - 1), False)
            for c in range(1, nc):
                jobs = _share(att, c - 1, nc - 1)
                g = _dot_paced(hn, words(wg[:, pl.ds(c * FC, FC)]), _share(jobs, 0, 2), zero)
                u = _dot(hn, wu[:, pl.ds(c * FC, FC)])
                acc = acc + _dot_paced(_geglu(g, u).astype(_BF16), words(wd[pl.ds(c * FC, FC), :]), _share(jobs, 1, 2), zero)
            out_s[rows(i, T), :] = acc.astype(_BF16)
            ocopy(i).start()

        with scope("sc_main"):
            jax.lax.fori_loop(0, n, ffn, None)
        with scope("sc_tail"):
            for i in range(n):
                ocopy(i).wait()

    any_spec = pl.BlockSpec(memory_space=pl.ANY)
    out = pl.pallas_call(
        kernel,
        out_shape=jax.ShapeDtypeStruct((S, D), A_x.dtype),
        in_specs=[any_spec] * 6,
        out_specs=any_spec,
        scratch_shapes=[
            pltpu.VMEM((S, D), _BF16)] + [pltpu.VMEM((D, D), _BF16), pltpu.VMEM((D, 2 * D), _BF16), pltpu.VMEM((D, D), _BF16)] + [
            pltpu.VMEM((D, F), _BF16), pltpu.VMEM((D, F), _BF16), pltpu.VMEM((F, D), _BF16)]
            + [pltpu.VMEM((D // 2, D), _I32)] * 4 + [
            pltpu.VMEM((8, _H * (_DH + 1), 128), _F32),
            pltpu.VMEM((S // 2, D), _I32),
            pltpu.VMEM((8, S, 128), _F32), pltpu.VMEM((8, S + _HALO, 128), _F32), pltpu.VMEM((8, S + _HALO, 128), _F32),
            pltpu.VMEM((T // 2, D), _I32), pltpu.VMEM((T // 2, D), _F32), pltpu.VMEM((T // 2, D), _F32), pltpu.VMEM((T // 4, D), _I32), pltpu.VMEM((T // 4, D), _I32),
            pltpu.VMEM((S, D), _BF16), pltpu.VMEM((8, 128), _I32),
            pltpu.SemaphoreType.DMA((NQ + 5,)), pltpu.SemaphoreType.DMA((n1,)), pltpu.SemaphoreType.DMA((n1,)), pltpu.SemaphoreType.DMA((n,)),
        ],
        compiler_params=pltpu.CompilerParams(vmem_limit_bytes=110 * 1024 * 1024, flags=CFG["flags"]),
    )(A_x.reshape(S, D), A_wqkv, A_wo, B_w_gate, B_w_up, B_w_down)
    return out.reshape(B, S, D)
```

```python
import functools
import numpy as np
import jax
import jax.numpy as jnp
import jax.experimental.pallas as pl
import jax.experimental.pallas.tpu as pltpu

CFG = dict(FC=512, PR=32, LR=32, LR2=16, QR=64, PM=2, QM=0, KR=176, F0=1, F1=5, F2=4, F3=1, flags={'XLA_TPU_EVENLY_DISTRIBUTE_CRITICAL_NODES':True}, scopes=False, QC=256, TK=512, AR=96, OS=512, AM=2, AM0=1, TM=256, ON='gd', S0=0, S1=-1)

_H, _DH, _W, _DIL = 32, 32, 8, 2
_HALO = 16
_EPS = 1e-5
_F32, _BF16, _I32 = jnp.float32, jnp.bfloat16, jnp.int32


def _dot(a, b):
    return jnp.dot(a, b, preferred_element_type=_F32)


def _words(x):
    return pltpu.bitcast(x, _I32)


def _pack(x):
    return _words(x.astype(_BF16))


def _unpack(x):
    return pltpu.bitcast(x, _BF16)


def _rows(i, size, extra=0):
    return pl.ds(i * size if isinstance(i, int) else pl.multiple_of(i * size, size), size + extra)


def _token(parts):
    tiles = [p[r:r + 8, c:c + 128] for p in parts
             for r in range(0, p.shape[0], 8) for c in range(0, p.shape[1], 128)]
    return functools.reduce(jnp.bitwise_or, tiles)


def _dot_paced(a, w, jobs, zero, first=0):
    if jobs:
        nt, nk = w.shape[1] // 128, w.shape[0] // 256
        top = [[w[k * 256:k * 256 + 8, t * 128:(t + 1) * 128] for t in range(nt)] for k in range(nk)]
        for j, job in enumerate(jobs):
            t, k = divmod(first + ((j + 1) * (nt * nk - first) - 1) // len(jobs), nk)
            top[k][t] = top[k][t] | (job() & zero)
        w = jnp.concatenate(
            [p for k in range(nk) for p in (jnp.concatenate(top[k], axis=1), w[k * 256 + 8:(k + 1) * 256])], axis=0)
    return _dot(a, _unpack(w))


def _share(jobs, j, parts):
    return jobs[j * len(jobs) // parts:(j + 1) * len(jobs) // parts]


def _merge(a, b):
    return sum([_share(a, j, len(b)) + [e] for j, e in enumerate(b)], [])


def _layernorm_rows(src, dst, r0, rows):
    x = src[pl.ds(r0, rows), :].astype(_F32)
    xc = x - jnp.mean(x, axis=-1, keepdims=True)
    var = jnp.mean(xc * xc, axis=-1, keepdims=True)
    y = _pack(xc * jax.lax.rsqrt(var + _EPS))
    dst[pl.ds(r0 // 2, rows // 2), :] = y
    return _token([y])


def _geglu(g, u):
    c1 = float(np.sqrt(2.0 / np.pi))
    c2 = c1 * 0.044715
    th = jnp.tanh(g * (c1 + c2 * (g * g)))
    hu = (0.5 * g) * u
    return hu * th + hu


def _head_minor(load, store):
    vs = []
    lanes = lambda: jax.lax.broadcasted_iota(_I32, vs[0].shape, 1)

    def skew():
        vs.extend(pltpu.roll(load(g), 4 * g, 1) if g else load(g) for g in range(8))
        return _token(vs[1:])

    def exchange():
        us = [vs[-j % 8] for j in range(8)]
        for b in range(3):
            m = (lanes() & (4 << b)) != 0
            us = [jnp.where(m, us[(j - (1 << b)) % 8], us[j]) for j in range(8)]
        vs[:] = [pltpu.roll(u, 128 - 4 * j, 1) if j else u for j, u in enumerate(us)]
        return _token(vs[1:])

    def shuffle():
        lane = lanes()
        idx = (lane & 3) * 32 + (lane & 28) + (lane >> 5)
        ys = [jnp.take_along_axis(v, idx, axis=1, mode="promise_in_bounds") for v in vs]
        for j, y in enumerate(ys):
            store(j, y)
        return _token(ys)

    return [skew, exchange, shuffle]


def _permute_weight_cols(src, dst, r0, rows):
    def store(j, v):
        dst[pl.ds(r0 // 2, rows // 2), pl.ds(j * 128, 128)] = v
    return _head_minor(lambda g: _words(src[pl.ds(r0, rows), pl.ds(g * 128, 128)]), store)


def _permute_q(src, dst, r0, rows):
    def store(j, v):
        dst[j, pl.ds(r0, rows), :] = _unpack(v).astype(_F32)
    return _head_minor(lambda g: src[pl.ds(r0 // 2, rows // 2), pl.ds(g * 128, 128)], store)


def _together(jobs):
    return lambda: functools.reduce(jnp.bitwise_or, [job() for job in jobs])


def _chain(jobs):
    return lambda: [job() for job in jobs][-1]


def _staggered(chains):
    depth = len(chains[0])
    return [_together([c[t - i] for i, c in enumerate(chains) if 0 <= t - i < depth])
            for t in range(len(chains) + depth - 1)]


def _permute_weight_rows(src, tmp, dst, c):
    cols = _rows(c, 128)

    def spread(h0, n):
        ys = []
        for h in range(h0, h0 + n):
            ys.append(src[pl.ds(h * _DH, _DH), cols])
            tmp[pl.ds(h * (_DH + 1), _DH), :] = ys[-1].astype(_F32)
        return _token([_words(y) for y in ys])

    def gather(d0, n):
        ys = []
        for d in range(d0, d0 + n):
            ys.append(_pack(tmp[pl.ds(d, _H, stride=_DH + 1), :]))
            dst[pl.ds(d * _H // 2, _H // 2), cols] = ys[-1]
        return _token(ys)

    return [functools.partial(f, j, 8) for f in (spread, gather) for j in range(0, _H, 8)]


def _attention(q_s, k_s, v_s, o_s, r0, pos0):
    rows, ls = 16, []

    def scores(w0, nw):
        q = [q_s[c, pl.ds(r0, rows), :] for c in range(8)]
        for w in range(w0, w0 + nw):
            s = _HALO + r0 - _DIL * w
            acc = q[0] * k_s[0, pl.ds(s, rows), :]
            for c in range(1, 8):
                acc = acc + q[c] * k_s[c, pl.ds(s, rows), :]
            ls.append(acc + pltpu.roll(acc, 64, 1))
        return _token([_words(l) for l in ls[w0:]])

    def probs():
        for w in range(_W):
            l = (ls[w] + pltpu.roll(ls[w], 32, 1)) * (_DH ** -0.5)
            if pos0 is not None and r0 < _DIL * w:
                pos = pos0 + r0 + jax.lax.broadcasted_iota(_I32, l.shape, 0)
                l = jnp.where(pos >= _DIL * w, l, -1e9)
            ls[w] = l
        m = functools.reduce(jnp.maximum, ls)
        es = [jnp.exp(l - m) for l in ls]
        inv = 1.0 / functools.reduce(jnp.add, es)
        ls[:] = [e * inv for e in es]
        return _token([_words(inv)])

    def mix(c0, nc):
        ys = []
        for c in range(c0, c0 + nc):
            acc = ls[0] * v_s[c, pl.ds(_HALO + r0, rows), :]
            for w in range(1, _W):
                acc = acc + ls[w] * v_s[c, pl.ds(_HALO + r0 - _DIL * w, rows), :]
            ys.append(_pack(acc))
            o_s[pl.ds(r0 // 2, rows // 2), pl.ds(c * 128, 128)] = ys[-1]
        return _token(ys)

    P = functools.partial
    return [
        [_chain([P(scores, 0, 8), probs, P(mix, 0, 8)])],
        [_chain([P(scores, 0, 8), probs]), P(mix, 0, 8)],
        [P(scores, 0, 8), probs, P(mix, 0, 8)],
        [P(scores, 0, 4), P(scores, 4, 4), probs, P(mix, 0, 4), P(mix, 4, 4)],
        [P(scores, 0, 8), _chain([probs, P(mix, 0, 4)]), P(mix, 4, 4)],
    ][CFG['AM0'] if pos0 is not None else CFG["AM"]]


class _NoScope:
    def __init__(self, name):
        pass

    def __enter__(self):
        pass

    def __exit__(self, *a):
        pass


@jax.jit
def pallas_sequential_preLN__sliding_local_dilated__glu_gated_geglu__prompt_kernel(
    A_x, A_wqkv, A_wo, B_x, B_w_gate, B_w_up, B_w_down,
):
    del B_x
    B, S, D = A_x.shape
    F = B_w_gate.shape[1]
    T = 256
    n = S // T
    FC, PR, LR, QR, QC, TK, AR = (CFG[k] for k in ("FC", "PR", "LR", "QR", "QC", "TK", "AR"))
    NK = 4
    scope = jax.named_scope if CFG["scopes"] else _NoScope
    P = functools.partial

    def kernel(x_hbm, wqkv_hbm, wo_hbm, wg_hbm, wu_hbm, wd_hbm, out_hbm,
               x_s, w_in, wo_in, wg, wu, wd, wk, wv, wo, wo32,
               xn_s, q_s, qf_s, k_s, v_s, o_s, ha_s, hb_s, hna_s, hnb_s, out_s, zero_s,
               sem, xsem, ksem, osem):
        def x_copy(i, size, s):
            return pltpu.make_async_copy(x_hbm.at[_rows(i, size)], x_s.at[_rows(i, size)], s)

        def xcp(i):
            return x_copy(i, T, xsem.at[i])

        def kvcp(j):
            return pltpu.make_async_copy(
                wqkv_hbm.at[_rows(j, D // NK), pl.ds(D, 2 * D)], w_in.at[_rows(j, D // NK), pl.ds(D, 2 * D)], ksem.at[j])

        def qcp(j):
            return pltpu.make_async_copy(wqkv_hbm.at[:, _rows(j, QC)], w_in.at[:, _rows(j, QC)], sem.at[6 + j])

        x0cp = [x_copy(j, T, sem.at[4 + j]) for j in range(2)]
        ocp, *fcp = [pltpu.make_async_copy(a, b, sem.at[j]) for j, (a, b) in enumerate((
            (wo_hbm, wo_in), (wg_hbm, wg), (wu_hbm, wu), (wd_hbm, wd)))]

        def ln1(i):
            return [P(_layernorm_rows, x_s.at[_rows(i, T)], xn_s.at[_rows(i, T // 2)], r0, LR) for r0 in range(0, T, LR)]

        with scope("sc_p0"):
            for c in [x0cp[0]] + [qcp(j) for j in range(D // QC)] + [x0cp[1]]:
                c.start()
            zero_s[...] = jnp.zeros((8, 128), _I32)
            k_s[:, pl.ds(0, AR + _HALO), :] = jnp.zeros((8, AR + _HALO, 128), _F32)
            qf_s[:, pl.ds(0, AR), :] = jnp.zeros((8, AR, 128), _F32)
            x0cp[0].wait()
            xcp(2).start()
            kvcp(0).start()
            _layernorm_rows(x_s, xn_s, 0, T)

        def q0_step(j, _):
            qcp(j).wait()
            q_s[pl.ds(0, T // 2), _rows(j, QC)] = _pack(_dot(_unpack(xn_s[pl.ds(0, T // 2), :]), w_in[:, _rows(j, QC)]))

        with scope("sc_q0"):
            jax.lax.fori_loop(0, D // QC, q0_step, None)
            x0cp[1].wait()
            _layernorm_rows(x_s, xn_s, T, T)

        def q_step(i, _):
            @pl.when(i + 2 < n)
            def _():
                xcp(i + 2).start()

            @pl.when(i < NK)
            def _():
                kvcp(i).start()

            @pl.when(i == n - 2)
            def _():
                ocp.start()

            @pl.when(i + 1 < n)
            def _():
                xcp(i + 1).wait()

            @pl.when((i > 1) & (i < NK + 2))
            def _():
                kvcp(i - 2).wait()
            kr = CFG['KR']
            r = pl.multiple_of(jnp.clip((i - 2) * kr, 0, D - kr), 16)
            rh = pl.multiple_of(jnp.clip((i - 2) * (kr // 2), 0, (D - kr) // 2), 8)
            extra = [_permute_weight_cols(w_in.at[pl.ds(r, kr), _rows(jnp.where(i > 1, j + 1, 0), D)], w.at[pl.ds(rh, kr // 2)], r0, min(PR, kr - r0))
                     for j, w in enumerate((wk, wv)) for r0 in range(0, kr, PR)]
            extra = [[_chain(e) for e in extra], sum(extra, []), _staggered(extra)][CFG["PM"]]
            jobs = ln1(jnp.minimum(i + 1, n - 1))
            jobs = _merge(jobs, extra)
            y = _dot_paced(_unpack(xn_s[_rows(i, T // 2), :]), _words(w_in[:, pl.ds(0, D)]), jobs, zero_s[...], CFG["F0"])
            q_s[_rows(i, T // 2), :] = _pack(y)

        with scope("sc_q"):
            jax.lax.fori_loop(1, n, q_step, None)

        def kv_step(i, _):
            def proj(w, dst, jobs):
                parts = TK // CFG["TM"]
                for p in range(parts):
                    t = CFG["TM"]
                    y = _dot_paced(_unpack(xn_s[_rows(i * parts + p, t // 2), :]), w[_rows((i >> 8) if p else 0, D // 2), :],
                                   _share(jobs, p, parts), zero_s[...])
                    d = dst.at[:, _rows(i * parts + p, t, _HALO), :]
                    for c in range(8):
                        d[c, pl.ds(_HALO, t), :] = y[:, c * 128:(c + 1) * 128]

            lead = S // TK - pl.cdiv(T, AR)
            r = pl.multiple_of(jnp.clip((i - lead) * AR, 0, T - AR), 16)
            rh = pl.ds(pl.multiple_of(jnp.clip((i - lead) * (AR // 2), 0, (T - AR) // 2), 8), AR // 2)
            att = [_attention(qf_s.at[:, pl.ds(r, AR), :], k_s.at[:, pl.ds(r, AR + _HALO), :], v_s.at[:, pl.ds(r, AR + _HALO), :],
                              o_s.at[rh], r0, r) for r0 in range(0, AR, 16)]
            groups = 8 * TK // S
            jobs = sum([_permute_weight_rows(wo_in, wo32.at[g], wo, i * groups + g) for g in range(groups)], [])
            proj(wv, v_s, _merge(jobs, sum([a[:-1] for a in att], [])))
            for c in range(8):
                v_s[c, pl.ds(0, _HALO), :] = jnp.broadcast_to(v_s[c, pl.ds(_HALO, 1), :], (_HALO, 128))
            jobs = [_permute_q(q_s.at[_rows(i, TK // 2)], qf_s.at[:, _rows(i, TK), :], r0, QR) for r0 in range(0, TK, QR)]
            jobs = [[_chain(e) for e in jobs], sum(jobs, []), _staggered(jobs)][CFG['QM']]
            proj(wk, k_s, _merge(jobs, [a[-1] for a in att]))

        with scope("sc_kv"):
            ocp.wait()
            for c in fcp:
                c.start()
            jax.lax.fori_loop(0, S // TK, kv_step, None)
            for c in fcp:
                c.wait()

        OS = CFG["OS"]
        pieces = (pl.ds(0, D - OS), pl.ds(D - OS, OS)) if OS else (pl.ds(0, D),)

        def ocopy(i, p):
            return pltpu.make_async_copy(out_s.at[_rows(i, T), pieces[p]], out_hbm.at[_rows(i, T), pieces[p]], osem.at[p * n + i])

        def main_step(i, _):
            zero = zero_s[...]
            nc, hf = F // FC, T // 2
            z = i >> 8
            x_t = x_s.at[_rows(i, T)]
            hs, hns = (ha_s, hb_s), (hna_s, hnb_s)
            ln2 = [[P(_layernorm_rows, hs[p].at[_rows(z, hf)], hns[p], r0, CFG["LR2"]) for r0 in range(0, hf, CFG["LR2"])] for p in range(2)]
            for p in range(2):
                hs[p][...] = x_t[pl.ds(p * hf, hf), :].astype(_F32) + _dot_paced(
                    _unpack(o_s[pl.ds(p * hf // 2, hf // 2), :]), wo[_rows(z if p else 0, D // 2), :],
                    ln2[0] if p else [], zero, CFG["F1"])
            g = []
            for p in range(2):
                g.append(_dot_paced(_unpack(hns[p][_rows(z, hf // 2), :]), _words(wg[_rows(z if p else 0, D), pl.ds(0, FC)]),
                                    [] if p else ln2[1], zero, CFG["F2"]))
            hn = _unpack(jnp.concatenate([r[_rows(z, hf // 2), :] for r in hns], axis=0))
            j = jnp.minimum(i + 1, n - 1)
            att = sum([_attention(qf_s.at[:, _rows(j, T), :], k_s.at[:, _rows(j, T, _HALO), :], v_s.at[:, _rows(j, T, _HALO), :],
                                  o_s, r0, None) for r0 in range(0, T, 16)], [])
            slots = [(c, m) for c in range(nc) for m in CFG["ON"] if (c, m) != (0, "g")][CFG["S0"]:CFG["S1"]]
            jobs = lambda c, m: _share(att, slots.index((c, m)), len(slots)) if (c, m) in slots else []
            acc = jnp.concatenate([r[_rows(z, hf), :] for r in hs], axis=0)
            for c in range(nc):
                g = _dot_paced(hn, _words(wg[:, pl.ds(c * FC, FC)]), jobs(c, "g"), zero) if c else jnp.concatenate(g, axis=0)
                u = _dot_paced(hn, _words(wu[:, pl.ds(c * FC, FC)]), jobs(c, "u"), zero)
                acc = acc + _dot_paced(_geglu(g, u).astype(_BF16), _words(wd[pl.ds(c * FC, FC), :]), jobs(c, "d"), zero)
            for p, cols in enumerate(pieces):
                out_s[_rows(i, T), cols] = acc[:, cols.start:cols.start + cols.size].astype(_BF16)
                ocopy(i, p).start()

        with scope("sc_main"):
            jax.lax.fori_loop(0, n, main_step, None)
        with scope("sc_tail"):
            for i in range(n):
                for p in range(len(pieces)):
                    ocopy(i, p).wait()

    vmem, dma = pltpu.VMEM, pltpu.SemaphoreType.DMA
    any_spec = pl.BlockSpec(memory_space=pl.ANY)
    out = pl.pallas_call(
        kernel,
        out_shape=jax.ShapeDtypeStruct((S, D), A_x.dtype),
        in_specs=[any_spec] * 6,
        out_specs=any_spec,
        scratch_shapes=[
            vmem((S, D), _BF16), vmem((D, 3 * D), _BF16), vmem((D, D), _BF16),
            vmem((D, F), _BF16), vmem((D, F), _BF16), vmem((F, D), _BF16),
            vmem((D // 2, D), _I32), vmem((D // 2, D), _I32), vmem((D // 2, D), _I32),
            vmem((8 * TK // S, _H * (_DH + 1), 128), _F32),
            vmem((S // 2, D), _I32), vmem((S // 2, D), _I32), vmem((8, S + 8, 128), _F32),
            vmem((8, S + _HALO + 8, 128), _F32), vmem((8, S + _HALO + 8, 128), _F32),
            vmem((T // 2, D), _I32), vmem((T // 2, D), _F32), vmem((T // 2, D), _F32),
            vmem((T // 4, D), _I32), vmem((T // 4, D), _I32),
            vmem((S, D), _BF16), vmem((8, 128), _I32),
            dma((6 + D // QC,)), dma((n,)), dma((NK,)), dma((2 * n,)),
        ],
        compiler_params=pltpu.CompilerParams(vmem_limit_bytes=110 * 1024 * 1024, flags=CFG["flags"]),
    )(A_x.reshape(S, D), A_wqkv, A_wo, B_w_gate, B_w_up, B_w_down)
    return out.reshape(B, S, D)
```

```python
import functools
import numpy as np
import jax
import jax.numpy as jnp
import jax.experimental.pallas as pl
import jax.experimental.pallas.tpu as pltpu

CFG = dict(FC=1024, PR=32, LR=32, LR2=16, QR=64, PM=2, QM=0, KR=176, F0=1, F1=5, F2=4, F3=1, flags={'XLA_TPU_EVENLY_DISTRIBUTE_CRITICAL_NODES':True}, scopes=False, QC=256, TK=512, AR=96, OS=512, AM=2, AM0=1, TM=256, ON='gud', S0=0, NJ=20, TOK=(0,), S1=-7)

_H, _DH, _W, _DIL = 32, 32, 8, 2
_HALO = 16
_EPS = 1e-5
_F32, _BF16, _I32 = jnp.float32, jnp.bfloat16, jnp.int32


def _dot(a, b):
    return jnp.dot(a, b, preferred_element_type=_F32)


def _words(x):
    return pltpu.bitcast(x, _I32)


def _pack(x):
    return _words(x.astype(_BF16))


def _unpack(x):
    return pltpu.bitcast(x, _BF16)


def _rows(i, size, extra=0):
    return pl.ds(i * size if isinstance(i, int) else pl.multiple_of(i * size, size), size + extra)


def _token(parts):
    tiles = [p[r:r + 8, c:c + 128] for p in parts
             for r in range(0, p.shape[0], 8) for c in range(0, p.shape[1], 128)]
    return functools.reduce(jnp.bitwise_or, tiles)


def _dot_paced(a, w, jobs, zero, first=0):
    if jobs:
        nt, nk = w.shape[1] // 128, pl.cdiv(w.shape[0], 256)
        top = [[w[k * 256:k * 256 + 8, t * 128:(t + 1) * 128] for t in range(nt)] for k in range(nk)]
        for queue in jobs if isinstance(jobs[0], list) else [jobs]:
            for j, job in enumerate(queue):
                t, k = divmod(first + ((j + 1) * (nt * nk - first) - 1) // len(queue), nk)
                top[k][t] = top[k][t] | (job() & zero)
        w = jnp.concatenate(
            [p for k in range(nk) for p in (jnp.concatenate(top[k], axis=1), w[k * 256 + 8:(k + 1) * 256])], axis=0)
    return _dot(a, _unpack(w))


def _share(jobs, j, parts):
    return jobs[j * len(jobs) // parts:(j + 1) * len(jobs) // parts]


def _merge(a, b):
    return sum([_share(a, j, len(b)) + [e] for j, e in enumerate(b)], [])


def _layernorm(x):
    xc = x - jnp.mean(x, axis=-1, keepdims=True)
    var = jnp.mean(xc * xc, axis=-1, keepdims=True)
    return xc * jax.lax.rsqrt(var + _EPS)


def _layernorm_rows(src, dst, r0, rows):
    y = _pack(_layernorm(src[pl.ds(r0, rows), :].astype(_F32)))
    dst[pl.ds(r0 // 2, rows // 2), :] = y
    return _token([y])


def _left(a11, a12, a21, a22):
    return (lambda: a11 + a22, lambda: a21 + a22, lambda: a11, lambda: a22,
            lambda: a11 + a12, lambda: a21 - a11, lambda: a12 - a22)


def _right(b11, b12, b21, b22):
    return (b11 + b22, b11, b12 - b22, b21 - b11, b22, b11 + b12, b21 + b22)


def _combine(m):
    return (((m[3] - m[4]) + m[0]) + m[6], m[2] + m[4], m[1] + m[3], ((m[2] - m[1]) + m[0]) + m[5])


def _right_operands(src, dst, tiles, zero):
    half = src.shape[2] // 2
    token = None
    for r0, c0 in tiles:
        b = [_words(src[j, pl.ds(r0, 16), pl.ds(k * half + c0, 128)]) for j in range(2) for k in range(2)]
        if token is not None:
            b[0] = b[0] | (token & zero)
        ys = [_pack(y) for y in _right(*[_unpack(v).astype(_F32) for v in b])]
        ys[1], ys[4] = b[0], b[3]
        for j, y in enumerate(ys):
            dst[j, pl.ds(r0 // 2, 8), pl.ds(c0, 128)] = y
        token = _token([ys[j] for j in CFG["TOK"]])
    return token


def _geglu(g, u):
    c1 = float(np.sqrt(2.0 / np.pi))
    c2 = c1 * 0.044715
    th = jnp.tanh(g * (c1 + c2 * (g * g)))
    hu = (0.5 * g) * u
    return hu * th + hu


def _head_minor(load, store):
    vs = []
    lanes = lambda: jax.lax.broadcasted_iota(_I32, vs[0].shape, 1)

    def skew():
        vs.extend(pltpu.roll(load(g), 4 * g, 1) if g else load(g) for g in range(8))
        return _token(vs[1:])

    def exchange():
        us = [vs[-j % 8] for j in range(8)]
        for b in range(3):
            m = (lanes() & (4 << b)) != 0
            us = [jnp.where(m, us[(j - (1 << b)) % 8], us[j]) for j in range(8)]
        vs[:] = [pltpu.roll(u, 128 - 4 * j, 1) if j else u for j, u in enumerate(us)]
        return _token(vs[1:])

    def shuffle():
        lane = lanes()
        idx = (lane & 3) * 32 + (lane & 28) + (lane >> 5)
        ys = [jnp.take_along_axis(v, idx, axis=1, mode="promise_in_bounds") for v in vs]
        for j, y in enumerate(ys):
            store(j, y)
        return _token(ys)

    return [skew, exchange, shuffle]


def _permute_weight_cols(src, dst, r0, rows):
    def store(j, v):
        dst[pl.ds(r0 // 2, rows // 2), pl.ds(j * 128, 128)] = v
    return _head_minor(lambda g: _words(src[pl.ds(r0, rows), pl.ds(g * 128, 128)]), store)


def _permute_q(src, dst, r0, rows):
    def store(j, v):
        dst[j, pl.ds(r0, rows), :] = _unpack(v).astype(_F32)
    return _head_minor(lambda g: src[pl.ds(r0 // 2, rows // 2), pl.ds(g * 128, 128)], store)


def _together(jobs):
    return lambda: functools.reduce(jnp.bitwise_or, [job() for job in jobs])


def _chain(jobs):
    return lambda: [job() for job in jobs][-1]


def _staggered(chains):
    depth = len(chains[0])
    return [_together([c[t - i] for i, c in enumerate(chains) if 0 <= t - i < depth])
            for t in range(len(chains) + depth - 1)]


def _permute_weight_rows(src, tmp, dst, c):
    cols = _rows(c, 128)

    def spread(h0, n):
        ys = []
        for h in range(h0, h0 + n):
            ys.append(src[pl.ds(h * _DH, _DH), cols])
            tmp[pl.ds(h * (_DH + 1), _DH), :] = ys[-1].astype(_F32)
        return _token([_words(y) for y in ys])

    def gather(d0, n):
        ys = []
        for d in range(d0, d0 + n):
            ys.append(_pack(tmp[pl.ds(d, _H, stride=_DH + 1), :]))
            dst[pl.ds(d * _H // 2, _H // 2), cols] = ys[-1]
        return _token(ys)

    return [functools.partial(f, j, 8) for f in (spread, gather) for j in range(0, _H, 8)]


def _attention(q_s, k_s, v_s, o_s, r0, pos0):
    rows, ls = 16, []

    def scores(w0, nw):
        q = [q_s[c, pl.ds(r0, rows), :] for c in range(8)]
        for w in range(w0, w0 + nw):
            s = _HALO + r0 - _DIL * w
            acc = q[0] * k_s[0, pl.ds(s, rows), :]
            for c in range(1, 8):
                acc = acc + q[c] * k_s[c, pl.ds(s, rows), :]
            ls.append(acc + pltpu.roll(acc, 64, 1))
        return _token([_words(l) for l in ls[w0:]])

    def probs():
        for w in range(_W):
            l = (ls[w] + pltpu.roll(ls[w], 32, 1)) * (_DH ** -0.5)
            if pos0 is not None and r0 < _DIL * w:
                pos = pos0 + r0 + jax.lax.broadcasted_iota(_I32, l.shape, 0)
                l = jnp.where(pos >= _DIL * w, l, -1e9)
            ls[w] = l
        m = functools.reduce(jnp.maximum, ls)
        es = [jnp.exp(l - m) for l in ls]
        inv = 1.0 / functools.reduce(jnp.add, es)
        ls[:] = [e * inv for e in es]
        return _token([_words(inv)])

    def mix(c0, nc):
        ys = []
        for c in range(c0, c0 + nc):
            acc = ls[0] * v_s[c, pl.ds(_HALO + r0, rows), :]
            for w in range(1, _W):
                acc = acc + ls[w] * v_s[c, pl.ds(_HALO + r0 - _DIL * w, rows), :]
            ys.append(_pack(acc))
            o_s[pl.ds(r0 // 2, rows // 2), pl.ds(c * 128, 128)] = ys[-1]
        return _token(ys)

    P = functools.partial
    return [
        [_chain([P(scores, 0, 8), probs, P(mix, 0, 8)])],
        [_chain([P(scores, 0, 8), probs]), P(mix, 0, 8)],
        [P(scores, 0, 8), probs, P(mix, 0, 8)],
        [P(scores, 0, 4), P(scores, 4, 4), probs, P(mix, 0, 4), P(mix, 4, 4)],
        [P(scores, 0, 8), _chain([probs, P(mix, 0, 4)]), P(mix, 4, 4)],
    ][CFG['AM0'] if pos0 is not None else CFG["AM"]]


class _NoScope:
    def __init__(self, name):
        pass

    def __enter__(self):
        pass

    def __exit__(self, *a):
        pass


@jax.jit
def pallas_sequential_preLN__sliding_local_dilated__glu_gated_geglu__prompt_kernel(
    A_x, A_wqkv, A_wo, B_x, B_w_gate, B_w_up, B_w_down,
):
    del B_x
    B, S, D = A_x.shape
    F = B_w_gate.shape[1]
    T = 256
    n = S // T
    FC, PR, LR, QR, QC, TK, AR = (CFG[k] for k in ("FC", "PR", "LR", "QR", "QC", "TK", "AR"))
    NK, NS = 4, S // TK
    scope = jax.named_scope if CFG["scopes"] else _NoScope
    P = functools.partial

    def kernel(x_hbm, wqkv_hbm, wo_hbm, wg_hbm, wu_hbm, wd_hbm, out_hbm,
               x_s, w_in, wo_in, wg_in, wu_in, wd_in, wg, wu, wd, wk, wv, wo, wo32,
               xn_s, q_s, qf_s, k_s, v_s, o_s, ha_s, hb_s, na_s, hna_s, hnb_s, out_s, zero_s,
               sem, xsem, ksem, fsem, osem):
        def x_copy(i, size, s):
            return pltpu.make_async_copy(x_hbm.at[_rows(i, size)], x_s.at[_rows(i, size)], s)

        def xcp(i):
            return x_copy(i, T, xsem.at[i])

        def kvcp(j):
            return pltpu.make_async_copy(
                wqkv_hbm.at[_rows(j, D // NK), pl.ds(D, 2 * D)], w_in.at[_rows(j, D // NK), pl.ds(D, 2 * D)], ksem.at[j])

        def qcp(j):
            return pltpu.make_async_copy(wqkv_hbm.at[:, _rows(j, QC)], w_in.at[:, _rows(j, QC)], sem.at[6 + j])

        x0cp = [x_copy(j, T, sem.at[4 + j]) for j in range(2)]
        ocp = pltpu.make_async_copy(wo_hbm, wo_in, sem.at[0])

        def fcp(i):
            return [pltpu.make_async_copy(w.at[_rows(j * NS + i, w.shape[0] // 2 // NS)], dst.at[i % 2, j], fsem.at[i * 6 + k * 2 + j])
                    for k, (w, dst) in enumerate(((wg_hbm, wg_in), (wu_hbm, wu_in), (wd_hbm, wd_in))) for j in range(2)]

        def ln1(i):
            return [P(_layernorm_rows, x_s.at[_rows(i, T)], xn_s.at[_rows(i, T // 2)], r0, LR) for r0 in range(0, T, LR)]

        with scope("sc_p0"):
            for c in [x0cp[0]] + [qcp(j) for j in range(D // QC)] + [x0cp[1]]:
                c.start()
            zero_s[...] = jnp.zeros((8, 128), _I32)
            k_s[:, pl.ds(0, AR + _HALO), :] = jnp.zeros((8, AR + _HALO, 128), _F32)
            qf_s[:, pl.ds(0, AR), :] = jnp.zeros((8, AR, 128), _F32)
            x0cp[0].wait()
            xcp(2).start()
            kvcp(0).start()
            _layernorm_rows(x_s, xn_s, 0, T)

        def q0_step(j, _):
            qcp(j).wait()
            q_s[pl.ds(0, T // 2), _rows(j, QC)] = _pack(_dot(_unpack(xn_s[pl.ds(0, T // 2), :]), w_in[:, _rows(j, QC)]))

        with scope("sc_q0"):
            jax.lax.fori_loop(0, D // QC, q0_step, None)
            x0cp[1].wait()
            _layernorm_rows(x_s, xn_s, T, T)

        def q_step(i, _):
            @pl.when(i < NK)
            def _():
                xcp(i + 2).start()
                kvcp(i).start()

            @pl.when(i == NK - 1)
            def _():
                for j in range(NK + 2, n):
                    xcp(j).start()

            @pl.when(i == NK)
            def _():
                ocp.start()
                for c in fcp(0):
                    c.start()

            @pl.when(i + 1 < n)
            def _():
                xcp(i + 1).wait()

            @pl.when((i > 1) & (i < NK + 2))
            def _():
                kvcp(i - 2).wait()
            kr = CFG['KR']
            r = pl.multiple_of(jnp.clip((i - 2) * kr, 0, D - kr), 16)
            rh = pl.multiple_of(jnp.clip((i - 2) * (kr // 2), 0, (D - kr) // 2), 8)
            extra = [_permute_weight_cols(w_in.at[pl.ds(r, kr), _rows(jnp.where(i > 1, j + 1, 0), D)], w.at[pl.ds(rh, kr // 2)], r0, min(PR, kr - r0))
                     for j, w in enumerate((wk, wv)) for r0 in range(0, kr, PR)]
            extra = [[_chain(e) for e in extra], sum(extra, []), _staggered(extra)][CFG["PM"]]
            jobs = ln1(jnp.minimum(i + 1, n - 1))
            jobs = _merge(jobs, extra)
            y = _dot_paced(_unpack(xn_s[_rows(i, T // 2), :]), _words(w_in[:, pl.ds(0, D)]), jobs, zero_s[...], CFG["F0"])
            q_s[_rows(i, T // 2), :] = _pack(y)

        with scope("sc_q"):
            jax.lax.fori_loop(1, n, q_step, None)

        def kv_step(i, _):
            @pl.when(i + 1 < NS)
            def _():
                for c in fcp(i + 1):
                    c.start()
            for c in fcp(i):
                c.wait()
            prep = []
            for src, dst in ((wg_in, wg), (wu_in, wu), (wd_in, wd)):
                size = src.shape[2]
                tiles = [(r0, c0) for r0 in range(0, size, 16) for c0 in range(0, dst.shape[2], 128)]
                prep += [P(_right_operands, src.at[i % 2], dst.at[:, _rows(i, size // 2), :], _share(tiles, t, CFG["NJ"]), zero_s[...])
                         for t in range(CFG["NJ"])]

            def proj(w, dst, jobs, more, first):
                parts = TK // CFG["TM"]
                for p in range(parts):
                    t = CFG["TM"]
                    y = _dot_paced(_unpack(xn_s[_rows(i * parts + p, t // 2), :]), w[_rows((i >> 8) if p else 0, D // 2), :],
                                   [_share(jobs, p, parts), _share(more, p, parts)], zero_s[...], 0 if p else first)
                    d = dst.at[:, _rows(i * parts + p, t, _HALO), :]
                    for c in range(8):
                        d[c, pl.ds(_HALO, t), :] = y[:, c * 128:(c + 1) * 128]

            lead = S // TK - pl.cdiv(T, AR)
            r = pl.multiple_of(jnp.clip((i - lead) * AR, 0, T - AR), 16)
            rh = pl.ds(pl.multiple_of(jnp.clip((i - lead) * (AR // 2), 0, (T - AR) // 2), 8), AR // 2)
            att = [_attention(qf_s.at[:, pl.ds(r, AR), :], k_s.at[:, pl.ds(r, AR + _HALO), :], v_s.at[:, pl.ds(r, AR + _HALO), :],
                              o_s.at[rh], r0, r) for r0 in range(0, AR, 16)]
            groups = 8 * TK // S
            jobs = sum([_permute_weight_rows(wo_in, wo32.at[g], wo, i * groups + g) for g in range(groups)], [])
            proj(wv, v_s, _share(prep, 0, 2), _merge(jobs, sum([a[:-1] for a in att], [])), 1)
            for c in range(8):
                v_s[c, pl.ds(0, _HALO), :] = jnp.broadcast_to(v_s[c, pl.ds(_HALO, 1), :], (_HALO, 128))
            jobs = [_permute_q(q_s.at[_rows(i, TK // 2)], qf_s.at[:, _rows(i, TK), :], r0, QR) for r0 in range(0, TK, QR)]
            jobs = [[_chain(e) for e in jobs], sum(jobs, []), _staggered(jobs)][CFG['QM']]
            proj(wk, k_s, _share(prep, 1, 2), _merge(jobs, [a[-1] for a in att]), 0)

        with scope("sc_kv"):
            ocp.wait()
            jax.lax.fori_loop(0, S // TK, kv_step, None)

        OS = CFG["OS"]
        pieces = (pl.ds(0, D - OS), pl.ds(D - OS, OS)) if OS else (pl.ds(0, D),)

        def ocopy(i, p):
            return pltpu.make_async_copy(out_s.at[_rows(2 * i + p, T // 2)], out_hbm.at[_rows(2 * i + p, T // 2)], osem.at[p * n + i])

        def main_step(i, _):
            zero = zero_s[...]
            hf, hd, lr = T // 2, D // 2, CFG["LR2"]
            z = i >> 8
            x_t = x_s.at[_rows(i, T)]
            hs = (ha_s, hb_s)
            early = (2, 4)

            def ln2(p, r0):
                y = _layernorm(hs[p].at[_rows(z, hf)][pl.ds(r0, lr), :])
                if p:
                    up = na_s.at[_rows(z, hf)][pl.ds(r0, lr), :]
                else:
                    na_s[pl.ds(r0, lr), :] = up = y
                left = _left(up[:, :hd], up[:, hd:], y[:, :hd], y[:, hd:])
                ys = {k: _pack(left[k]()) for k in range(7) if (k in early) != bool(p)}
                for k, v in ys.items():
                    (hnb_s if p else hna_s)[k, pl.ds(r0 // 2, lr // 2), :] = v
                return _token(ys.values())

            ln = [[P(ln2, p, r0) for r0 in range(0, hf, lr)] for p in range(2)]
            for p in range(2):
                hs[p][...] = x_t[pl.ds(p * hf, hf), :].astype(_F32) + _dot_paced(
                    _unpack(o_s[pl.ds(p * hf // 2, hf // 2), :]), wo[_rows(z if p else 0, D // 2), :],
                    ln[0] if p else [], zero, CFG["F1"])
            hn = lambda k: _unpack((hna_s if k in early else hnb_s)[k, _rows(z, hf // 2), :])
            j = jnp.minimum(i + 1, n - 1)
            att = sum([_attention(qf_s.at[:, _rows(j, T), :], k_s.at[:, _rows(j, T, _HALO), :], v_s.at[:, _rows(j, T, _HALO), :],
                                  o_s, r0, None) for r0 in range(0, T, 16)], [])
            chunks = [(c0, min(FC, F // 2 - c0)) for c0 in range(0, F // 2, FC)]
            up_order, down_order = (2, 4, 1, 3, 0, 5, 6), (1, 3, 6, 0, 2, 4, 5)
            steps = [(0, m, k) for m in "gu" for k in early]
            for c in range(len(chunks)):
                steps += [(c, m, k) for m in "gud" for k in (down_order if m == "d" else up_order) if (c, m, k) not in steps]
            slots = [st for st in steps[4:] if st[1] in CFG["ON"]][CFG["S0"]:CFG["S1"]]
            jobs = {st: _share(att, t, len(slots)) for t, st in enumerate(slots)}
            jobs.update({steps[1 + t]: _share(ln[1], t, 3) for t in range(3)})
            prod, down = {}, {}
            for st in steps:
                c, m, k = st
                c0, width = chunks[c]
                if m == "d":
                    if k == down_order[0]:
                        g, u = (_combine([prod[c, w, t] for t in range(7)]) for w in "gu")
                        left = _left(*[_geglu(*gu) for gu in zip(g, u)])
                    y = _dot_paced(left[k]().astype(_BF16), wd[k, pl.ds(c0 // 2, width // 2), :], jobs.get(st), zero)
                    down[k] = down[k] + y if c else y
                else:
                    prod[st] = _dot_paced(hn(k), (wg if m == "g" else wu)[k, :, pl.ds(c0, width)], jobs.get(st), zero)
            out = _combine(down)
            out_t = out_s.at[_rows(i, T)]
            for p in range(2):
                for t in range(2):
                    cols = pl.ds(t * hd, hd)
                    out_t[pl.ds(p * hf, hf), cols] = (hs[p][_rows(z, hf), cols] + out[2 * p + t]).astype(_BF16)
                ocopy(i, p).start()

        with scope("sc_main"):
            jax.lax.fori_loop(0, n, main_step, None)
        with scope("sc_tail"):
            for i in range(n):
                for p in range(len(pieces)):
                    ocopy(i, p).wait()

    vmem, dma = pltpu.VMEM, pltpu.SemaphoreType.DMA
    any_spec = pl.BlockSpec(memory_space=pl.ANY)
    out = pl.pallas_call(
        kernel,
        out_shape=jax.ShapeDtypeStruct((S, D), A_x.dtype),
        in_specs=[any_spec] * 6,
        out_specs=any_spec,
        scratch_shapes=[
            vmem((S, D), _BF16), vmem((D, 3 * D), _BF16), vmem((D, D), _BF16),
            vmem((2, 2, D // 2 // NS, F), _BF16), vmem((2, 2, D // 2 // NS, F), _BF16), vmem((2, 2, F // 2 // NS, D), _BF16),
            vmem((7, D // 4, F // 2), _I32), vmem((7, D // 4, F // 2), _I32), vmem((7, F // 4, D // 2), _I32),
            vmem((D // 2, D), _I32), vmem((D // 2, D), _I32), vmem((D // 2, D), _I32),
            vmem((8 * TK // S, _H * (_DH + 1), 128), _F32),
            vmem((S // 2, D), _I32), vmem((S // 2, D), _I32), vmem((8, S + 8, 128), _F32),
            vmem((8, S + _HALO + 8, 128), _F32), vmem((8, S + _HALO + 8, 128), _F32),
            vmem((T // 2, D), _I32), vmem((T // 2, D), _F32), vmem((T // 2, D), _F32),
            vmem((T // 2, D), _F32), vmem((7, T // 4, D // 2), _I32), vmem((7, T // 4, D // 2), _I32),
            vmem((S, D), _BF16), vmem((8, 128), _I32),
            dma((6 + D // QC,)), dma((n,)), dma((NK,)), dma((6 * NS,)), dma((2 * n,)),
        ],
        compiler_params=pltpu.CompilerParams(vmem_limit_bytes=120 * 1024 * 1024, flags=CFG["flags"]),
    )(A_x.reshape(S, D), A_wqkv, A_wo, B_w_gate, B_w_up, B_w_down)
    return out.reshape(B, S, D)
```

```python
import functools
import numpy as np
import jax
import jax.numpy as jnp
import jax.experimental.pallas as pl
import jax.experimental.pallas.tpu as pltpu

CFG = dict(FC=(768, 1024), F1=0, AS=64, AR_=0, LR=16, LR2=16, QR=64, F0=3, scopes=False, QC=256, TK=512, AR=48, KR=96, PM=2, QM=0, AM=3, AM0=1,
           ON='gud', S0=0, S1=-7, NJ=20, SK=True, U=1, G=0, GC=-2, GK=0, SV=True, QS=True,
           flags={'XLA_TPU_EVENLY_DISTRIBUTE_CRITICAL_NODES': True})

_H, _DH, _W, _DIL = 32, 32, 8, 2
_HALO = 16
_EPS = 1e-5
_F32, _BF16, _I32 = jnp.float32, jnp.bfloat16, jnp.int32
P = functools.partial


def _dot(a, b):
    return jnp.dot(a, b, preferred_element_type=_F32)


def _words(x):
    return pltpu.bitcast(x, _I32)


def _pack(x):
    return _words(x.astype(_BF16))


def _unpack(x):
    return pltpu.bitcast(x, _BF16)


def _rows(i, size, extra=0):
    return pl.ds(i * size if isinstance(i, int) else pl.multiple_of(i * size, size), size + extra)


def _clamped(i, size, total, extra=0):
    return pl.ds(pl.multiple_of(jnp.clip(i * size, 0, total - size), 8 if size % 16 else 16), size + extra)


def _token(parts):
    tiles = [p[r:r + 8, c:c + 128] for p in parts
             for r in range(0, p.shape[0], 8) for c in range(0, p.shape[1], 128)]
    return functools.reduce(jnp.bitwise_or, tiles)


def _dot_paced(a, w, zero, queues=(), first=0):
    if any(queues):
        nt, nk, step = w.shape[1] // 128, pl.cdiv(w.shape[0], 256), CFG["AS"]
        due = {}
        for queue in queues:
            for j, job in enumerate(queue):
                due.setdefault(divmod(first + ((j + 1) * (nt * nk - first) - 1) // len(queue), nk), []).append(job())
        due = {slot: _token(tokens) & zero for slot, tokens in due.items()}
        parts = []
        for r in range(0, w.shape[0], step):
            top = [w[r:r + 8, t * 128:(t + 1) * 128] for t in range(nt)]
            top = [v | due[t, r // 256] if (t, r // 256) in due and (r // 64 % 4 == [0, (t * nk + r // 256) % 4, 3][CFG['AR_']] % min(4, (w.shape[0] - r // 256 * 256) // 64)) else v for t, v in enumerate(top)]
            parts += [jnp.concatenate(top, axis=1), w[r + 8:r + step]]
        w = jnp.concatenate(parts, axis=0)
    return _dot(a if a.dtype == _BF16 else _unpack(a), _unpack(w))


def _share(jobs, j, parts):
    return jobs[j * len(jobs) // parts:(j + 1) * len(jobs) // parts]


def _merge(a, b):
    return sum([_share(a, j, len(b)) + [e] for j, e in enumerate(b)], [])


def _together(jobs):
    return lambda: functools.reduce(jnp.bitwise_or, [job() for job in jobs])


def _chain(jobs):
    return lambda: [job() for job in jobs][-1]


def _staggered(chains):
    depth = len(chains[0])
    return [_together([c[t - i] for i, c in enumerate(chains) if 0 <= t - i < depth])
            for t in range(len(chains) + depth - 1)]


def _arrange(chains, mode):
    return [[_chain(e) for e in chains], sum(chains, []), _staggered(chains)][mode]


def _left(a11, a12, a21, a22):
    return (a11 + a22, a21 + a22, a11, a22, a11 + a12, a21 - a11, a12 - a22)


def _right(b11, b12, b21, b22):
    return (b11 + b22, b11, b12 - b22, b21 - b11, b22, b11 + b12, b21 + b22)


def _combine(m):
    return (((m[3] - m[4]) + m[0]) + m[6], m[2] + m[4], m[1] + m[3], ((m[2] - m[1]) + m[0]) + m[5])


_ORDER = (2, 4, 1, 3, 0, 5, 6)


def _store_operands(dst, rows, cols, ys):
    ys = [_pack(y) for y in ys]
    for k, y in enumerate(ys):
        dst.at[k][rows, cols] = y
    return ys


def _load_f32(src, r0, rows, cols):
    return jnp.concatenate([src[pl.ds(r, 8), cols].astype(_F32) for r in range(r0, r0 + rows, 8)], axis=0)


def _right_operands(upper, lower, dst, tiles, zero, gate):
    half = upper.shape[1] // 2
    token = gate[-1] if gate else None
    for r0, c0 in tiles:
        b = [src[pl.ds(r0, 16), pl.ds(k * half + c0, 128)].astype(_F32) for src in (upper, lower) for k in range(2)]
        if token is not None:
            b[0] = jnp.concatenate([pltpu.bitcast(_words(b[0][:8]) | (token & zero), _F32), b[0][8:]], axis=0)
        token = _store_operands(dst, pl.ds(r0 // 2, 8), pl.ds(c0, 128), _right(*b))[0]
    return token


def _layernorm(x):
    xc = x - jnp.mean(x, axis=-1, keepdims=True)
    var = jnp.mean(xc * xc, axis=-1, keepdims=True)
    return xc * jax.lax.rsqrt(var + _EPS)


_SUMS = (0, 1, 4, 5, 6)


def _layernorm_left(src, plain, sums, r0, rows):
    hf, hd = src.shape[0] // 2, src.shape[1] // 2
    a, b = (_layernorm(src[pl.ds(p * hf + r0, rows), :].astype(_F32)) for p in range(2))
    ys = _store_operands(plain, pl.ds(r0 // 2, rows // 2), slice(None), (a, b))
    if CFG["SK"] or CFG["SV"]:
        left = _left(a[:, :hd], a[:, hd:], b[:, :hd], b[:, hd:])
        ys = _store_operands(sums, pl.ds(r0 // 2, rows // 2), slice(None), [left[k] for k in _SUMS])[1:3]
    return _token(ys)


def _geglu(g, u):
    c1 = float(np.sqrt(2.0 / np.pi))
    c2 = c1 * 0.044715
    th = jnp.tanh(g * (c1 + c2 * (g * g)))
    hu = (0.5 * g) * u
    return hu * th + hu


def _head_minor(load, store):
    vs = []
    lanes = lambda: jax.lax.broadcasted_iota(_I32, vs[0].shape, 1)

    def skew():
        vs.extend(pltpu.roll(load(g), 4 * g, 1) if g else load(g) for g in range(8))
        return _token(vs[1:])

    def exchange():
        us = [vs[-j % 8] for j in range(8)]
        for b in range(3):
            m = (lanes() & (4 << b)) != 0
            us = [jnp.where(m, us[(j - (1 << b)) % 8], us[j]) for j in range(8)]
        vs[:] = [pltpu.roll(u, 128 - 4 * j, 1) if j else u for j, u in enumerate(us)]
        return _token(vs[1:])

    def shuffle():
        lane = lanes()
        idx = (lane & 3) * 32 + (lane & 28) + (lane >> 5)
        return store([jnp.take_along_axis(v, idx, axis=1, mode="promise_in_bounds") for v in vs])

    return [skew, exchange, shuffle]


def _prepare_kv_weight(upper, lower, dst, r0):
    def load(g):
        return jnp.concatenate([_words(src[pl.ds(r0, 16), pl.ds(g * 128, 128)]) for src in (upper, lower)], axis=0)

    def store(vs):
        if dst.shape[0] == 2:
            for j, v in enumerate(vs):
                for p in range(2):
                    dst[p, pl.ds(r0 // 2, 8), pl.ds(j * 128, 128)] = v[8 * p:8 * p + 8]
            return _token(vs)
        vs = [_unpack(v).astype(_F32) for v in vs]
        return _token([_store_operands(dst, pl.ds(r0 // 2, 8), pl.ds(j * 128, 128),
                                       _right(vs[j][:16], vs[j + 4][:16], vs[j][16:], vs[j + 4][16:]))[0] for j in range(4)])
    return _head_minor(load, store)


def _prepare_q(src, dst, r0, rows):
    def store(vs):
        for j, v in enumerate(vs):
            if CFG["QS"]:
                dst[j, pl.ds(r0, rows // 2, stride=2), :] = pltpu.bitcast(v << 16, _F32)
                dst[j, pl.ds(r0 + 1, rows // 2, stride=2), :] = pltpu.bitcast(v & -65536, _F32)
            else:
                dst[j, pl.ds(r0, rows), :] = _unpack(v).astype(_F32)
        return _token(vs)
    return _head_minor(lambda g: src[pl.ds(r0 // 2, rows // 2), pl.ds(g * 128, 128)], store)


def _prepare_out_weight(src, tmp, dst, c):
    def spread(h0):
        ys = []
        for h in range(h0, h0 + 4):
            for k in range(2):
                ys.append(src[pl.ds(h * _DH, _DH), _rows(c + 4 * k, 128)].astype(_F32))
                tmp[k, pl.ds(h * (_DH + 1), _DH), :] = ys[-1]
        return _token([_words(y[:8]) for y in ys])

    def gather(d0):
        ys = []
        for d in range(d0, d0 + 2):
            b = [tmp[k, pl.ds(d + j * _DH // 2, _H, stride=_DH + 1), :] for j in range(2) for k in range(2)]
            ys.append(_store_operands(dst, pl.ds(d * _H // 2, _H // 2), _rows(c, 128), _right(*b))[0])
        return _token(ys)

    return [P(spread, h) for h in range(0, _H, 4)] + [P(gather, d) for d in range(0, _DH // 2, 2)]


def _after(x, gate):
    return x if not gate else pltpu.bitcast(_words(x) | jnp.tile(gate[-1], (x.shape[0] // 8, 1)), x.dtype)


def _attention(q_s, k_s, v_s, r0, pos0, store, mode, gate):
    rows, ls = 16, []

    def scores():
        q = [q_s[c, pl.ds(r0, rows), :] for c in range(8)]
        q[0] = _after(q[0], gate)
        for w in range(_W):
            s = _HALO + r0 - _DIL * w
            acc = q[0] * k_s[0, pl.ds(s, rows), :]
            for c in range(1, 8):
                acc = acc + q[c] * k_s[c, pl.ds(s, rows), :]
            ls.append(acc + pltpu.roll(acc, 64, 1))
        return _token([_words(l) for l in ls])

    def probs():
        for w in range(_W):
            l = (ls[w] + pltpu.roll(ls[w], 32, 1)) * (_DH ** -0.5)
            if pos0 is not None and r0 < _DIL * w:
                pos = pos0 + r0 + jax.lax.broadcasted_iota(_I32, l.shape, 0)
                l = jnp.where(pos >= _DIL * w, l, -1e9)
            ls[w] = l
        m = functools.reduce(jnp.maximum, ls)
        es = [jnp.exp(l - m) for l in ls]
        inv = 1.0 / functools.reduce(jnp.add, es)
        ls[:] = [e * inv for e in es]
        return _token([_words(inv)])

    def mix(c0, nc):
        p0 = _after(ls[0], gate if CFG['G'] > 1 else None)

        def group(c):
            acc = p0 * v_s[c, pl.ds(_HALO + r0, rows), :]
            for w in range(1, _W):
                acc = acc + ls[w] * v_s[c, pl.ds(_HALO + r0 - _DIL * w, rows), :]
            return acc
        return _token([y for c in range(c0, c0 + nc) for y in store(r0, c, group(c), group(c + 4))])

    return [[_chain([scores, probs, P(mix, 0, 4)])],
            [_chain([scores, probs]), P(mix, 0, 4)],
            [scores, probs, P(mix, 0, 4)],
            [scores, probs, P(mix, 0, 2), P(mix, 2, 2)],
            [scores, _chain([probs, P(mix, 0, 2)]), P(mix, 2, 2)]][mode]


def _attention_pairs(views, keep, dst, pos0, mode, gate):
    def store_upper(r0, c, a11, a12):
        keep[c, pl.ds(r0, 16), :] = a11
        keep[c + 4, pl.ds(r0, 16), :] = a12
        return [_words(a11), _words(a12)]

    def store_lower(r0, c, a21, a22):
        left = _left(keep[c, pl.ds(r0, 16), :], keep[c + 4, pl.ds(r0, 16), :], a21, a22)
        return _store_operands(dst, pl.ds(r0 // 2, 8), pl.ds(c * 128, 128), left)[1:2]

    return [_attention(*views[p], r0, None if p else pos0, store, mode, gate)
            for r0 in range(0, views[0][0].shape[1], 16) for p, store in enumerate((store_upper, store_lower))]


class _NoScope:
    def __init__(self, name):
        pass

    def __enter__(self):
        pass

    def __exit__(self, *a):
        pass


@jax.jit
def pallas_sequential_preLN__sliding_local_dilated__glu_gated_geglu__prompt_kernel(
    A_x, A_wqkv, A_wo, B_x, B_w_gate, B_w_up, B_w_down,
):
    del B_x
    B, S, D = A_x.shape
    F = B_w_gate.shape[1]
    T = 256
    n, hf, hd = S // T, T // 2, D // 2
    FC, LR, QR, QC, TK, AR, KR = (CFG[k] for k in ("FC", "LR", "QR", "QC", "TK", "AR", "KR"))
    NK, NS = 4, S // TK
    scope = jax.named_scope if CFG["scopes"] else _NoScope

    def kernel(x_hbm, wqkv_hbm, wo_hbm, wg_hbm, wu_hbm, wd_hbm, out_hbm,
               x_s, w_in, wo_in, wg_in, wu_in, wd_in, wg, wu, wd, wk, wv, wo, wo32,
               xn_s, xl_s, q_s, qf_s, k_s, v_s, keep_s, o_s, ha_s, hb_s, na_s, hna_s, hnb_s, zero_s,
               sem, ksem, fsem, osem):
        def xcp(i):
            return pltpu.make_async_copy(x_hbm.at[_rows(i, T)], x_s.at[_rows(i, T)], sem.at[i])

        def qcp(j):
            return pltpu.make_async_copy(wqkv_hbm.at[:, _rows(j, QC)], w_in.at[:, _rows(j, QC)], sem.at[n + j])

        def kvcp(j):
            at = lambda ref, p: ref.at[_rows(p * NK + j, hd // NK), pl.ds(D, 2 * D)]
            return [pltpu.make_async_copy(at(wqkv_hbm, p), at(w_in, p), ksem.at[2 * j + p]) for p in range(2)]

        ocp = pltpu.make_async_copy(wo_hbm, wo_in, ksem.at[2 * NK])

        def fcp(i):
            return [pltpu.make_async_copy(w.at[_rows(j * NS + i, w.shape[0] // 2 // NS)], dst.at[i % 2, j], fsem.at[i * 6 + k * 2 + j])
                    for k, (w, dst) in enumerate(((wg_hbm, wg_in), (wu_hbm, wu_in), (wd_hbm, wd_in))) for j in range(2)]

        def norm1(i, rows):
            at = lambda ref: ref.at[:, _rows(i, hf // 2), :]
            return [P(_layernorm_left, x_s.at[_rows(i, T)], at(xn_s), at(xl_s), r0, rows) for r0 in range(0, hf, rows)]

        def normed(i):
            return jnp.concatenate([xn_s[p, _rows(i, hf // 2), :] for p in range(2)], axis=0)

        with scope("sc_p0"):
            for c in [xcp(0)] + [qcp(j) for j in range(D // QC)] + [xcp(1), xcp(2)]:
                c.start()
            zero_s[...] = jnp.zeros((8, 128), _I32)
            for p in range(2):
                k_s[:, pl.ds(p * hf, AR + _HALO), :] = jnp.zeros((8, AR + _HALO, 128), _F32)
                qf_s[:, pl.ds(p * hf, AR), :] = jnp.zeros((8, AR, 128), _F32)
            xcp(0).wait()
            for c in kvcp(0):
                c.start()
            norm1(0, hf)[0]()

        def q0_step(j, _):
            qcp(j).wait()
            q_s[pl.ds(0, hf), _rows(j, QC)] = _pack(_dot(_unpack(normed(0)), w_in[:, _rows(j, QC)]))

        with scope("sc_q0"):
            jax.lax.fori_loop(0, D // QC, q0_step, None)
            xcp(1).wait()
            norm1(1, hf)[0]()

        def q_step(i, _):
            @pl.when(i < NK)
            def _():
                xcp(i + 2).start()
                for c in kvcp(i):
                    c.start()

            @pl.when(i == NK - 1)
            def _():
                for j in range(NK + 2, n):
                    xcp(j).start()

            @pl.when(i == NK)
            def _():
                ocp.start()
                for c in fcp(0):
                    c.start()

            @pl.when(i + 1 < n)
            def _():
                xcp(i + 1).wait()

            @pl.when((i > 1) & (i < NK + 2))
            def _():
                for c in kvcp(i - 2):
                    c.wait()
            prep = []
            for j, w in enumerate((wk, wv)):
                src = [w_in.at[_rows(p, hd), _rows(jnp.where(i > 1, j + 1, 0), D)].at[_clamped(i - 2, KR, hd)] for p in range(2)]
                prep += [_prepare_kv_weight(*src, w.at[:, _clamped(i - 2, KR // 2, hd // 2), :], r0) for r0 in range(0, KR, 16)]
            y = _dot_paced(normed(i), _words(w_in[:, pl.ds(0, D)]), zero_s[...],
                           [_arrange(prep, CFG["PM"]), norm1(jnp.minimum(i + 1, n - 1), LR)], CFG["F0"])
            q_s[_rows(i, hf), :] = _pack(y)

        with scope("sc_q"):
            jax.lax.fori_loop(1, n, q_step, None)

        def kv_step(i, _):
            @pl.when(i + 1 < NS)
            def _():
                for c in fcp(i + 1):
                    c.start()
            for c in fcp(i):
                c.wait()
            prep, gate = [], []
            for src, dst in ((wg_in, wg), (wu_in, wu), (wd_in, wd)):
                size = src.shape[2]
                tiles = [(r0, c0) for r0 in range(0, size, 16) for c0 in range(0, dst.shape[2], 128)]
                prep += [P(_right_operands, src.at[i % 2, 0], src.at[i % 2, 1], dst.at[:, _rows(i, size // 2), :],
                           _share(tiles, t, CFG["NJ"]), zero_s[...], gate) for t in range(CFG["NJ"])]

            def proj(z, w, dst, queues, first):
                dst = dst.at[:, _rows(i, TK, _HALO), :]
                if w.shape[0] == 2:
                    for t in range(TK // T):
                        wt = jnp.concatenate([w[p, _rows((i >> 8) if t else 0, D // 4), :] for p in range(2)], axis=0)
                        y = _dot_paced(normed((i + z) * (TK // T) + t), wt, zero_s[...],
                                       [_share(q, t, TK // T) for q in queues], 0 if t else first)
                        for c in range(8):
                            dst[c, pl.ds(_HALO + t * T, T), :] = y[:, c * 128:(c + 1) * 128]
                    return
                rows = _rows(i + z, TK // 4)
                left = lambda k: xl_s[_SUMS.index(k), rows, :] if k in _SUMS else xn_s[k - 2, rows, _rows(k - 2, hd)]
                m = {}
                for t, k in enumerate(_ORDER):
                    m[k] = _dot_paced(left(k), w[k], zero_s[...], [_share(q, t, 7) for q in queues], 0 if t else first)
                    if CFG["GK"]:
                        gate.append(_words(m[k][:8, CFG["GK"] * 128:][:, :128]) & zero_s[...])
                y = _combine(m)
                for t in range(TK // T):
                    for p in range(2):
                        for c in range(8):
                            dst[c, pl.ds(_HALO + t * T + p * hf, hf), :] = (
                                y[2 * p + c // 4][t * hf:(t + 1) * hf, c % 4 * 128:(c % 4 + 1) * 128])

            step = i - (NS - pl.cdiv(hf, AR))
            views = [[ref.at[:, _rows(p, hf, extra), :].at[:, _clamped(step, AR, hf, extra), :]
                      for ref, extra in ((qf_s, 0), (k_s, _HALO), (v_s, _HALO))] for p in range(2)]
            att = _attention_pairs(views, keep_s, o_s.at[:, _clamped(step, AR // 2, hf // 2), :],
                                   jnp.clip(step * AR, 0, hf - AR), CFG["AM0"], gate)
            proj(0, wv, v_s, [_share(prep, 0, 2), _merge(_prepare_out_weight(wo_in, wo32, wo, i), sum([a[:-1] for a in att], []))], 1)
            for c in range(8):
                v_s[c, pl.ds(0, _HALO), :] = jnp.broadcast_to(v_s[c, pl.ds(_HALO, 1), :], (_HALO, 128))
            jobs = [_prepare_q(q_s.at[_rows(i, TK // 2)], qf_s.at[:, _rows(i, TK), :], r0, QR) for r0 in range(0, TK, QR)]
            proj(i >> 8, wk, k_s, [_share(prep, 1, 2), _merge(_arrange(jobs, CFG["QM"]), [a[-1] for a in att])], 0)

        with scope("sc_kv"):
            ocp.wait()
            jax.lax.fori_loop(0, NS, kv_step, None)

        def ocopy(i):
            return pltpu.make_async_copy(x_s.at[_rows(i, hf)], out_hbm.at[_rows(i, hf)], osem.at[i])

        def main_step(i, _):
            zero = zero_s[...]
            lr = CFG["LR2"]
            z = i >> 8
            hs = (ha_s, hb_s)
            early = _ORDER[:2]

            def norm(p, r0):
                y = _layernorm(hs[p].at[_rows(z, hf)][pl.ds(r0, lr), :])
                if p:
                    up = na_s.at[_rows(z, hf)][pl.ds(r0, lr), :]
                else:
                    na_s[pl.ds(r0, lr), :] = up = y
                left = _left(up[:, :hd], up[:, hd:], y[:, :hd], y[:, hd:])
                ys = {k: _pack(left[k]) for k in range(7) if (k in early) != bool(p)}
                for k, v in ys.items():
                    (hnb_s if p else hna_s).at[k][pl.ds(r0 // 2, lr // 2), :] = v
                return _token([ys[1 if p else 4]])

            def residual(p, c1, c2):
                for t, c in enumerate((c1, c2)):
                    hs[p][:, _rows(t, hd)] = x_s[_rows(2 * i + p, hf), _rows(t, hd)].astype(_F32) + c

            norms = [[P(norm, p, r0) for r0 in range(0, hf, lr)] for p in range(2)]
            m = {k: _dot_paced(o_s[k], wo[k], zero) for k in (2, 4, 3, 0, 6)}
            residual(0, ((m[3] - m[4]) + m[0]) + m[6], m[2] + m[4])
            f1 = CFG.get("F1", 2)
            m[1] = _dot_paced(o_s[1], wo[1], zero, [norms[0][:f1]], 3)
            m[5] = _dot_paced(o_s[5], wo[5], zero, [norms[0][f1:]])
            residual(1, *_combine(m)[2:])

            hn = lambda k, use: (hna_s if k in early else hnb_s).at[k][_rows(i >> (8 + use * CFG['U']), hf // 2), :]
            j = jnp.minimum(i + 1, n - 1)
            views = [[ref.at[:, _rows(2 * j + p, hf, extra), :] for ref, extra in ((qf_s, 0), (k_s, _HALO), (v_s, _HALO))]
                     for p in range(2)]
            gate = []
            att = sum(_attention_pairs(views, keep_s, o_s, None, CFG["AM"], gate), [])
            chunks = list(zip(np.cumsum((0,) + FC).tolist(), FC))
            down_order = (1, 3, 6, 0, 2, 4, 5)
            steps = [(0, w, k) for w in "gu" for k in early]
            for c in range(len(chunks)):
                steps += [(c, w, k) for w in "gud" for k in (down_order if w == "d" else _ORDER) if (c, w, k) not in steps]
            slots = [st for st in steps[4:] if st[1] in CFG["ON"]][CFG["S0"]:CFG["S1"]]
            jobs = {st: _share(att, t, len(slots)) for t, st in enumerate(slots)}
            jobs.update({steps[1 + t]: _share(norms[1], t, 3) for t in range(3)})
            prod, down = {}, {}
            for st in steps:
                c, w, k = st
                c0, width = chunks[c]
                if w == "d":
                    if k == down_order[0]:
                        g, u = (_combine([prod[c, v, t] for t in range(7)]) for v in "gu")
                        left = _left(*[_geglu(*gu) for gu in zip(g, u)])
                    cuts = sorted({0, width // 512 * 512, width})
                    for t, (k0, k1) in enumerate(zip(cuts, cuts[1:])):
                        y = _dot_paced(left[k][:, k0:k1].astype(_BF16), wd.at[k][pl.ds((c0 + k0) // 2, (k1 - k0) // 2), :], zero,
                                       [] if t else [jobs.get(st)])
                        down[k] = down[k] + y if k in down else y
                else:
                    prod[st] = y = _dot_paced(hn(k, 2 * c + (w == 'u')), (wg if w == "g" else wu)[k, :, pl.ds(c0, width)], zero, [jobs.get(st)])
                if CFG['G']:
                    gate.append(_words(y[:8, CFG['GC'] * 128:][:, :128]) & zero)
            out = _combine(down)
            for p in range(2):
                for t in range(2):
                    x_s[_rows(2 * i + p, hf), _rows(t, hd)] = (hs[p][_rows(z, hf), _rows(t, hd)] + out[2 * p + t]).astype(_BF16)
                ocopy(2 * i + p).start()

        with scope("sc_main"):
            jax.lax.fori_loop(0, n, main_step, None)
        with scope("sc_tail"):
            for i in range(2 * n):
                ocopy(i).wait()

    vmem, dma = pltpu.VMEM, pltpu.SemaphoreType.DMA
    any_spec = pl.BlockSpec(memory_space=pl.ANY)
    out = pl.pallas_call(
        kernel,
        out_shape=jax.ShapeDtypeStruct((S, D), A_x.dtype),
        in_specs=[any_spec] * 6,
        out_specs=any_spec,
        scratch_shapes=[
            vmem((S, D), _BF16), vmem((D, 3 * D), _BF16), vmem((D, D), _BF16),
            vmem((2, 2, hd // NS, F), _BF16), vmem((2, 2, hd // NS, F), _BF16), vmem((2, 2, F // 2 // NS, D), _BF16),
            vmem((7, D // 4, F // 2), _I32), vmem((7, D // 4, F // 2), _I32), vmem((7, F // 4, hd), _I32),
            *[vmem((7, D // 4, hd) if f else (2, D // 4, D), _I32) for f in (CFG['SK'], CFG['SV'], True)],
            vmem((2, _H * (_DH + 1), 128), _F32),
            vmem((2, S // 4, D), _I32), vmem((5, S // 4, hd), _I32), vmem((S // 2, D), _I32), vmem((8, S + 8, 128), _F32),
            vmem((8, S + _HALO + 8, 128), _F32), vmem((8, S + _HALO + 8, 128), _F32),
            vmem((8, hf, 128), _F32), vmem((7, hf // 2, hd), _I32),
            vmem((hf, D), _F32), vmem((hf, D), _F32), vmem((hf, D), _F32),
            vmem((7, hf // 2, hd), _I32), vmem((7, hf // 2, hd), _I32),
            vmem((8, 128), _I32),
            dma((n + D // QC,)), dma((2 * NK + 1,)), dma((6 * NS,)), dma((2 * n,)),
        ],
        compiler_params=pltpu.CompilerParams(vmem_limit_bytes=126 * 1024 * 1024, flags=CFG["flags"]),
    )(A_x.reshape(S, D), A_wqkv, A_wo, B_w_gate, B_w_up, B_w_down)
    return out.reshape(B, S, D)
```

```python
import functools
import numpy as np
import jax
import jax.numpy as jnp
import jax.experimental.pallas as pl
import jax.experimental.pallas.tpu as pltpu

CFG = dict(FC=(128,) * 7, ST=13, LD=2, DC=(512, 384), GM=1, N0=4, A0=True, CR=True, CO=True, CL=True, TOK=(2,), F1=0, AS=64, AR_=0, LR=16, LR2=16, QR=64, F0=3, scopes=False, QC=256, TK=512, AR=48, KR=96, PM=2, QM=0, AM=3, AM0=1,
           ON='gud', S0=0, S1=-6, NJ=20, SK=True, U=1, G=0, GC=-2, GK=0, SV=True, QS=True,
           flags={'XLA_TPU_EVENLY_DISTRIBUTE_CRITICAL_NODES': True})

_H, _DH, _W, _DIL = 32, 32, 8, 2
_HALO = 16
_EPS = 1e-5
_F32, _BF16, _I32 = jnp.float32, jnp.bfloat16, jnp.int32
P = functools.partial


def _dot(a, b):
    return jnp.dot(a, b, preferred_element_type=_F32)


def _words(x):
    return pltpu.bitcast(x, _I32)


def _pack(x):
    return _words(x.astype(_BF16))


def _unpack(x):
    return pltpu.bitcast(x, _BF16)


def _rows(i, size, extra=0):
    return pl.ds(i * size if isinstance(i, int) else pl.multiple_of(i * size, size), size + extra)


def _clamped(i, size, total, extra=0):
    return pl.ds(pl.multiple_of(jnp.clip(i * size, 0, total - size), 8 if size % 16 else 16), size + extra)


def _token(parts):
    tiles = [p[r:r + 8, c:c + 128] for p in parts
             for r in range(0, p.shape[0], 8) for c in range(0, p.shape[1], 128)]
    return functools.reduce(jnp.bitwise_or, tiles)


def _dot_paced(a, w, zero, queues=(), first=0):
    if any(queues):
        nt, nk, step = w.shape[1] // 128, pl.cdiv(w.shape[0], 256), CFG["AS"]
        due = {}
        for queue in queues:
            for j, job in enumerate(queue):
                due.setdefault(divmod(first + ((j + 1) * (nt * nk - first) - 1) // len(queue), nk), []).append(job())
        due = {slot: _token(tokens) & zero for slot, tokens in due.items()}
        parts = []
        for r in range(0, w.shape[0], step):
            top = [w[r:r + 8, t * 128:(t + 1) * 128] for t in range(nt)]
            top = [v | due[t, r // 256] if (t, r // 256) in due and (r // 64 % 4 == [0, (t * nk + r // 256) % 4, 3][CFG['AR_']] % min(4, (w.shape[0] - r // 256 * 256) // 64)) else v for t, v in enumerate(top)]
            parts += [jnp.concatenate(top, axis=1), w[r + 8:r + step]]
        w = jnp.concatenate(parts, axis=0)
    return _dot(a if a.dtype == _BF16 else _unpack(a), _unpack(w))


def _share(jobs, j, parts):
    return jobs[j * len(jobs) // parts:(j + 1) * len(jobs) // parts]


def _merge(a, b):
    return sum([_share(a, j, len(b)) + [e] for j, e in enumerate(b)], [])


def _together(jobs):
    return lambda: functools.reduce(jnp.bitwise_or, [job() for job in jobs])


def _chain(jobs):
    return lambda: [job() for job in jobs][-1]


def _staggered(chains):
    depth = len(chains[0])
    return [_together([c[t - i] for i, c in enumerate(chains) if 0 <= t - i < depth])
            for t in range(len(chains) + depth - 1)]


def _arrange(chains, mode):
    return [[_chain(e) for e in chains], sum(chains, []), _staggered(chains)][mode]


def _left(a11, a12, a21, a22):
    return (a11 + a22, a21 + a22, a11, a22, a11 + a12, a21 - a11, a12 - a22)


def _right(b11, b12, b21, b22):
    return (b11 + b22, b11, b12 - b22, b21 - b11, b22, b11 + b12, b21 + b22)


def _combine(m):
    return (((m[3] - m[4]) + m[0]) + m[6], m[2] + m[4], m[1] + m[3], ((m[2] - m[1]) + m[0]) + m[5])


_ORDER = (2, 4, 1, 3, 0, 5, 6)

_HK = [[[" +-".find(ch) * 2 - 3 if ch != "." else 0 for ch in part] for part in row.split()] for row in (
    "+....... +-......+....... +...-...",
    ".+...... ...++-.-.-...... .-......",
    "...+.... ...+.......-+-.- ...-...+",
    "+.-..... ........+....... -.+.....",
    ".+-..... .........+...... .-+..+-.",
    "..+-.... ...........+.... ..++....",
    "++.+.... ...+............ ++.+....",
    ".....+.. .+...--.....+-.. .....-..",
    "......+. ..+......++...+. ..-...+.",
    "+...+... +.+.-........... ....+...",
    "..+...+. ......+.+.+-.... ..+.....",
    "...+...+ ...+...-....+.+- .......-",
    "....++.. .+..........-... --..++..",
    "....+.-. ..+............. ....-.+.",
    "+.....+. ..+.....-....... ..+.-...",
    ".....+.- ............+-.. .-.+.+.-",
    "......+- ..............+. ......--",
    "...+..+. ...........+..+. ..+....+",
    "+...++.. .+..-........... ++..-...",
    ".+-...-. ......+..-...... ..+..+-.",
    "...+.-.+ ...+...-....-+.. .+.-...+",
    "....++.+ ............+... ....++.+",
    "...+--.. ...+........-... --.....-",
    "++..++.. ...+-........... --......",
    ".+-..+-. ......+......... .....-+.",
    ".+.-.+.- ...+...-........ .+.-....",
)]
_HK_LEFT, _HK_RIGHT = ([[-c for c in row[k]] for row in _HK] for k in range(2))
_HK_OUT = [[-row[2][o] for row in _HK] for o in range(8)]


def _sums(rows, xs, share=True, ready=None):
    xs, ready = list(xs), list(ready or range(len(xs)))
    rows = [{j: c for j, c in enumerate(row) if c} for row in rows]
    while share:
        count = {}
        for row in rows:
            for a in row:
                for b in row:
                    if a < b:
                        count[a, b, row[a] * row[b]] = count.get((a, b, row[a] * row[b]), 0) + 1
        best = max(sorted(count), key=count.get, default=None)
        if best is None or count[best] < 2:
            break
        a, b, sign = best
        xs.append(xs[a] + xs[b] if sign > 0 else xs[a] - xs[b])
        ready.append(max(ready[a], ready[b]))
        for row in rows:
            if row.get(a, 0) * row.get(b, 0) == sign:
                row[len(xs) - 1] = row.pop(a)
                del row[b]
    out = []
    for row in rows:
        (j, sign), *rest = sorted(row.items(), key=lambda t: (ready[t[0]], t[0]))
        acc = xs[j]
        for j, c in rest:
            acc = acc + xs[j] if c == sign else acc - xs[j] if sign > 0 else xs[j] - acc
            sign = max(sign, c)
        out.append(acc if sign > 0 else -acc)
    return out


_HK_FIRST = (4, 1, 6, 5, 0, 3, 2, 12, 22, 21, 19, 20, 15, 18, 25, 24, 23, 13, 7, 14, 9, 8, 16, 17, 10, 11)
_HK_ORDER = (15, 24, 22, 18, 19, 21, 6, 23, 4, 13, 12, 16, 8, 3, 0, 14, 9, 25, 7, 20, 1, 5, 2, 17, 10, 11)


def _store_operands(dst, rows, cols, ys):
    ys = [_pack(y) for y in ys]
    for k, y in enumerate(ys):
        dst.at[k][rows, cols] = y
    return ys


def _load_f32(src, r0, rows, cols):
    return jnp.concatenate([src[pl.ds(r, 8), cols].astype(_F32) for r in range(r0, r0 + rows, 8)], axis=0)


def _right_operands(src, dst, r0, c0, d0):
    quarter = src.shape[2] // 4
    b = [src.at[j][pl.ds(r0, 16), pl.ds(k * quarter + c0, 128)].astype(_F32) for j in range(4) for k in range(4)]
    ys = _store_operands(dst, pl.ds(r0 // 2, 8), pl.ds(d0, 128), _sums(_HK_RIGHT, b, CFG["CR"]))
    return _token([ys[k] for k in CFG["TOK"]])


def _layernorm(x):
    xc = x - jnp.mean(x, axis=-1, keepdims=True)
    var = jnp.mean(xc * xc, axis=-1, keepdims=True)
    return xc * jax.lax.rsqrt(var + _EPS)


_SUMS = (0, 1, 4, 5, 6)


def _layernorm_left(src, plain, sums, r0, rows):
    hf, hd = src.shape[0] // 2, src.shape[1] // 2
    a, b = (_layernorm(src[pl.ds(p * hf + r0, rows), :].astype(_F32)) for p in range(2))
    ys = _store_operands(plain, pl.ds(r0 // 2, rows // 2), slice(None), (a, b))
    if CFG["SK"] or CFG["SV"]:
        left = _left(a[:, :hd], a[:, hd:], b[:, :hd], b[:, hd:])
        ys = _store_operands(sums, pl.ds(r0 // 2, rows // 2), slice(None), [left[k] for k in _SUMS])[1:3]
    return _token(ys)


def _geglu(g, u):
    c1 = float(np.sqrt(2.0 / np.pi))
    c2 = c1 * 0.044715
    th = jnp.tanh(g * (c1 + c2 * (g * g)))
    hu = (0.5 * g) * u
    return hu * th + hu


def _head_minor(load, store):
    vs = []
    lanes = lambda: jax.lax.broadcasted_iota(_I32, vs[0].shape, 1)

    def skew():
        vs.extend(pltpu.roll(load(g), 4 * g, 1) if g else load(g) for g in range(8))
        return _token(vs[1:])

    def exchange():
        us = [vs[-j % 8] for j in range(8)]
        for b in range(3):
            m = (lanes() & (4 << b)) != 0
            us = [jnp.where(m, us[(j - (1 << b)) % 8], us[j]) for j in range(8)]
        vs[:] = [pltpu.roll(u, 128 - 4 * j, 1) if j else u for j, u in enumerate(us)]
        return _token(vs[1:])

    def shuffle():
        lane = lanes()
        idx = (lane & 3) * 32 + (lane & 28) + (lane >> 5)
        return store([jnp.take_along_axis(v, idx, axis=1, mode="promise_in_bounds") for v in vs])

    return [skew, exchange, shuffle]


def _prepare_kv_weight(upper, lower, dst, r0):
    def load(g):
        return jnp.concatenate([_words(src[pl.ds(r0, 16), pl.ds(g * 128, 128)]) for src in (upper, lower)], axis=0)

    def store(vs):
        if dst.shape[0] == 2:
            for j, v in enumerate(vs):
                for p in range(2):
                    dst[p, pl.ds(r0 // 2, 8), pl.ds(j * 128, 128)] = v[8 * p:8 * p + 8]
            return _token(vs)
        vs = [_unpack(v).astype(_F32) for v in vs]
        return _token([_store_operands(dst, pl.ds(r0 // 2, 8), pl.ds(j * 128, 128),
                                       _right(vs[j][:16], vs[j + 4][:16], vs[j][16:], vs[j + 4][16:]))[0] for j in range(4)])
    return _head_minor(load, store)


def _prepare_q(src, dst, r0, rows):
    def store(vs):
        for j, v in enumerate(vs):
            if CFG["QS"]:
                dst[j, pl.ds(r0, rows // 2, stride=2), :] = pltpu.bitcast(v << 16, _F32)
                dst[j, pl.ds(r0 + 1, rows // 2, stride=2), :] = pltpu.bitcast(v & -65536, _F32)
            else:
                dst[j, pl.ds(r0, rows), :] = _unpack(v).astype(_F32)
        return _token(vs)
    return _head_minor(lambda g: src[pl.ds(r0 // 2, rows // 2), pl.ds(g * 128, 128)], store)


def _prepare_out_weight(src, tmp, dst, c):
    def spread(h0):
        ys = []
        for h in range(h0, h0 + 4):
            for k in range(2):
                ys.append(src[pl.ds(h * _DH, _DH), _rows(c + 4 * k, 128)].astype(_F32))
                tmp[k, pl.ds(h * (_DH + 1), _DH), :] = ys[-1]
        return _token([_words(y[:8]) for y in ys])

    def gather(d0):
        ys = []
        for d in range(d0, d0 + 2):
            b = [tmp[k, pl.ds(d + j * _DH // 2, _H, stride=_DH + 1), :] for j in range(2) for k in range(2)]
            ys.append(_store_operands(dst, pl.ds(d * _H // 2, _H // 2), _rows(c, 128), _right(*b))[0])
        return _token(ys)

    return [P(spread, h) for h in range(0, _H, 4)] + [P(gather, d) for d in range(0, _DH // 2, 2)]


def _after(x, gate):
    return x if not gate else pltpu.bitcast(_words(x) | jnp.tile(gate[-1], (x.shape[0] // 8, 1)), x.dtype)


def _attention(q_s, k_s, v_s, r0, pos0, store, mode, gate):
    rows, ls = 16, []

    def scores():
        q = [q_s[c, pl.ds(r0, rows), :] for c in range(8)]
        q[0] = _after(q[0], gate)
        for w in range(_W):
            s = _HALO + r0 - _DIL * w
            acc = q[0] * k_s[0, pl.ds(s, rows), :]
            for c in range(1, 8):
                acc = acc + q[c] * k_s[c, pl.ds(s, rows), :]
            ls.append(acc + pltpu.roll(acc, 64, 1))
        return _token([_words(l) for l in ls])

    def probs():
        for w in range(_W):
            l = (ls[w] + pltpu.roll(ls[w], 32, 1)) * (_DH ** -0.5)
            if pos0 is not None and r0 < _DIL * w:
                pos = pos0 + r0 + jax.lax.broadcasted_iota(_I32, l.shape, 0)
                l = jnp.where(pos >= _DIL * w, l, -1e9)
            ls[w] = l
        m = functools.reduce(jnp.maximum, ls)
        es = [jnp.exp(l - m) for l in ls]
        inv = 1.0 / functools.reduce(jnp.add, es)
        ls[:] = [e * inv for e in es]
        return _token([_words(inv)])

    def mix(c0, nc):
        p0 = _after(ls[0], gate if CFG['G'] > 1 else None)

        def group(c):
            acc = p0 * v_s[c, pl.ds(_HALO + r0, rows), :]
            for w in range(1, _W):
                acc = acc + ls[w] * v_s[c, pl.ds(_HALO + r0 - _DIL * w, rows), :]
            return acc
        return _token([y for c in range(c0, c0 + nc) for y in store(r0, c, group(c), group(c + 4))])

    return [[_chain([scores, probs, P(mix, 0, 4)])],
            [_chain([scores, probs]), P(mix, 0, 4)],
            [scores, probs, P(mix, 0, 4)],
            [scores, probs, P(mix, 0, 2), P(mix, 2, 2)],
            [scores, _chain([probs, P(mix, 0, 2)]), P(mix, 2, 2)]][mode]


def _attention_pairs(views, keep, dst, pos0, mode, gate):
    def store_upper(r0, c, a11, a12):
        keep[c, pl.ds(r0, 16), :] = a11
        keep[c + 4, pl.ds(r0, 16), :] = a12
        return [_words(a11), _words(a12)]

    def store_lower(r0, c, a21, a22):
        left = _left(keep[c, pl.ds(r0, 16), :], keep[c + 4, pl.ds(r0, 16), :], a21, a22)
        return _store_operands(dst, pl.ds(r0 // 2, 8), pl.ds(c * 128, 128), left)[1:2]

    return [_attention(*views[p], r0, None if p else pos0, store, mode, gate)
            for r0 in range(0, views[0][0].shape[1], 16) for p, store in enumerate((store_upper, store_lower))]


class _NoScope:
    def __init__(self, name):
        pass

    def __enter__(self):
        pass

    def __exit__(self, *a):
        pass


@jax.jit
def pallas_sequential_preLN__sliding_local_dilated__glu_gated_geglu__prompt_kernel(
    A_x, A_wqkv, A_wo, B_x, B_w_gate, B_w_up, B_w_down,
):
    del B_x
    B, S, D = A_x.shape
    F = B_w_gate.shape[1]
    T = 256
    n, hf, hd = S // T, T // 2, D // 2
    FC, LR, QR, QC, TK, AR, KR = (CFG[k] for k in ("FC", "LR", "QR", "QC", "TK", "AR", "KR"))
    NK, NS = 4, S // TK
    scope = jax.named_scope if CFG["scopes"] else _NoScope

    def kernel(x_hbm, wqkv_hbm, wo_hbm, wg_hbm, wu_hbm, wd_hbm, out_hbm,
               x_s, w_in, wo_in, wg_in, wu_in, wd_in, wgu, wd, wk, wv, wo, wo32,
               xn_s, xl_s, q_s, qf_s, k_s, v_s, keep_s, o_s, ha_s, hb_s, na_s, hna_s, hnb_s, zero_s,
               sem, ksem, fsem, osem):
        def xcp(i):
            return pltpu.make_async_copy(x_hbm.at[_rows(i, T)], x_s.at[_rows(i, T)], sem.at[i])

        def qcp(j):
            return pltpu.make_async_copy(wqkv_hbm.at[:, _rows(j, QC)], w_in.at[:, _rows(j, QC)], sem.at[n + j])

        def kvcp(j):
            at = lambda ref, p: ref.at[_rows(p * NK + j, hd // NK), pl.ds(D, 2 * D)]
            return [pltpu.make_async_copy(at(wqkv_hbm, p), at(w_in, p), ksem.at[2 * j + p]) for p in range(2)]

        ocp = pltpu.make_async_copy(wo_hbm, wo_in, ksem.at[2 * NK])

        def fcp(i):
            return [pltpu.make_async_copy(w.at[:, _rows(i, w.shape[1] // NS), :], dst.at[i % 2], fsem.at[i * 3 + k])
                    for k, (w, dst) in enumerate(((wg_hbm, wg_in), (wu_hbm, wu_in), (wd_hbm, wd_in)))]

        def norm1(i, rows):
            at = lambda ref: ref.at[:, _rows(i, hf // 2), :]
            return [P(_layernorm_left, x_s.at[_rows(i, T)], at(xn_s), at(xl_s), r0, rows) for r0 in range(0, hf, rows)]

        def normed(i):
            return jnp.concatenate([xn_s[p, _rows(i, hf // 2), :] for p in range(2)], axis=0)

        with scope("sc_p0"):
            for c in [xcp(0)] + [qcp(j) for j in range(D // QC)] + [xcp(1), xcp(2)]:
                c.start()
            zero_s[...] = jnp.zeros((8, 128), _I32)
            for p in range(2):
                k_s[:, pl.ds(p * hf, AR + _HALO), :] = jnp.zeros((8, AR + _HALO, 128), _F32)
                qf_s[:, pl.ds(p * hf, AR), :] = jnp.zeros((8, AR, 128), _F32)
            xcp(0).wait()
            for c in kvcp(0):
                c.start()
            norm1(0, hf)[0]()

        def q0_step(j, _):
            qcp(j).wait()
            q_s[pl.ds(0, hf), _rows(j, QC)] = _pack(_dot(_unpack(normed(0)), w_in[:, _rows(j, QC)]))

        with scope("sc_q0"):
            jax.lax.fori_loop(0, D // QC, q0_step, None)
            xcp(1).wait()
            norm1(1, hf)[0]()

        def q_step(i, _):
            @pl.when(i < NK)
            def _():
                xcp(i + 2).start()
                for c in kvcp(i):
                    c.start()

            @pl.when(i == NK - 1)
            def _():
                for j in range(NK + 2, n):
                    xcp(j).start()

            @pl.when(i == NK)
            def _():
                ocp.start()
                for c in fcp(0):
                    c.start()

            @pl.when(i + 1 < n)
            def _():
                xcp(i + 1).wait()

            @pl.when((i > 1) & (i < NK + 2))
            def _():
                for c in kvcp(i - 2):
                    c.wait()
            prep = []
            for j, w in enumerate((wk, wv)):
                src = [w_in.at[_rows(p, hd), _rows(jnp.where(i > 1, j + 1, 0), D)].at[_clamped(i - 2, KR, hd)] for p in range(2)]
                prep += [_prepare_kv_weight(*src, w.at[:, _clamped(i - 2, KR // 2, hd // 2), :], r0) for r0 in range(0, KR, 16)]
            y = _dot_paced(normed(i), _words(w_in[:, pl.ds(0, D)]), zero_s[...],
                           [_arrange(prep, CFG["PM"]), norm1(jnp.minimum(i + 1, n - 1), LR)], CFG["F0"])
            q_s[_rows(i, hf), :] = _pack(y)

        with scope("sc_q"):
            jax.lax.fori_loop(1, n, q_step, None)

        def kv_step(i, _):
            @pl.when(i + 1 < NS)
            def _():
                for c in fcp(i + 1):
                    c.start()
            for c in fcp(i):
                c.wait()
            prep, gate = [], []
            for src, dst, scale, shift in ((wg_in, wgu, 2, 0), (wu_in, wgu, 2, 128), (wd_in, wd, 1, 0)):
                size = src.shape[2]
                prep += [P(_right_operands, src.at[i % 2], dst.at[:, _rows(i, size // 2), :], r0, c0, scale * c0 + shift)
                         for r0 in range(0, size, 16) for c0 in range(0, src.shape[3] // 4, 128)]

            def proj(z, w, dst, queues, first):
                dst = dst.at[:, _rows(i, TK, _HALO), :]
                if w.shape[0] == 2:
                    for t in range(TK // T):
                        wt = jnp.concatenate([w[p, _rows((i >> 8) if t else 0, D // 4), :] for p in range(2)], axis=0)
                        y = _dot_paced(normed((i + z) * (TK // T) + t), wt, zero_s[...],
                                       [_share(q, t, TK // T) for q in queues], 0 if t else first)
                        for c in range(8):
                            dst[c, pl.ds(_HALO + t * T, T), :] = y[:, c * 128:(c + 1) * 128]
                    return
                rows = _rows(i + z, TK // 4)
                left = lambda k: xl_s[_SUMS.index(k), rows, :] if k in _SUMS else xn_s[k - 2, rows, _rows(k - 2, hd)]
                m = {}
                for t, k in enumerate(_ORDER):
                    m[k] = _dot_paced(left(k), w[k], zero_s[...], [_share(q, t, 7) for q in queues], 0 if t else first)
                    if CFG["GK"]:
                        gate.append(_words(m[k][:8, CFG["GK"] * 128:][:, :128]) & zero_s[...])
                y = _combine(m)
                for t in range(TK // T):
                    for p in range(2):
                        for c in range(8):
                            dst[c, pl.ds(_HALO + t * T + p * hf, hf), :] = (
                                y[2 * p + c // 4][t * hf:(t + 1) * hf, c % 4 * 128:(c % 4 + 1) * 128])

            step = i - (NS - pl.cdiv(hf, AR))
            views = [[ref.at[:, _rows(p, hf, extra), :].at[:, _clamped(step, AR, hf, extra), :]
                      for ref, extra in ((qf_s, 0), (k_s, _HALO), (v_s, _HALO))] for p in range(2)]
            att = _attention_pairs(views, keep_s, o_s.at[:, _clamped(step, AR // 2, hf // 2), :],
                                   jnp.clip(step * AR, 0, hf - AR), CFG["AM0"], gate)
            proj(0, wv, v_s, [_share(prep, 0, 2), _merge(_prepare_out_weight(wo_in, wo32, wo, i), sum([a[:-1] for a in att], []))], 1)
            for c in range(8):
                v_s[c, pl.ds(0, _HALO), :] = jnp.broadcast_to(v_s[c, pl.ds(_HALO, 1), :], (_HALO, 128))
            jobs = [_prepare_q(q_s.at[_rows(i, TK // 2)], qf_s.at[:, _rows(i, TK), :], r0, QR) for r0 in range(0, TK, QR)]
            proj(i >> 8, wk, k_s, [_share(prep, 1, 2), _merge(_arrange(jobs, CFG["QM"]), [a[-1] for a in att])], 0)

        with scope("sc_kv"):
            ocp.wait()
            jax.lax.fori_loop(0, NS, kv_step, None)

        def ocopy(i):
            return pltpu.make_async_copy(x_s.at[_rows(i, hf)], out_hbm.at[_rows(i, hf)], osem.at[i])

        def main_step(i, _):
            zero = zero_s[...]
            lr = CFG["LR2"]
            z = i >> 8
            hs = (ha_s, hb_s)
            early, qd = 7, D // 4

            def norm(p, r0):
                y = _layernorm(hs[p].at[_rows(z, hf)][pl.ds(r0, lr), :])
                if p:
                    up = na_s.at[_rows(z, hf)][pl.ds(r0, lr), :]
                else:
                    na_s[pl.ds(r0, lr), :] = up = y
                blocks = [v[:, k * qd:(k + 1) * qd] for v in (up, y) for k in range(4)]
                left = _sums(_HK_LEFT[early:] if p else _HK_LEFT[:early], blocks)
                return _token(_store_operands(hnb_s if p else hna_s, pl.ds(r0 // 2, lr // 2), slice(None), left)[-3:])

            def residual(p, c1, c2):
                for t, c in enumerate((c1, c2)):
                    hs[p][:, _rows(t, hd)] = x_s[_rows(2 * i + p, hf), _rows(t, hd)].astype(_F32) + c

            norms = [[P(norm, p, r0) for r0 in range(0, hf, lr)] for p in range(2)]
            m = {k: _dot_paced(o_s[k], wo[k], zero) for k in (2, 4, 3, 0, 6)}
            residual(0, ((m[3] - m[4]) + m[0]) + m[6], m[2] + m[4])
            f1 = CFG.get("F1", 2)
            m[1] = _dot_paced(o_s[1], wo[1], zero, [norms[0][:f1]], 3)
            m[5] = _dot_paced(o_s[5], wo[5], zero, [norms[0][f1:]])
            residual(1, *_combine(m)[2:])

            hn = lambda k, use: (hna_s.at[k] if k < early else hnb_s.at[k - early])[_rows(i >> (8 + use), hf // 2), :]
            j = jnp.minimum(i + 1, n - 1)
            views = [[ref.at[:, _rows(2 * j + p, hf, extra), :] for ref, extra in ((qf_s, 0), (k_s, _HALO), (v_s, _HALO))]
                     for p in range(2)]
            gate = []
            att = sum(_attention_pairs(views, keep_s, o_s, None, CFG["AM"], gate), [])
            chunks = list(zip(np.cumsum((0,) + FC).tolist(), FC))
            downs = list(zip(np.cumsum((0,) + CFG["DC"]).tolist(), CFG["DC"]))
            lead = CFG['LD']
            orders = [_HK_FIRST if u < lead else _HK_ORDER for u in range(len(chunks))]
            ups = sorted([(t if u < lead and t < early else t + CFG["ST"] * u, u, k) for u, order in enumerate(orders) for t, k in enumerate(order)])
            steps = [("u", u, k) for _, u, k in ups] + [("w", u, k) for u in range(len(downs)) for k in _HK_ORDER]
            jobs = {st: [] for st in steps}

            def spread(queue, steps):
                for t, st in enumerate(steps):
                    jobs[st].append(_share(queue, t, len(steps)))

            def activation(u):
                ready = [orders[u].index(k) for k in range(26)]
                half = lambda y, p: jnp.concatenate([y[:, t:t + 128] for t in range(p * 128, y.shape[1], 256)], axis=1)
                gu = _sums(_HK_OUT, [prod["u", u, k] for k in range(26)], CFG["CO"], ready)
                ready = [max(t for t, c in zip(ready, row) if c) for row in _HK_OUT]
                return _sums(_HK_LEFT, [_geglu(half(y, 0), half(y, 1)) for y in gu], CFG["CL"], ready)

            spread(norms[1], steps[CFG["N0"]:early * lead])
            spread(att, steps[len(ups):][CFG["S0"]:CFG["S1"]] if not CFG["A0"] else steps[early * lead:CFG["S1"]])
            prod, down = {}, {}
            for st in steps:
                w, u, k = st
                if w == "w":
                    if not down:
                        left = [jnp.concatenate(v, axis=1) for v in zip(*[activation(t) for t in range(len(chunks))])]
                    c0, width = downs[u]
                    y = _dot_paced(left[k][:, c0:c0 + width].astype(_BF16), wd.at[k][pl.ds(c0 // 2, width // 2), :], zero, jobs[st])
                    down[k] = down[k] + y if c0 else y
                else:
                    c0, width = chunks[u]
                    prod[st] = _dot_paced(hn(k, u), wgu.at[k][:, pl.ds(2 * c0, 2 * width)], zero, jobs[st])
            out = _sums(_HK_OUT, [down[k] for k in range(26)], CFG["CO"], [_HK_ORDER.index(k) for k in range(26)])
            for p in range(2):
                for t in range(4):
                    x_s[_rows(2 * i + p, hf), _rows(t, qd)] = (hs[p][_rows(z, hf), _rows(t, qd)] + out[4 * p + t]).astype(_BF16)
                ocopy(2 * i + p).start()

        with scope("sc_main"):
            jax.lax.fori_loop(0, n, main_step, None)
        with scope("sc_tail"):
            for i in range(2 * n):
                ocopy(i).wait()

    vmem, dma = pltpu.VMEM, pltpu.SemaphoreType.DMA
    any_spec = pl.BlockSpec(memory_space=pl.ANY)
    out = pl.pallas_call(
        kernel,
        out_shape=jax.ShapeDtypeStruct((S, D), A_x.dtype),
        in_specs=[any_spec] * 6,
        out_specs=any_spec,
        scratch_shapes=[
            vmem((S, D), _BF16), vmem((D, 3 * D), _BF16), vmem((D, D), _BF16),
            vmem((2, 4, D // 4 // NS, F), _BF16), vmem((2, 4, D // 4 // NS, F), _BF16), vmem((2, 4, F // 4 // NS, D), _BF16),
            vmem((26, D // 8, F // 2), _I32), vmem((26, F // 8, D // 4), _I32),
            *[vmem((7, D // 4, hd) if f else (2, D // 4, D), _I32) for f in (CFG['SK'], CFG['SV'], True)],
            vmem((2, _H * (_DH + 1), 128), _F32),
            vmem((2, S // 4, D), _I32), vmem((5, S // 4, hd), _I32), vmem((S // 2, D), _I32), vmem((8, S + 8, 128), _F32),
            vmem((8, S + _HALO + 8, 128), _F32), vmem((8, S + _HALO + 8, 128), _F32),
            vmem((8, hf, 128), _F32), vmem((7, hf // 2, hd), _I32),
            vmem((hf, D), _F32), vmem((hf, D), _F32), vmem((hf, D), _F32),
            vmem((7, hf // 2, D // 4), _I32), vmem((19, hf // 2, D // 4), _I32),
            vmem((8, 128), _I32),
            dma((n + D // QC,)), dma((2 * NK + 1,)), dma((6 * NS,)), dma((2 * n,)),
        ],
        compiler_params=pltpu.CompilerParams(vmem_limit_bytes=126 * 1024 * 1024, flags=CFG["flags"]),
    )(A_x.reshape(S, D), A_wqkv, A_wo, *(w.reshape(4, w.shape[0] // 4, w.shape[1]) for w in (B_w_gate, B_w_up, B_w_down)))
    return out.reshape(B, S, D)
```

```python
import functools
import numpy as np
import jax
import jax.numpy as jnp
import jax.experimental.pallas as pl
import jax.experimental.pallas.tpu as pltpu

CFG = dict(FC=(128,) * 7, ST=13, LD=4, DC=(896,), TH=1, QV=0, TS=6, GM=1, N0=2, A0=True, CR=True, CO=True, CL=True, TOK=1, OP=((1, 0, 3), (0, 0, 2), (0, 2, 2), (1, 3, 1)), PV=8, OV=0, GR=True, F2=4, F1=0, AS=64, AR_=0, LR=16, LR2=16, QR=64, F0=2, scopes=False, QC=256, TK=512, AR=48, KR=96, PM=2, QM=2, AM=4, AM0=1,
           ON='gud', S0=0, S1=-3, NJ=20, SK=True, U=1, Z=1, G=0, GC=-2, GK=0, SV=True, QS=True,
           flags={'XLA_TPU_EVENLY_DISTRIBUTE_CRITICAL_NODES': True})

_H, _DH, _W, _DIL = 32, 32, 8, 2
_HALO = 16
_EPS = 1e-5
_F32, _BF16, _I32 = jnp.float32, jnp.bfloat16, jnp.int32
P = functools.partial


def _dot(a, b):
    return jnp.dot(a, b, preferred_element_type=_F32)


def _words(x):
    return pltpu.bitcast(x, _I32)


def _pack(x):
    return _words(x.astype(_BF16))


def _unpack(x):
    return pltpu.bitcast(x, _BF16)


def _rows(i, size, extra=0):
    return pl.ds(i * size if isinstance(i, int) else pl.multiple_of(i * size, size), size + extra)


def _clamped(i, size, total, extra=0):
    return pl.ds(pl.multiple_of(jnp.clip(i * size, 0, total - size), 8 if size % 16 else 16), size + extra)


def _token(parts):
    tiles = [p[r:r + 8, c:c + 128] for p in parts
             for r in range(0, p.shape[0], 8) for c in range(0, p.shape[1], 128)]
    return functools.reduce(jnp.bitwise_or, tiles)


def _dot_paced(a, w, zero, queues=(), first=0):
    if any(queues):
        nt, nk, step = w.shape[1] // 128, pl.cdiv(w.shape[0], 256), CFG["AS"]
        due = {}
        for queue in queues:
            for j, job in enumerate(queue):
                due.setdefault(divmod(first + ((j + 1) * (nt * nk - first) - 1) // len(queue), nk), []).append(job())
        due = {slot: _token(tokens) & zero for slot, tokens in due.items()}
        parts = []
        for r in range(0, w.shape[0], step):
            top = [w[r:r + 8, t * 128:(t + 1) * 128] for t in range(nt)]
            top = [v | due[t, r // 256] if (t, r // 256) in due and (r // 64 % 4 == [0, (t * nk + r // 256) % 4, 3][CFG['AR_']] % min(4, (w.shape[0] - r // 256 * 256) // 64)) else v for t, v in enumerate(top)]
            parts += [jnp.concatenate(top, axis=1), w[r + 8:r + step]]
        w = jnp.concatenate(parts, axis=0)
    return _dot(a if a.dtype == _BF16 else _unpack(a), _unpack(w))


def _share(jobs, j, parts):
    return jobs[j * len(jobs) // parts:(j + 1) * len(jobs) // parts]


def _merge(a, b):
    return sum([_share(a, j, len(b)) + [e] for j, e in enumerate(b)], [])


def _together(jobs):
    return lambda: functools.reduce(jnp.bitwise_or, [job() for job in jobs])


def _chain(jobs):
    return lambda: [job() for job in jobs][-1]


def _staggered(chains):
    depth = len(chains[0])
    return [_together([c[t - i] for i, c in enumerate(chains) if 0 <= t - i < depth])
            for t in range(len(chains) + depth - 1)]


def _arrange(chains, mode):
    return [[_chain(e) for e in chains], sum(chains, []), _staggered(chains)][mode]


def _left(a11, a12, a21, a22):
    return (a11 + a22, a21 + a22, a11, a22, a11 + a12, a21 - a11, a12 - a22)


def _right(b11, b12, b21, b22):
    return (b11 + b22, b11, b12 - b22, b21 - b11, b22, b11 + b12, b21 + b22)


def _combine(m):
    return (((m[3] - m[4]) + m[0]) + m[6], m[2] + m[4], m[1] + m[3], ((m[2] - m[1]) + m[0]) + m[5])


_ORDER = (2, 4, 1, 3, 0, 5, 6)

_HK = [[[" +-".find(ch) * 2 - 3 if ch != "." else 0 for ch in part] for part in row.split()] for row in (
    "+....... +-......+....... +...-...",
    ".+...... ...++-.-.-...... .-......",
    "...+.... ...+.......-+-.- ...-...+",
    "+.-..... ........+....... -.+.....",
    ".+-..... .........+...... .-+..+-.",
    "..+-.... ...........+.... ..++....",
    "++.+.... ...+............ ++.+....",
    ".....+.. .+...--.....+-.. .....-..",
    "......+. ..+......++...+. ..-...+.",
    "+...+... +.+.-........... ....+...",
    "..+...+. ......+.+.+-.... ..+.....",
    "...+...+ ...+...-....+.+- .......-",
    "....++.. .+..........-... --..++..",
    "....+.-. ..+............. ....-.+.",
    "+.....+. ..+.....-....... ..+.-...",
    ".....+.- ............+-.. .-.+.+.-",
    "......+- ..............+. ......--",
    "...+..+. ...........+..+. ..+....+",
    "+...++.. .+..-........... ++..-...",
    ".+-...-. ......+..-...... ..+..+-.",
    "...+.-.+ ...+...-....-+.. .+.-...+",
    "....++.+ ............+... ....++.+",
    "...+--.. ...+........-... --.....-",
    "++..++.. ...+-........... --......",
    ".+-..+-. ......+......... .....-+.",
    ".+.-.+.- ...+...-........ .+.-....",
)]
_HK_LEFT, _HK_RIGHT = ([[-c for c in row[k]] for row in _HK] for k in range(2))
_HK_OUT = [[-row[2][o] for row in _HK] for o in range(8)]


def _sums(rows, xs, share=True, ready=None):
    xs, ready = list(xs), list(ready or range(len(xs)))
    rows = [{j: c for j, c in enumerate(row) if c} for row in rows]
    while share:
        count = {}
        for row in rows:
            for a in row:
                for b in row:
                    if a < b:
                        count[a, b, row[a] * row[b]] = count.get((a, b, row[a] * row[b]), 0) + 1
        best = max(sorted(count), key=count.get, default=None)
        if best is None or count[best] < 2:
            break
        a, b, sign = best
        xs.append(xs[a] + xs[b] if sign > 0 else xs[a] - xs[b])
        ready.append(max(ready[a], ready[b]))
        for row in rows:
            if row.get(a, 0) * row.get(b, 0) == sign:
                row[len(xs) - 1] = row.pop(a)
                del row[b]
    out = []
    for row in rows:
        (j, sign), *rest = sorted(row.items(), key=lambda t: (ready[t[0]], t[0]))
        acc = xs[j]
        for j, c in rest:
            acc = acc + xs[j] if c == sign else acc - xs[j] if sign > 0 else xs[j] - acc
            sign = max(sign, c)
        out.append(acc if sign > 0 else -acc)
    return out


_HK_FIRST = (4, 1, 6, 5, 0, 3, 2, 12, 22, 21, 19, 20, 15, 18, 25, 24, 23, 13, 7, 14, 9, 8, 16, 17, 10, 11)
_HK_ORDER = (15, 24, 22, 18, 19, 21, 6, 23, 4, 13, 12, 16, 8, 3, 0, 14, 9, 25, 7, 20, 1, 5, 2, 17, 10, 11)


def _store_operands(dst, rows, cols, ys):
    ys = [_pack(y) for y in ys]
    for k, y in enumerate(ys):
        dst.at[k][rows, cols] = y
    return ys


def _load_f32(src, r0, rows, cols):
    return jnp.concatenate([src[pl.ds(r, 8), cols].astype(_F32) for r in range(r0, r0 + rows, 8)], axis=0)


_HK_GROUPS = ((2, 11, 15, 20, 21, 22, 25, 6), (8, 10, 13, 14, 16, 17, 19, 24, 3, 4, 5), (1, 7, 0, 9, 12, 18, 23))


def _right_operands(src, dst, r0, c0, d0, group):
    quarter = src.shape[2] // 4
    b = [src.at[j // 4][pl.ds(r0, 16), pl.ds(j % 4 * quarter + c0, 128)].astype(_F32)
         if any(_HK_RIGHT[k][j] for k in group) else None for j in range(16)]
    ys = [_pack(y) for y in _sums([_HK_RIGHT[k] for k in group], b)]
    for k, y in zip(group, ys):
        dst.at[k][pl.ds(r0 // 2, 8), pl.ds(d0, 128)] = y
    return _token(ys[:CFG["TOK"]])


def _layernorm(x):
    xc = x - jnp.mean(x, axis=-1, keepdims=True)
    var = jnp.mean(xc * xc, axis=-1, keepdims=True)
    return xc * jax.lax.rsqrt(var + _EPS)


_SUMS = (0, 1, 4, 5, 6)


def _layernorm_left(src, plain, sums, r0, rows):
    hd = src[0].shape[1] // 2
    a, b = (_layernorm(src[p][pl.ds(r0, rows), :].astype(_F32)) for p in range(2))
    ys = _store_operands(plain, pl.ds(r0 // 2, rows // 2), slice(None), (a, b))
    if CFG["SK"] or CFG["SV"]:
        left = _left(a[:, :hd], a[:, hd:], b[:, :hd], b[:, hd:])
        ys = _store_operands(sums, pl.ds(r0 // 2, rows // 2), slice(None), [left[k] for k in _SUMS])[1:3]
    return _token(ys)


def _geglu(g, u):
    c1 = float(np.sqrt(2.0 / np.pi))
    c2 = c1 * 0.044715
    th = jnp.tanh(g * (c1 + c2 * (g * g)))
    hu = (0.5 * g) * u
    return hu * th + hu


def _head_minor(load, store):
    vs = []
    lanes = lambda: jax.lax.broadcasted_iota(_I32, vs[0].shape, 1)

    def skew():
        vs.extend(pltpu.roll(load(g), 4 * g, 1) if g else load(g) for g in range(8))
        return _token(vs[CFG["TH"]:])

    def exchange():
        us = [vs[-j % 8] for j in range(8)]
        for b in range(3):
            m = (lanes() & (4 << b)) != 0
            us = [jnp.where(m, us[(j - (1 << b)) % 8], us[j]) for j in range(8)]
        vs[:] = [pltpu.roll(u, 128 - 4 * j, 1) if j else u for j, u in enumerate(us)]
        return _token(vs[CFG["TH"]:])

    def shuffle():
        lane = lanes()
        idx = (lane & 3) * 32 + (lane & 28) + (lane >> 5)
        return store([jnp.take_along_axis(v, idx, axis=1, mode="promise_in_bounds") for v in vs])

    return [skew, exchange, shuffle]


def _prepare_kv_weight(upper, lower, dst, r0):
    def load(g):
        return jnp.concatenate([_words(src[pl.ds(r0, 16), pl.ds(g * 128, 128)]) for src in (upper, lower)], axis=0)

    def store(vs):
        if dst.shape[0] == 2:
            for j, v in enumerate(vs):
                for p in range(2):
                    dst[p, pl.ds(r0 // 2, 8), pl.ds(j * 128, 128)] = v[8 * p:8 * p + 8]
            return _token(vs[CFG["TH"]:])
        vs = [_unpack(v).astype(_F32) for v in vs]
        return _token([_store_operands(dst, pl.ds(r0 // 2, 8), pl.ds(j * 128, 128),
                                       _right(vs[j][:16], vs[j + 4][:16], vs[j][16:], vs[j + 4][16:]))[0] for j in range(4)])
    return _head_minor(load, store)


def _prepare_q(src, dst, r0, rows):
    def store(vs):
        for j, v in enumerate(vs):
            dst[pl.ds(r0, rows), pl.ds(j * 128, 128)] = _unpack(v)
        return _token(vs[CFG["TH"]:])
    return _head_minor(lambda g: src[pl.ds(r0 // 2, rows // 2), pl.ds(g * 128, 128)], store)


def _prepare_out_weight(src, tmp, dst, c):
    def spread(h0):
        ys = []
        for h in range(h0, h0 + 4):
            for k in range(2):
                ys.append(src[pl.ds(h * _DH, _DH), _rows(c + 4 * k, 128)].astype(_F32))
                tmp[k, pl.ds(h * (_DH + 1), _DH), :] = ys[-1]
        return _token([_words(y[:8]) for y in ys])

    def gather(d0):
        ys = []
        for d in range(d0, d0 + 2):
            b = [tmp[k, pl.ds(d + j * _DH // 2, _H, stride=_DH + 1), :] for j in range(2) for k in range(2)]
            ys.append(_store_operands(dst, pl.ds(d * _H // 2, _H // 2), _rows(c, 128), _right(*b))[0])
        return _token(ys)

    return [P(spread, h) for h in range(0, _H, 4)] + [P(gather, d) for d in range(0, _DH // 2, 2)]


def _after(x, gate):
    return x if not gate else pltpu.bitcast(_words(x) | jnp.tile(gate[-1], (x.shape[0] // 8, 1)), x.dtype)


def _attention(q_s, k_s, v_s, r0, pos0, store, mode, gate):
    rows, ls = 16, []

    def scores():
        q = [q_s[pl.ds(r0, rows), pl.ds(c * 128, 128)].astype(_F32) for c in range(8)]
        q[0] = _after(q[0], gate)
        for w in range(_W):
            s = _HALO + r0 - _DIL * w
            acc = q[0] * k_s[0, pl.ds(s, rows), :]
            for c in range(1, 8):
                acc = acc + q[c] * k_s[c, pl.ds(s, rows), :]
            ls.append(acc + pltpu.roll(acc, 64, 1))
        return _token([_words(l) for l in ls[CFG["TS"]:]])

    def probs():
        for w in range(_W):
            l = (ls[w] + pltpu.roll(ls[w], 32, 1)) * (_DH ** -0.5)
            if pos0 is not None and r0 < _DIL * w:
                pos = pos0 + r0 + jax.lax.broadcasted_iota(_I32, l.shape, 0)
                l = jnp.where(pos >= _DIL * w, l, -1e9)
            ls[w] = l
        m = functools.reduce(jnp.maximum, ls)
        es = [jnp.exp(l - m) for l in ls]
        inv = 1.0 / functools.reduce(jnp.add, es)
        ls[:] = [e * inv for e in es]
        return _token([_words(inv)])

    def mix(c0, nc):
        p0 = _after(ls[0], gate if CFG['G'] > 1 else None)

        def group(c):
            acc = p0 * v_s[c, pl.ds(_HALO + r0, rows), :]
            for w in range(1, _W):
                acc = acc + ls[w] * v_s[c, pl.ds(_HALO + r0 - _DIL * w, rows), :]
            return acc
        return _token([y for c in range(c0, c0 + nc) for y in store(r0, c, group(c), group(c + 4))])

    return [[_chain([scores, probs, P(mix, 0, 4)])],
            [_chain([scores, probs]), P(mix, 0, 4)],
            [scores, probs, P(mix, 0, 4)],
            [scores, probs, P(mix, 0, 2), P(mix, 2, 2)],
            [scores, _chain([probs, P(mix, 0, 2)]), P(mix, 2, 2)]][mode]


def _attention_pairs(views, keep, dst, pos0, mode, gate):
    def store_upper(r0, c, a11, a12):
        keep[c, pl.ds(r0, 16), :] = a11
        keep[c + 4, pl.ds(r0, 16), :] = a12
        return [_words(a11), _words(a12)]

    def store_lower(r0, c, a21, a22):
        left = _left(keep[c, pl.ds(r0, 16), :], keep[c + 4, pl.ds(r0, 16), :], a21, a22)
        return _store_operands(dst, pl.ds(r0 // 2, 8), pl.ds(c * 128, 128), left)[1:2]

    return [_attention(*views[p], r0, None if p else pos0, store, mode, gate)
            for r0 in range(0, views[0][0].shape[0], 16) for p, store in enumerate((store_upper, store_lower))]


class _NoScope:
    def __init__(self, name):
        pass

    def __enter__(self):
        pass

    def __exit__(self, *a):
        pass


@jax.jit
def pallas_sequential_preLN__sliding_local_dilated__glu_gated_geglu__prompt_kernel(
    A_x, A_wqkv, A_wo, B_x, B_w_gate, B_w_up, B_w_down,
):
    del B_x
    B, S, D = A_x.shape
    F = B_w_gate.shape[1]
    T = 256
    n, hf, hd = S // T, T // 2, D // 2
    FC, LR, QR, QC, TK, AR, KR = (CFG[k] for k in ("FC", "LR", "QR", "QC", "TK", "AR", "KR"))
    NK, NS, NQ = 4, S // TK, D // QC
    scope = jax.named_scope if CFG["scopes"] else _NoScope

    def kernel(x_hbm, wqkv_hbm, wo_hbm, wg_hbm, wu_hbm, wd_hbm, out_hbm,
               x_s, w_in, wo_in, wg_in, wu_in, wd_in, wgu, wd, wk, wv, wo, wo32,
               xn_s, xl_s, wq, q_s, qf_s, k_s, v_s, keep_s, o_s, ha_s, hb_s, na_s, hna_s, hnb_s, zero_s,
               sem, ksem, fsem, osem):
        def xcp(i):
            return pltpu.make_async_copy(x_hbm.at[_rows(i, T)], x_s.at[_rows(i, T)], sem.at[i])

        def qcp(j):
            at = lambda ref, p: ref.at[_rows((2 + p) * NQ + j, hf // NQ)]
            return [pltpu.make_async_copy(a, b, sem.at[n + j]) for a, b in (
                (at(x_hbm, 0), at(x_s, 0)), (at(x_hbm, 1), at(x_s, 1)), (wqkv_hbm.at[:, _rows(j, QC)], w_in.at[:, _rows(j, QC)]))]

        def kvcp(j):
            at = lambda ref, p: ref.at[_rows(p * NK + j, hd // NK), pl.ds(D, 2 * D)]
            return [pltpu.make_async_copy(at(wqkv_hbm, p), at(w_in, p), ksem.at[j]) for p in range(2)]

        ocp = pltpu.make_async_copy(wo_hbm, wo_in, ksem.at[NK])

        def fcp(i):
            return [pltpu.make_async_copy(w.at[:, _rows(i, w.shape[1] // NS), :], dst.at[i % 2], fsem.at[i % 2])
                    for k, (w, dst) in enumerate(((wg_hbm, wg_in), (wu_hbm, wu_in), (wd_hbm, wd_in)))]

        def norm1(i, rows):
            at = lambda ref: ref.at[:, _rows(i, hf // 2), :]
            return [P(_layernorm_left, [x_s.at[_rows(2 * i + p, hf)] for p in range(2)], at(xn_s), at(xl_s), r0, rows) for r0 in range(0, hf, rows)]

        def normed(i):
            return jnp.concatenate([xn_s[p, _rows(i, hf // 2), :] for p in range(2)], axis=0)

        with scope("sc_p0"):
            for c in [xcp(0)] + qcp(0) + qcp(1):
                c.start()
            zero_s[...] = jnp.zeros((8, 128), _I32)
            for p in range(2):
                k_s[:, pl.ds(p * hf, AR + _HALO), :] = jnp.zeros((8, AR + _HALO, 128), _F32)
                qf_s[pl.ds(p * hf, AR), :] = jnp.zeros((AR, D), _BF16)
            xcp(0).wait()
            norm1(0, hf)[0]()

        def q0_step(j, _):
            @pl.when(j + 2 < NQ)
            def _():
                for c in qcp(j + 2):
                    c.start()

            @pl.when(j + 2 == NQ)
            def _():
                for c in [xcp(2)] + kvcp(0):
                    c.start()
            for c in qcp(j):
                c.wait()
            lr = hf // NQ
            at = lambda ref: ref.at[:, _rows(NQ + j, lr // 2), :]
            jobs = [P(_layernorm_left, [x_s.at[_rows((2 + p) * NQ + j, lr)] for p in range(2)], at(xn_s), at(xl_s), r0, 16)
                    for r0 in range(0, lr, 16)]
            wq[:, _rows(j, QC)] = w = _words(w_in[:, _rows(j, QC)])
            q_s[pl.ds(0, hf), _rows(j, QC)] = _pack(_dot_paced(normed(0), w, zero_s[...], [jobs], 2))

        with scope("sc_q0"):
            jax.lax.fori_loop(0, NQ, q0_step, None)

        def q_step(i, _):
            @pl.when(i < NK)
            def _():
                xcp(i + 2).start()
                for c in kvcp(i):
                    c.start()

            @pl.when(i == NK - 1)
            def _():
                for j in range(NK + 2, n):
                    xcp(j).start()

            @pl.when(i == NK)
            def _():
                ocp.start()
                for c in fcp(0):
                    c.start()

            @pl.when(i + 1 < n)
            def _():
                xcp(i + 1).wait()

            @pl.when((i > 1) & (i < NK + 2))
            def _():
                for c in kvcp(i - 2):
                    c.wait()
            prep = []
            for j, w in enumerate((wk, wv)):
                src = [w_in.at[_rows(p, hd), _rows(jnp.where(i > 1, j + 1, 0), D)].at[_clamped(i - 2, KR, hd)] for p in range(2)]
                prep += [_prepare_kv_weight(*src, w.at[:, _clamped(i - 2, KR // 2, hd // 2), :], r0) for r0 in range(0, KR, 16)]
            y = _dot_paced(normed(i), wq[...], zero_s[...],
                           [_arrange(prep, CFG["PM"]), norm1(jnp.minimum(i + 1, n - 1), LR)], CFG["F0"])
            q_s[_rows(i, hf), :] = _pack(y)

        with scope("sc_q"):
            jax.lax.fori_loop(1, n, q_step, None)

        def kv_step(i, _):
            @pl.when(i + 1 < NS)
            def _():
                for c in fcp(i + 1):
                    c.start()
            for c in fcp(i):
                c.wait()
            prep, gate = [], []
            for src, dst, scale, shift in ((wg_in, wgu, 2, 0), (wu_in, wgu, 2, 128), (wd_in, wd, 1, 0)):
                size = src.shape[2]
                prep += [P(_right_operands, src.at[i % 2], dst.at[:, _rows(i, size // 2), :], r0, c0, scale * c0 + shift, group)
                         for r0 in range(0, size, 16) for c0 in range(0, src.shape[3] // 4, 128)
                         for group in (_HK_GROUPS if CFG['GR'] else [range(26)])]

            def proj(z, w, dst, queues, first):
                dst = dst.at[:, _rows(i, TK, _HALO), :]
                if w.shape[0] == 2:
                    for t in range(TK // T):
                        wt = jnp.concatenate([w[p, _rows((i >> 8) if t else 0, D // 4), :] for p in range(2)], axis=0)
                        y = _dot_paced(normed((i + z) * (TK // T) + t), wt, zero_s[...],
                                       [_share(q, t, TK // T) for q in queues], 0 if t else first)
                        for c in range(8):
                            dst[c, pl.ds(_HALO + t * T, T), :] = y[:, c * 128:(c + 1) * 128]
                    return
                rows = _rows(i + z, TK // 4)
                left = lambda k: xl_s[_SUMS.index(k), rows, :] if k in _SUMS else xn_s[k - 2, rows, _rows(k - 2, hd)]
                m = {}
                for t, k in enumerate(_ORDER):
                    m[k] = _dot_paced(left(k), w[k], zero_s[...], [_share(q, t, 7) for q in queues], 0 if t else first)
                    if CFG["GK"]:
                        gate.append(_words(m[k][:8, CFG["GK"] * 128:][:, :128]) & zero_s[...])
                y = _combine(m)
                for t in range(TK // T):
                    for p in range(2):
                        for c in range(8):
                            dst[c, pl.ds(_HALO + t * T + p * hf, hf), :] = (
                                y[2 * p + c // 4][t * hf:(t + 1) * hf, c % 4 * 128:(c % 4 + 1) * 128])

            step = i - (NS - pl.cdiv(hf, AR))
            views = [[qf_s.at[_rows(p, hf)].at[_clamped(step, AR, hf)]]
                     + [ref.at[:, _rows(p, hf, _HALO), :].at[:, _clamped(step, AR, hf, _HALO), :] for ref in (k_s, v_s)]
                     for p in range(2)]
            att = _attention_pairs(views, keep_s, o_s.at[:, _clamped(step, AR // 2, hf // 2), :],
                                   jnp.clip(step * AR, 0, hf - AR), CFG["AM0"], gate)
            jobs = [_prepare_q(q_s.at[_rows(i, TK // 2)], qf_s.at[_rows(i, TK)], r0, QR) for r0 in range(0, TK, QR)]
            jobs = [[c[:CFG['QV']] for c in jobs], [c[CFG['QV']:] for c in jobs]]
            cut, outw = len(prep) * CFG['PV'] // 16, _prepare_out_weight(wo_in, wo32, wo, i)
            proj(0, wv, v_s, [prep[:cut], outw[:CFG['OV']], _arrange(jobs[0], 2) if CFG['QV'] else [], sum([a[:-1] for a in att], [])], 1)
            for c in range(8):
                v_s[c, pl.ds(0, _HALO), :] = jnp.broadcast_to(v_s[c, pl.ds(_HALO, 1), :], (_HALO, 128))
            proj(i >> 8, wk, k_s, [prep[cut:], outw[CFG['OV']:], _arrange(jobs[1], CFG["QM"]), [a[-1] for a in att]], 0)

        with scope("sc_kv"):
            ocp.wait()
            jax.lax.fori_loop(0, NS, kv_step, None)

        def main_step(i, _):
            zero = zero_s[...]
            lr = CFG["LR2"]
            z = (i >> 8) if CFG["Z"] else 0
            hs = (ha_s, hb_s)
            early, qd = 7, D // 4

            def norm(p, r0):
                y = _layernorm(hs[p].at[_rows(z, hf)][pl.ds(r0, lr), :])
                if p:
                    up = na_s.at[_rows(z, hf)][pl.ds(r0, lr), :]
                else:
                    na_s[pl.ds(r0, lr), :] = up = y
                blocks = [v[:, k * qd:(k + 1) * qd] for v in (up, y) for k in range(4)]
                left = _sums(_HK_LEFT[early:] if p else _HK_LEFT[:early], blocks)
                return _token(_store_operands(hnb_s if p else hna_s, pl.ds(r0 // 2, lr // 2), slice(None), left)[-3:])

            def residual(p, c1, c2):
                for t, c in enumerate((c1, c2)):
                    hs[p][:, _rows(t, hd)] = x_s[_rows(2 * i + p, hf), _rows(t, hd)].astype(_F32) + c

            norms = [[P(norm, p, r0) for r0 in range(0, hf, lr)] for p in range(2)]
            m = {k: _dot_paced(o_s[k], wo[k], zero) for k in (2, 4, 3, 0, 6)}
            residual(0, ((m[3] - m[4]) + m[0]) + m[6], m[2] + m[4])
            f1 = CFG.get("F1", 2)
            m[1] = _dot_paced(o_s[1], wo[1], zero, [norms[0][:f1]], 3)
            m[5] = _dot_paced(o_s[5], wo[5], zero, [norms[0][f1:CFG['F2']]])
            for job in norms[0][CFG['F2']:]:
                job()
            residual(1, *_combine(m)[2:])

            hn = lambda k, use: (hna_s.at[k] if k < early else hnb_s.at[k - early])[_rows([0, i >> (8 + use), i >> 8][CFG["U"]], hf // 2), :]
            j = jnp.minimum(i + 1, n - 1)
            views = [[qf_s.at[_rows(2 * j + p, hf)]] + [ref.at[:, _rows(2 * j + p, hf, _HALO), :] for ref in (k_s, v_s)]
                     for p in range(2)]
            gate = []
            att = sum(_attention_pairs(views, keep_s, o_s, None, CFG["AM"], gate), [])
            chunks = list(zip(np.cumsum((0,) + FC).tolist(), FC))
            downs = list(zip(np.cumsum((0,) + CFG["DC"]).tolist(), CFG["DC"]))
            lead = CFG['LD']
            orders = [_HK_FIRST if u < lead else _HK_ORDER for u in range(len(chunks))]
            ups = sorted([(t if u < lead and t < early else t + CFG["ST"] * u, u, k) for u, order in enumerate(orders) for t, k in enumerate(order)])
            steps = [("u", u, k) for _, u, k in ups] + [("w", u, k) for u in range(len(downs)) for k in _HK_ORDER]
            jobs = {st: [] for st in steps}

            def spread(queue, steps):
                for t, st in enumerate(steps):
                    jobs[st].append(_share(queue, t, len(steps)))

            def activation(u):
                ready = [orders[u].index(k) for k in range(26)]
                half = lambda y, p: jnp.concatenate([y[:, t:t + 128] for t in range(p * 128, y.shape[1], 256)], axis=1)
                gu = _sums(_HK_OUT, [prod["u", u, k] for k in range(26)], CFG["CO"], ready)
                ready = [max(t for t, c in zip(ready, row) if c) for row in _HK_OUT]
                return _sums(_HK_LEFT, [_geglu(half(y, 0), half(y, 1)) for y in gu], CFG["CL"], ready)

            spread(norms[1], steps[CFG["N0"]:early * lead])
            spread(att, steps[len(ups):][CFG["S0"]:CFG["S1"]] if not CFG["A0"] else steps[early * lead:CFG["S1"]])
            prod, down = {}, {}
            for st in steps:
                w, u, k = st
                if w == "w":
                    if not down:
                        left = [jnp.concatenate(v, axis=1) for v in zip(*[activation(t) for t in range(len(chunks))])]
                    c0, width = downs[u]
                    y = _dot_paced(left[k][:, c0:c0 + width].astype(_BF16), wd.at[k][pl.ds(c0 // 2, width // 2), :], zero, jobs[st])
                    down[k] = down[k] + y if c0 else y
                else:
                    c0, width = chunks[u]
                    prod[st] = _dot_paced(hn(k, u), wgu.at[k][:, pl.ds(2 * c0, 2 * width)], zero, jobs[st])
            out = _sums(_HK_OUT, [down[k] for k in range(26)], CFG["CO"], [_HK_ORDER.index(k) for k in range(26)])
            for p, t0, nt in CFG["OP"]:
                for t in range(t0, t0 + nt):
                    x_s[_rows(2 * i + p, hf), _rows(t, qd)] = (hs[p][_rows(z, hf), _rows(t, qd)] + out[4 * p + t]).astype(_BF16)
                at = lambda ref: ref.at[_rows(2 * i + p, hf), pl.ds(t0 * qd, nt * qd)]
                pltpu.make_async_copy(at(x_s), at(out_hbm), osem).start()

        with scope("sc_main"):
            jax.lax.fori_loop(0, n, main_step, None)
        with scope("sc_tail"):
            pltpu.make_async_copy(x_s, out_hbm, osem).wait()

    vmem, dma = pltpu.VMEM, pltpu.SemaphoreType.DMA
    any_spec = pl.BlockSpec(memory_space=pl.ANY)
    out = pl.pallas_call(
        kernel,
        out_shape=jax.ShapeDtypeStruct((S, D), A_x.dtype),
        in_specs=[any_spec] * 6,
        out_specs=any_spec,
        scratch_shapes=[
            vmem((S, D), _BF16), vmem((D, 3 * D), _BF16), vmem((D, D), _BF16),
            vmem((2, 4, D // 4 // NS, F), _BF16), vmem((2, 4, D // 4 // NS, F), _BF16), vmem((2, 4, F // 4 // NS, D), _BF16),
            vmem((26, D // 8, F // 2), _I32), vmem((26, F // 8, D // 4), _I32),
            *[vmem((7, D // 4, hd) if f else (2, D // 4, D), _I32) for f in (CFG['SK'], CFG['SV'], True)],
            vmem((2, _H * (_DH + 1), 128), _F32),
            vmem((2, S // 4, D), _I32), vmem((5, S // 4, hd), _I32), vmem((D // 2, D), _I32), vmem((S // 2, D), _I32), vmem((S, D), _BF16),
            vmem((8, S + _HALO + 8, 128), _F32), vmem((8, S + _HALO + 8, 128), _F32),
            vmem((8, hf, 128), _F32), vmem((7, hf // 2, hd), _I32),
            vmem((hf, D), _F32), vmem((hf, D), _F32), vmem((hf, D), _F32),
            vmem((7, hf // 2, D // 4), _I32), vmem((19, hf // 2, D // 4), _I32),
            vmem((8, 128), _I32),
            dma((n + D // QC,)), dma((NK + 1,)), dma((2,)), dma(()),
        ],
        compiler_params=pltpu.CompilerParams(vmem_limit_bytes=126 * 1024 * 1024, flags=CFG["flags"]),
    )(A_x.reshape(S, D), A_wqkv, A_wo, *(w.reshape(4, w.shape[0] // 4, w.shape[1]) for w in (B_w_gate, B_w_up, B_w_down)))
    return out.reshape(B, S, D)
```

```python
import functools

import jax
import jax.experimental.pallas as pl
import jax.experimental.pallas.tpu as pltpu
import jax.numpy as jnp
import numpy as np

_HEADS, _HEAD_DIM, _WINDOW, _DILATION = 32, 32, 8, 2
_HALO = 16
_EPS = 1e-5
_F32, _BF16, _I32 = jnp.float32, jnp.bfloat16, jnp.int32
_bind = functools.partial


def _words(x):
    return pltpu.bitcast(x, _I32)


def _pack(x):
    return _words(x.astype(_BF16))


def _unpack(x):
    return pltpu.bitcast(x, _BF16)


def _block(i, size, extra=0):
    return pl.ds(i * size if isinstance(i, int) else pl.multiple_of(i * size, size), size + extra)


def _clamped(i, size, total, extra=0):
    start = jnp.clip(i * size, 0, total - size)
    return pl.ds(pl.multiple_of(start, 8 if size % 16 else 16), size + extra)


def _store_packed(dst, rows, cols, ys):
    ys = [_pack(y) for y in ys]
    for k, y in enumerate(ys):
        dst.at[k][rows, cols] = y
    return ys


def _token(parts):
    return functools.reduce(jnp.bitwise_or, [
        p[r:r + 8, c:c + 128] for p in parts
        for r in range(0, p.shape[0], 8) for c in range(0, p.shape[1], 128)])


def _dot(a, w, zero, queues=(), first=0):
    if any(queues):
        nt, nk = w.shape[1] // 128, pl.cdiv(w.shape[0], 256)
        due = {}
        for queue in queues:
            for j, job in enumerate(queue):
                slot = first + ((j + 1) * (nt * nk - first) - 1) // len(queue)
                due.setdefault(divmod(slot, nk), []).append(job())
        parts = []
        for k in range(nk):
            top = [w[k * 256:k * 256 + 8, t * 128:(t + 1) * 128] for t in range(nt)]
            top = [v | (_token(due[t, k]) & zero) if (t, k) in due else v for t, v in enumerate(top)]
            parts += [jnp.concatenate(top, axis=1), w[k * 256 + 8:(k + 1) * 256]]
        w = jnp.concatenate(parts, axis=0)
    return jnp.dot(a if a.dtype == _BF16 else _unpack(a), _unpack(w), preferred_element_type=_F32)


def _share(jobs, j, parts):
    return jobs[j * len(jobs) // parts:(j + 1) * len(jobs) // parts]


def _chain(*jobs):
    return lambda: [job() for job in jobs][-1]


def _staggered(chains):
    depth = len(chains[0])
    return [_bind(lambda jobs: _token([job() for job in jobs]),
                  [c[t - i] for i, c in enumerate(chains) if 0 <= t - i < depth])
            for t in range(len(chains) + depth - 1)]


def _strassen_left(a11, a12, a21, a22):
    return (a11 + a22, a21 + a22, a11, a22, a11 + a12, a21 - a11, a12 - a22)


def _strassen_right(b11, b12, b21, b22):
    return (b11 + b22, b11, b12 - b22, b21 - b11, b22, b11 + b12, b21 + b22)


def _strassen_upper(m):
    return (((m[3] - m[4]) + m[0]) + m[6], m[2] + m[4])


def _strassen_lower(m):
    return (m[1] + m[3], ((m[2] - m[1]) + m[0]) + m[5])


_STRASSEN_SUMS = (0, 1, 4, 5, 6)

_HK = [[[{"+": 1, ".": 0, "-": -1}[ch] for ch in part] for part in line.split()] for line in (
    "+....... +-......+....... +...-...",
    ".+...... ...++-.-.-...... .-......",
    "...+.... ...+.......-+-.- ...-...+",
    "+.-..... ........+....... -.+.....",
    ".+-..... .........+...... .-+..+-.",
    "..+-.... ...........+.... ..++....",
    "++.+.... ...+............ ++.+....",
    ".....+.. .+...--.....+-.. .....-..",
    "......+. ..+......++...+. ..-...+.",
    "+...+... +.+.-........... ....+...",
    "..+...+. ......+.+.+-.... ..+.....",
    "...+...+ ...+...-....+.+- .......-",
    "....++.. .+..........-... --..++..",
    "....+.-. ..+............. ....-.+.",
    "+.....+. ..+.....-....... ..+.-...",
    ".....+.- ............+-.. .-.+.+.-",
    "......+- ..............+. ......--",
    "...+..+. ...........+..+. ..+....+",
    "+...++.. .+..-........... ++..-...",
    ".+-...-. ......+..-...... ..+..+-.",
    "...+.-.+ ...+...-....-+.. .+.-...+",
    "....++.+ ............+... ....++.+",
    "...+--.. ...+........-... --.....-",
    "++..++.. ...+-........... --......",
    ".+-..+-. ......+......... .....-+.",
    ".+.-.+.- ...+...-........ .+.-....",
)]
_HK_LEFT, _HK_RIGHT = ([line[k] for line in _HK] for k in range(2))
_HK_OUT = [[line[2][o] for line in _HK] for o in range(8)]
_HK_EARLY = 7
_HK_FIRST = (4, 1, 6, 5, 0, 3, 2, 12, 22, 21, 19, 20, 15, 18, 25, 24, 23, 13, 7, 14, 9, 8, 16, 17, 10, 11)
_HK_ORDER = (15, 24, 22, 18, 19, 21, 6, 23, 4, 13, 12, 16, 8, 3, 0, 14, 9, 25, 7, 20, 1, 5, 2, 17, 10, 11)
_HK_GROUPS = ((2, 11, 15, 20, 21, 22, 25, 6), (8, 10, 13, 14, 16, 17, 19, 24, 3, 4, 5), (1, 7, 0, 9, 12, 18, 23))


def _sums(rows, xs, ready=None):
    xs, ready = list(xs), list(ready or range(len(xs)))
    rows = [{j: c for j, c in enumerate(row) if c} for row in rows]
    while True:
        count = {}
        for row in rows:
            for pair in [(a, b, row[a] * row[b]) for a in row for b in row if a < b]:
                count[pair] = count.get(pair, 0) + 1
        best = max(sorted(count), key=count.get, default=None)
        if best is None or count[best] < 2:
            break
        a, b, sign = best
        xs.append(xs[a] + xs[b] if sign > 0 else xs[a] - xs[b])
        ready.append(max(ready[a], ready[b]))
        for row in rows:
            if row.get(a, 0) * row.get(b, 0) == sign:
                row[len(xs) - 1] = row.pop(a)
                del row[b]
    out = []
    for row in rows:
        (j, sign), *rest = sorted(row.items(), key=lambda t: (ready[t[0]], t[0]))
        acc = xs[j]
        for j, c in rest:
            acc = acc + xs[j] if c == sign else acc - xs[j] if sign > 0 else xs[j] - acc
            sign = max(sign, c)
        out.append(acc if sign > 0 else -acc)
    return out


def _layernorm(x):
    xc = x - jnp.mean(x, axis=-1, keepdims=True)
    var = jnp.mean(xc * xc, axis=-1, keepdims=True)
    return xc * jax.lax.rsqrt(var + _EPS)


def _geglu(g, u):
    c = float(np.sqrt(2.0 / np.pi))
    th = jnp.tanh(g * (c + (c * 0.044715) * (g * g)))
    half = (0.5 * g) * u
    return half * th + half


def _normalize_input(src, plain, sums, r0, rows):
    hd = src[0].shape[1] // 2
    a, b = (_layernorm(ref[pl.ds(r0, rows), :].astype(_F32)) for ref in src)
    at = pl.ds(r0 // 2, rows // 2)
    _store_packed(plain, at, slice(None), (a, b))
    left = _strassen_left(a[:, :hd], a[:, hd:], b[:, :hd], b[:, hd:])
    return _token(_store_packed(sums, at, slice(None), [left[k] for k in _STRASSEN_SUMS])[1:3])


def _heads_minor(load, store):
    vs = []
    lanes = lambda: jax.lax.broadcasted_iota(_I32, vs[0].shape, 1)

    def skew():
        vs.extend(pltpu.roll(load(g), 4 * g, 1) if g else load(g) for g in range(8))
        return _token(vs[1:])

    def exchange():
        us = [vs[-j % 8] for j in range(8)]
        for b in (1, 2, 4):
            moved = (lanes() & (4 * b)) != 0
            us = [jnp.where(moved, us[(j - b) % 8], us[j]) for j in range(8)]
        vs[:] = [pltpu.roll(u, 128 - 4 * j, 1) if j else u for j, u in enumerate(us)]
        return _token(vs[1:])

    def shuffle():
        lane = lanes()
        idx = (lane & 3) * 32 + (lane & 28) + (lane >> 5)
        return store([jnp.take_along_axis(v, idx, axis=1, mode="promise_in_bounds") for v in vs])

    return [skew, exchange, shuffle]


def _prepare_q(src, dst, r0, rows):
    def store(vs):
        for j, v in enumerate(vs):
            dst[pl.ds(r0, rows), _block(j, 128)] = _unpack(v)
        return _token(vs[1:])

    return _heads_minor(lambda g: src[pl.ds(r0 // 2, rows // 2), _block(g, 128)], store)


def _prepare_kv_weight(src, dst, r0):
    def load(g):
        return jnp.concatenate([_words(ref[pl.ds(r0, 16), _block(g, 128)]) for ref in src], axis=0)

    def store(vs):
        vs = [_unpack(v).astype(_F32) for v in vs]
        return _token([_store_packed(
            dst, pl.ds(r0 // 2, 8), _block(j, 128),
            _strassen_right(vs[j][:16], vs[j + 4][:16], vs[j][16:], vs[j + 4][16:]))[0] for j in range(4)])

    return _heads_minor(load, store)


def _prepare_out_weight(src, tmp, dst, c):
    pitch = _HEAD_DIM + 1

    def spread(h0):
        ys = []
        for h in range(h0, h0 + 4):
            for k in range(2):
                ys.append(src[_block(h, _HEAD_DIM), _block(c + 4 * k, 128)].astype(_F32))
                tmp[k, pl.ds(h * pitch, _HEAD_DIM), :] = ys[-1]
        return _token([_words(y[:8]) for y in ys])

    def gather(d0):
        ys = []
        for d in range(d0, d0 + 2):
            b = [tmp[k, pl.ds(d + j * _HEAD_DIM // 2, _HEADS, stride=pitch), :] for j in range(2) for k in range(2)]
            ys.append(_store_packed(dst, _block(d, _HEADS // 2), _block(c, 128), _strassen_right(*b))[0])
        return _token(ys)

    return ([_bind(spread, h) for h in range(0, _HEADS, 4)]
            + [_bind(gather, d) for d in range(0, _HEAD_DIM // 2, 2)])


def _prepare_ffn_weight(src, dst, r0, c0, d0, group):
    quarter = src.shape[2] // 4
    b = [src.at[j // 4][pl.ds(r0, 16), pl.ds(j % 4 * quarter + c0, 128)].astype(_F32)
         if any(_HK_RIGHT[k][j] for k in group) else None for j in range(16)]
    ys = [_pack(y) for y in _sums([_HK_RIGHT[k] for k in group], b)]
    for k, y in zip(group, ys):
        dst.at[k][pl.ds(r0 // 2, 8), pl.ds(d0, 128)] = y
    return ys[0]


def _attention(q_s, k_s, v_s, r0, pos0, store):
    ls = []
    window = lambda w: pl.ds(_HALO + r0 - _DILATION * w, 16)

    def scores():
        q = [q_s[pl.ds(r0, 16), _block(c, 128)].astype(_F32) for c in range(8)]
        for w in range(_WINDOW):
            acc = q[0] * k_s[0, window(w), :]
            for c in range(1, 8):
                acc = acc + q[c] * k_s[c, window(w), :]
            ls.append(acc + pltpu.roll(acc, 64, 1))
        return _token([_words(l) for l in ls[-2:]])

    def softmax():
        for w in range(_WINDOW):
            l = (ls[w] + pltpu.roll(ls[w], 32, 1)) * (_HEAD_DIM ** -0.5)
            if pos0 is not None and r0 < _DILATION * w:
                pos = pos0 + r0 + jax.lax.broadcasted_iota(_I32, l.shape, 0)
                l = jnp.where(pos >= _DILATION * w, l, -1e9)
            ls[w] = l
        top = functools.reduce(jnp.maximum, ls)
        es = [jnp.exp(l - top) for l in ls]
        inv = 1.0 / functools.reduce(jnp.add, es)
        ls[:] = [e * inv for e in es]
        return _token([_words(inv)])

    def mix(*groups):
        def weighted(c):
            acc = ls[0] * v_s[c, window(0), :]
            for w in range(1, _WINDOW):
                acc = acc + ls[w] * v_s[c, window(w), :]
            return acc

        return _token([y for c in groups for y in store(r0, c, weighted(c), weighted(c + 4))])

    return scores, softmax, mix


def _attention_halves(views, keep, dst, pos0):
    def store_upper(r0, c, a11, a12):
        keep[c, pl.ds(r0, 16), :] = a11
        keep[c + 4, pl.ds(r0, 16), :] = a12
        return [_words(a11), _words(a12)]

    def store_lower(r0, c, a21, a22):
        left = _strassen_left(keep[c, pl.ds(r0, 16), :], keep[c + 4, pl.ds(r0, 16), :], a21, a22)
        return _store_packed(dst, pl.ds(r0 // 2, 8), _block(c, 128), left)[1:2]

    return [_attention(*views[p], r0, None if p else pos0, store)
            for r0 in range(0, views[0][0].shape[0], 16) for p, store in enumerate((store_upper, store_lower))]


@jax.jit
def pallas_sequential_preLN__sliding_local_dilated__glu_gated_geglu__prompt_kernel(
    A_x: jax.Array,
    A_wqkv: jax.Array,
    A_wo: jax.Array,
    B_x: jax.Array,
    B_w_gate: jax.Array,
    B_w_up: jax.Array,
    B_w_down: jax.Array,
):
    del B_x
    B, S, D = A_x.shape
    F = B_w_gate.shape[1]
    assert (B, S, D) == (1, 2048, _HEADS * _HEAD_DIM) and F % 512 == 0
    T = 256
    n, hf, hd, qd = S // T, T // 2, D // 2, D // 4
    NQ = NK = NS = 4
    QC, TK = D // NQ, S // NS
    KR, AR = 96, 48

    def kernel(x_hbm, wqkv_hbm, wo_hbm, wg_hbm, wu_hbm, wd_hbm, out_hbm,
               x_s, w_in, wo_in, wg_in, wu_in, wd_in, wgu, wd, wk, wv, wo, wo_tmp,
               xn_s, xsum_s, wq, qraw_s, q_s, k_s, v_s, keep_s, o_s, ha_s, hb_s, na_s, hna_s, hnb_s, zero_s,
               xsem, wsem, fsem, osem):
        def x_copy(i):
            return [pltpu.make_async_copy(x_hbm.at[_block(i, T)], x_s.at[_block(i, T)], xsem.at[i])]

        def q_copy(j):
            at = lambda ref, p: ref.at[_block((2 + p) * NQ + j, hf // NQ)]
            return [pltpu.make_async_copy(a, b, xsem.at[n + j]) for a, b in (
                (at(x_hbm, 0), at(x_s, 0)), (at(x_hbm, 1), at(x_s, 1)),
                (wqkv_hbm.at[:, _block(j, QC)], w_in.at[:, _block(j, QC)]))]

        def kv_copy(j):
            at = lambda ref, p: ref.at[_block(p * NK + j, hd // NK), pl.ds(D, 2 * D)]
            return [pltpu.make_async_copy(at(wqkv_hbm, p), at(w_in, p), wsem.at[j]) for p in range(2)]

        def o_copy():
            return [pltpu.make_async_copy(wo_hbm, wo_in, wsem.at[NK])]

        def ffn_copy(i):
            return [pltpu.make_async_copy(w.at[:, _block(i, w.shape[1] // NS), :], dst.at[i % 2], fsem.at[i % 2])
                    for w, dst in ((wg_hbm, wg_in), (wu_hbm, wu_in), (wd_hbm, wd_in))]

        def start(copies):
            for c in copies:
                c.start()

        def wait(copies):
            for c in copies:
                c.wait()

        def normalize(i, rows):
            at = lambda ref: ref.at[:, _block(i, hf // 2), :]
            src = [x_s.at[_block(2 * i + p, hf)] for p in range(2)]
            return [_bind(_normalize_input, src, at(xn_s), at(xsum_s), r0, rows) for r0 in range(0, hf, rows)]

        def normalized(i):
            return jnp.concatenate([xn_s[p, _block(i, hf // 2), :] for p in range(2)], axis=0)

        def first_q_step(j, _):
            pl.when(j + 2 < NQ)(lambda: start(q_copy(j + 2)))
            pl.when(j + 2 == NQ)(lambda: start(x_copy(2) + kv_copy(0)))
            wait(q_copy(j))
            rows = hf // NQ
            at = lambda ref: ref.at[:, _block(NQ + j, rows // 2), :]
            src = [x_s.at[_block((2 + p) * NQ + j, rows)] for p in range(2)]
            jobs = [_bind(_normalize_input, src, at(xn_s), at(xsum_s), r0, 16) for r0 in range(0, rows, 16)]
            wq[:, _block(j, QC)] = w = _words(w_in[:, _block(j, QC)])
            qraw_s[pl.ds(0, hf), _block(j, QC)] = _pack(_dot(normalized(0), w, zero_s[...], [jobs], 2))

        def q_step(i, _):
            pl.when(i < NK)(lambda: start(x_copy(i + 2) + kv_copy(i)))
            pl.when(i == NK - 1)(lambda: start(sum([x_copy(j) for j in range(NK + 2, n)], [])))
            pl.when(i == NK)(lambda: start(o_copy() + ffn_copy(0)))
            pl.when(i + 1 < n)(lambda: wait(x_copy(i + 1)))
            pl.when((i > 1) & (i < NK + 2))(lambda: wait(kv_copy(i - 2)))
            prepare = []
            for j, w in enumerate((wk, wv)):
                cols = _block(jnp.where(i > 1, j + 1, 0), D)
                src = [w_in.at[_block(p, hd), cols].at[_clamped(i - 2, KR, hd)] for p in range(2)]
                dst = w.at[:, _clamped(i - 2, KR // 2, hd // 2), :]
                prepare += [_prepare_kv_weight(src, dst, r0) for r0 in range(0, KR, 16)]
            queues = [_staggered(prepare), normalize(jnp.minimum(i + 1, n - 1), 16)]
            qraw_s[_block(i, hf), :] = _pack(_dot(normalized(i), wq[...], zero_s[...], queues, 2))

        def kv_step(i, _):
            pl.when(i + 1 < NS)(lambda: start(ffn_copy(i + 1)))
            wait(ffn_copy(i))

            def project(i_again, w, dst, queues, first):
                dst = dst.at[:, _block(i, TK, _HALO), :]
                rows, m = _block(i_again, TK // 4), {}
                for t, k in enumerate((2, 4, 1, 3, 0, 5, 6)):
                    a = (xsum_s[_STRASSEN_SUMS.index(k), rows, :] if k in _STRASSEN_SUMS
                         else xn_s[k - 2, rows, _block(k - 2, hd)])
                    m[k] = _dot(a, w[k], zero_s[...], [_share(q, t, 7) for q in queues], 0 if t else first)
                y = _strassen_upper(m) + _strassen_lower(m)
                for t in range(TK // T):
                    for p in range(2):
                        for c in range(8):
                            dst[c, pl.ds(_HALO + t * T + p * hf, hf), :] = (
                                y[2 * p + c // 4][t * hf:(t + 1) * hf, c % 4 * 128:(c % 4 + 1) * 128])

            prepare = []
            for src, dst, scale, shift in ((wg_in, wgu, 2, 0), (wu_in, wgu, 2, 128), (wd_in, wd, 1, 0)):
                size = src.shape[2]
                prepare += [_bind(_prepare_ffn_weight, src.at[i % 2], dst.at[:, _block(i, size // 2), :],
                                  r0, c0, scale * c0 + shift, group)
                            for r0 in range(0, size, 16) for c0 in range(0, src.shape[3] // 4, 128)
                            for group in _HK_GROUPS]
            views = [[q_s.at[_block(p, hf)].at[_clamped(i - 1, AR, hf)]]
                     + [ref.at[:, _block(p, hf, _HALO), :].at[:, _clamped(i - 1, AR, hf, _HALO), :]
                        for ref in (k_s, v_s)] for p in range(2)]
            attend = _attention_halves(views, keep_s, o_s.at[:, _clamped(i - 1, AR // 2, hf // 2), :],
                                       jnp.clip((i - 1) * AR, 0, hf - AR))
            cut = len(prepare) * 8 // 16
            project(i, wv, v_s, [prepare[:cut], [_chain(a, b) for a, b, _ in attend]], 1)
            for c in range(8):
                v_s[c, pl.ds(0, _HALO), :] = jnp.broadcast_to(v_s[c, pl.ds(_HALO, 1), :], (_HALO, 128))
            layout = [_prepare_q(qraw_s.at[_block(i, TK // 2)], q_s.at[_block(i, TK)], r0, 64)
                      for r0 in range(0, TK, 64)]
            project(i + (i >> 8), wk, k_s,
                    [prepare[cut:], _prepare_out_weight(wo_in, wo_tmp, wo, i), _staggered(layout),
                     [_bind(mix, 0, 1, 2, 3) for _, _, mix in attend]], 0)

        def main_step(i, _):
            zero = zero_s[...]
            whole = lambda rows, use=0: _block(i >> (8 + use), rows)
            hs = (ha_s, hb_s)

            def residual(p, blocks):
                for t, y in enumerate(blocks):
                    hs[p][:, _block(t, hd)] = x_s[_block(2 * i + p, hf), _block(t, hd)].astype(_F32) + y

            def norm(p, r0):
                y = _layernorm(hs[p].at[whole(hf)][pl.ds(r0, 16), :])
                if p:
                    upper = na_s.at[whole(hf)][pl.ds(r0, 16), :]
                else:
                    na_s[pl.ds(r0, 16), :] = upper = y
                blocks = [v[:, k * qd:(k + 1) * qd] for v in (upper, y) for k in range(4)]
                left = _sums(_HK_LEFT[_HK_EARLY:] if p else _HK_LEFT[:_HK_EARLY], blocks)
                return _token(_store_packed(hnb_s if p else hna_s, pl.ds(r0 // 2, 8), slice(None), left)[-3:])

            norms = [[_bind(norm, p, r0) for r0 in range(0, hf, 16)] for p in range(2)]
            m = {k: _dot(o_s[k], wo[k], zero) for k in (2, 4, 3, 0, 6)}
            residual(0, _strassen_upper(m))
            m[1] = _dot(o_s[1], wo[1], zero)
            m[5] = _dot(o_s[5], wo[5], zero, [norms[0][:4]])
            _chain(*norms[0][4:])()
            residual(1, _strassen_lower(m))

            j = jnp.minimum(i + 1, n - 1)
            views = [[q_s.at[_block(2 * j + p, hf)]]
                     + [ref.at[:, _block(2 * j + p, hf, _HALO), :] for ref in (k_s, v_s)] for p in range(2)]
            attend = [job for scores, softmax, mix in _attention_halves(views, keep_s, o_s, None)
                      for job in (scores, _chain(softmax, _bind(mix, 0, 1)), _bind(mix, 2, 3))]

            lead, tiles = 4, F // 512
            orders = [_HK_FIRST if u < lead else _HK_ORDER for u in range(tiles)]
            ups = [step[1:] for step in sorted(
                (t if u < lead and t < _HK_EARLY else t + 13 * u, u, k)
                for u, order in enumerate(orders) for t, k in enumerate(order))]
            steps = ups + list(_HK_ORDER)
            jobs = {}
            for queue, span in ((norms[1], steps[2:_HK_EARLY * lead]), (attend, steps[_HK_EARLY * lead:-3])):
                jobs.update({step: [_share(queue, t, len(span))] for t, step in enumerate(span)})
            up = {}
            for u, k in ups:
                a = hna_s.at[k] if k < _HK_EARLY else hnb_s.at[k - _HK_EARLY]
                up[u, k] = _dot(a[whole(hf // 2, u), :], wgu.at[k][:, _block(u, 256)], zero, jobs.get((u, k), ()))

            def activation(u):
                ready = [orders[u].index(k) for k in range(len(_HK))]
                gate_up = _sums(_HK_OUT, [up[u, k] for k in range(len(_HK))], ready)
                ready = [max(t for t, c in zip(ready, row) if c) for row in _HK_OUT]
                return _sums(_HK_LEFT, [_geglu(y[:, :128], y[:, 128:]) for y in gate_up], ready)

            left = [jnp.concatenate(v, axis=1) for v in zip(*[activation(u) for u in range(tiles)])]
            down = {k: _dot(left[k].astype(_BF16), wd.at[k][...], zero, jobs.get(k, ())) for k in _HK_ORDER}
            out = _sums(_HK_OUT, [down[k] for k in range(len(_HK))], [_HK_ORDER.index(k) for k in range(len(_HK))])

            for p, t0, nt in ((1, 0, 3), (0, 0, 2), (0, 2, 2), (1, 3, 1)):
                for t in range(t0, t0 + nt):
                    y = hs[p][whole(hf), _block(t, qd)] + out[4 * p + t]
                    x_s[_block(2 * i + p, hf), _block(t, qd)] = y.astype(_BF16)
                at = lambda ref: ref.at[_block(2 * i + p, hf), pl.ds(t0 * qd, nt * qd)]
                pltpu.make_async_copy(at(x_s), at(out_hbm), osem).start()

        start(x_copy(0) + q_copy(0) + q_copy(1))
        zero_s[...] = jnp.zeros(zero_s.shape, _I32)
        wo_tmp[...] = jnp.zeros(wo_tmp.shape, _F32)
        for p in range(2):
            k_s[:, pl.ds(p * hf, AR + _HALO), :] = jnp.zeros((8, AR + _HALO, 128), _F32)
            q_s[pl.ds(p * hf, AR), :] = jnp.zeros((AR, D), _BF16)
        wait(x_copy(0))
        _chain(*normalize(0, hf))()
        jax.lax.fori_loop(0, NQ, first_q_step, None)
        jax.lax.fori_loop(1, n, q_step, None)
        wait(o_copy())
        jax.lax.fori_loop(0, NS, kv_step, None)
        jax.lax.fori_loop(0, n, main_step, None)
        pltpu.make_async_copy(x_s, out_hbm, osem).wait()

    vmem, dma = pltpu.VMEM, pltpu.SemaphoreType.DMA
    in_hbm = pl.BlockSpec(memory_space=pl.ANY)
    row_blocks = lambda w: w.reshape(4, w.shape[0] // 4, w.shape[1])
    out = pl.pallas_call(
        kernel,
        out_shape=jax.ShapeDtypeStruct((S, D), A_x.dtype),
        in_specs=[in_hbm] * 6,
        out_specs=in_hbm,
        scratch_shapes=[
            vmem((S, D), _BF16), vmem((D, 3 * D), _BF16), vmem((D, D), _BF16),
            vmem((2, 4, qd // NS, F), _BF16), vmem((2, 4, qd // NS, F), _BF16), vmem((2, 4, F // 4 // NS, D), _BF16),
            vmem((len(_HK), qd // 2, F // 2), _I32), vmem((len(_HK), F // 8, qd), _I32),
            vmem((7, hd // 2, hd), _I32), vmem((7, hd // 2, hd), _I32), vmem((7, hd // 2, hd), _I32),
            vmem((2, _HEADS * (_HEAD_DIM + 2), 128), _F32),
            vmem((2, S // 4, D), _I32), vmem((len(_STRASSEN_SUMS), S // 4, hd), _I32),
            vmem((D // 2, D), _I32), vmem((S // 2, D), _I32), vmem((S, D), _BF16),
            vmem((8, S + _HALO + 8, 128), _F32), vmem((8, S + _HALO + 8, 128), _F32),
            vmem((8, hf, 128), _F32), vmem((7, hf // 2, hd), _I32),
            vmem((hf, D), _F32), vmem((hf, D), _F32), vmem((hf, D), _F32),
            vmem((_HK_EARLY, hf // 2, qd), _I32), vmem((len(_HK) - _HK_EARLY, hf // 2, qd), _I32),
            vmem((8, 128), _I32),
            dma((n + NQ,)), dma((NK + 1,)), dma((2,)), dma(()),
        ],
        compiler_params=pltpu.CompilerParams(
            vmem_limit_bytes=126 * 1024 * 1024,
            flags={"XLA_TPU_EVENLY_DISTRIBUTE_CRITICAL_NODES": True},
        ),
    )(A_x.reshape(S, D), A_wqkv, A_wo, row_blocks(B_w_gate), row_blocks(B_w_up), row_blocks(B_w_down))
    return out.reshape(B, S, D)
```

```python
import functools

import jax
import jax.experimental.pallas as pl
import jax.experimental.pallas.tpu as pltpu
import jax.numpy as jnp
import numpy as np

_HEADS, _HEAD_DIM, _WINDOW, _DILATION = 32, 32, 8, 2
_HALO = 16
_EPS = 1e-5
_F32, _BF16, _I32 = jnp.float32, jnp.bfloat16, jnp.int32
_bind = functools.partial


def _words(x):
    return pltpu.bitcast(x, _I32)


def _pack(x):
    return _words(x.astype(_BF16))


def _unpack(x):
    return pltpu.bitcast(x, _BF16)


def _block(i, size, extra=0):
    return pl.ds(i * size if isinstance(i, int) else pl.multiple_of(i * size, size), size + extra)


def _clamped(i, size, total, extra=0):
    start = jnp.clip(i * size, 0, total - size)
    return pl.ds(pl.multiple_of(start, 8 if size % 16 else 16), size + extra)


def _store_packed(dst, rows, cols, ys):
    ys = [_pack(y) for y in ys]
    for k, y in enumerate(ys):
        dst.at[k][rows, cols] = y
    return ys


def _token(parts):
    return functools.reduce(jnp.bitwise_or, [
        p[r:r + 8, c:c + 128] for p in parts
        for r in range(0, p.shape[0], 8) for c in range(0, p.shape[1], 128)])


def _dot(a, w, zero, queues=(), first=0):
    if any(queues):
        nt, nk = w.shape[1] // 128, pl.cdiv(w.shape[0], 256)
        due = {}
        for queue in queues:
            for j, job in enumerate(queue):
                slot = first + ((j + 1) * (nt * nk - first) - 1) // len(queue)
                due.setdefault(divmod(slot, nk), []).append(job())
        parts = []
        for k in range(nk):
            top = [w[k * 256:k * 256 + 8, t * 128:(t + 1) * 128] for t in range(nt)]
            top = [v | (_token(due[t, k]) & zero) if (t, k) in due else v for t, v in enumerate(top)]
            parts += [jnp.concatenate(top, axis=1), w[k * 256 + 8:(k + 1) * 256]]
        w = jnp.concatenate(parts, axis=0)
    return jnp.dot(a if a.dtype == _BF16 else _unpack(a), _unpack(w), preferred_element_type=_F32)


def _share(jobs, j, parts):
    return jobs[j * len(jobs) // parts:(j + 1) * len(jobs) // parts]


def _chain(*jobs):
    return lambda: [job() for job in jobs][-1]


def _staggered(chains):
    depth = len(chains[0])
    return [_bind(lambda jobs: _token([job() for job in jobs]),
                  [c[t - i] for i, c in enumerate(chains) if 0 <= t - i < depth])
            for t in range(len(chains) + depth - 1)]


def _strassen_left(a11, a12, a21, a22):
    return (a11 + a22, a21 + a22, a11, a22, a11 + a12, a21 - a11, a12 - a22)


def _strassen_right(b11, b12, b21, b22):
    return (b11 + b22, b11, b12 - b22, b21 - b11, b22, b11 + b12, b21 + b22)


def _strassen_upper(m):
    return (((m[3] - m[4]) + m[0]) + m[6], m[2] + m[4])


def _strassen_lower(m):
    return (m[1] + m[3], ((m[2] - m[1]) + m[0]) + m[5])


_STRASSEN_SUMS = (0, 1, 4, 5, 6)

_HK = [[[{"+": 1, ".": 0, "-": -1}[ch] for ch in part] for part in line.split()] for line in (
    "+....... +-......+....... +...-...",
    ".+...... ...++-.-.-...... .-......",
    "...+.... ...+.......-+-.- ...-...+",
    "+.-..... ........+....... -.+.....",
    ".+-..... .........+...... .-+..+-.",
    "..+-.... ...........+.... ..++....",
    "++.+.... ...+............ ++.+....",
    ".....+.. .+...--.....+-.. .....-..",
    "......+. ..+......++...+. ..-...+.",
    "+...+... +.+.-........... ....+...",
    "..+...+. ......+.+.+-.... ..+.....",
    "...+...+ ...+...-....+.+- .......-",
    "....++.. .+..........-... --..++..",
    "....+.-. ..+............. ....-.+.",
    "+.....+. ..+.....-....... ..+.-...",
    ".....+.- ............+-.. .-.+.+.-",
    "......+- ..............+. ......--",
    "...+..+. ...........+..+. ..+....+",
    "+...++.. .+..-........... ++..-...",
    ".+-...-. ......+..-...... ..+..+-.",
    "...+.-.+ ...+...-....-+.. .+.-...+",
    "....++.+ ............+... ....++.+",
    "...+--.. ...+........-... --.....-",
    "++..++.. ...+-........... --......",
    ".+-..+-. ......+......... .....-+.",
    ".+.-.+.- ...+...-........ .+.-....",
)]
_HK_LEFT, _HK_RIGHT = ([line[k] for line in _HK] for k in range(2))
_HK_OUT = [[line[2][o] for line in _HK] for o in range(8)]
_HK_EARLY = 7
_HK_FIRST = (4, 1, 6, 5, 0, 3, 2, 12, 22, 21, 19, 20, 15, 18, 25, 24, 23, 13, 7, 14, 9, 8, 16, 17, 10, 11)
_HK_ORDER = (15, 24, 22, 18, 19, 21, 6, 23, 4, 13, 12, 16, 8, 3, 0, 14, 9, 25, 7, 20, 1, 5, 2, 17, 10, 11)
_HK_GROUPS = ((2, 11, 15, 20, 21, 22, 25, 6), (8, 10, 13, 14, 16, 17, 19, 24, 3, 4, 5), (1, 7, 0, 9, 12, 18, 23))


def _sums(rows, xs, ready=None):
    xs, ready = list(xs), list(ready or range(len(xs)))
    rows = [{j: c for j, c in enumerate(row) if c} for row in rows]
    while True:
        count = {}
        for row in rows:
            for pair in [(a, b, row[a] * row[b]) for a in row for b in row if a < b]:
                count[pair] = count.get(pair, 0) + 1
        best = max(sorted(count), key=count.get, default=None)
        if best is None or count[best] < 2:
            break
        a, b, sign = best
        xs.append(xs[a] + xs[b] if sign > 0 else xs[a] - xs[b])
        ready.append(max(ready[a], ready[b]))
        for row in rows:
            if row.get(a, 0) * row.get(b, 0) == sign:
                row[len(xs) - 1] = row.pop(a)
                del row[b]
    out = []
    for row in rows:
        (j, sign), *rest = sorted(row.items(), key=lambda t: (ready[t[0]], t[0]))
        acc = xs[j]
        for j, c in rest:
            acc = acc + xs[j] if c == sign else acc - xs[j] if sign > 0 else xs[j] - acc
            sign = max(sign, c)
        out.append(acc if sign > 0 else -acc)
    return out


def _layernorm(x, moments=None):
    mean = moments[0] if moments else jnp.mean(x, axis=-1, keepdims=True)
    xc = x - mean
    scale = moments[1] if moments else jax.lax.rsqrt(jnp.mean(xc * xc, axis=-1, keepdims=True) + _EPS)
    return xc * scale, (mean, scale)


def _geglu(g, u):
    c = float(np.sqrt(2.0 / np.pi))
    th = jnp.tanh(g * (c + (c * 0.044715) * (g * g)))
    half = (0.5 * g) * u
    return half * th + half


def _normalize_input(src, plain, sums, r0, rows):
    hd = src[0].shape[1] // 2
    a, b = (_layernorm(ref[pl.ds(r0, rows), :].astype(_F32))[0] for ref in src)
    at = pl.ds(r0 // 2, rows // 2)
    _store_packed(plain, at, slice(None), (a, b))
    left = _strassen_left(a[:, :hd], a[:, hd:], b[:, :hd], b[:, hd:])
    return _token(_store_packed(sums, at, slice(None), [left[k] for k in _STRASSEN_SUMS])[1:3])


def _heads_minor(load, store):
    vs = []
    lanes = lambda: jax.lax.broadcasted_iota(_I32, vs[0].shape, 1)

    def skew():
        vs.extend(pltpu.roll(load(g), 4 * g, 1) if g else load(g) for g in range(8))
        return _token(vs[1:])

    def exchange():
        us = [vs[-j % 8] for j in range(8)]
        for b in (1, 2, 4):
            moved = (lanes() & (4 * b)) != 0
            us = [jnp.where(moved, us[(j - b) % 8], us[j]) for j in range(8)]
        vs[:] = [pltpu.roll(u, 128 - 4 * j, 1) if j else u for j, u in enumerate(us)]
        return _token(vs[1:])

    def shuffle():
        lane = lanes()
        idx = (lane & 3) * 32 + (lane & 28) + (lane >> 5)
        return store([jnp.take_along_axis(v, idx, axis=1, mode="promise_in_bounds") for v in vs])

    return [skew, exchange, shuffle]


def _prepare_q(src, dst, r0, rows):
    def store(vs):
        for j, v in enumerate(vs):
            dst[pl.ds(r0, rows), _block(j, 128)] = _unpack(v)
        return _token(vs[1:])

    return _heads_minor(lambda g: src[pl.ds(r0 // 2, rows // 2), _block(g, 128)], store)


def _prepare_kv_weight(src, dst, r0):
    def load(g):
        return jnp.concatenate([_words(ref[pl.ds(r0, 16), _block(g, 128)]) for ref in src], axis=0)

    def store(vs):
        vs = [_unpack(v).astype(_F32) for v in vs]
        return _token([_store_packed(
            dst, pl.ds(r0 // 2, 8), _block(j, 128),
            _strassen_right(vs[j][:16], vs[j + 4][:16], vs[j][16:], vs[j + 4][16:]))[0] for j in range(4)])

    return _heads_minor(load, store)


def _prepare_out_weight(src, tmp, dst, c):
    pitch = _HEAD_DIM + 1

    def spread(h0):
        ys = []
        for h in range(h0, h0 + 4):
            for k in range(2):
                ys.append(src[_block(h, _HEAD_DIM), _block(c + 4 * k, 128)].astype(_F32))
                tmp[k, pl.ds(h * pitch, _HEAD_DIM), :] = ys[-1]
        return _token([_words(y[:8]) for y in ys])

    def gather(d0):
        ys = []
        for d in range(d0, d0 + 2):
            b = [tmp[k, pl.ds(d + j * _HEAD_DIM // 2, _HEADS, stride=pitch), :] for j in range(2) for k in range(2)]
            ys.append(_store_packed(dst, _block(d, _HEADS // 2), _block(c, 128), _strassen_right(*b))[0])
        return _token(ys)

    return ([_bind(spread, h) for h in range(0, _HEADS, 4)]
            + [_bind(gather, d) for d in range(0, _HEAD_DIM // 2, 2)])


def _prepare_ffn_weight(src, dst, r0, c0, d0, group):
    quarter = src.shape[2] // 4
    b = [src.at[j // 4][pl.ds(r0, 16), pl.ds(j % 4 * quarter + c0, 128)].astype(_F32)
         if any(_HK_RIGHT[k][j] for k in group) else None for j in range(16)]
    ys = [_pack(y) for y in _sums([_HK_RIGHT[k] for k in group], b)]
    for k, y in zip(group, ys):
        dst.at[k][pl.ds(r0 // 2, 8), pl.ds(d0, 128)] = y
    return ys[0]


def _attention(q_s, k_s, v_s, r0, pos0, store):
    ls = []
    window = lambda w: pl.ds(_HALO + r0 - _DILATION * w, 16)

    def scores():
        q = [q_s[pl.ds(r0, 16), _block(c, 128)].astype(_F32) for c in range(8)]
        for w in range(_WINDOW):
            acc = q[0] * k_s[0, window(w), :]
            for c in range(1, 8):
                acc = acc + q[c] * k_s[c, window(w), :]
            ls.append(acc + pltpu.roll(acc, 64, 1))
        return _token([_words(l) for l in ls[-2:]])

    def softmax():
        for w in range(_WINDOW):
            l = (ls[w] + pltpu.roll(ls[w], 32, 1)) * (_HEAD_DIM ** -0.5)
            if pos0 is not None and r0 < _DILATION * w:
                pos = pos0 + r0 + jax.lax.broadcasted_iota(_I32, l.shape, 0)
                l = jnp.where(pos >= _DILATION * w, l, -1e9)
            ls[w] = l
        top = functools.reduce(jnp.maximum, ls)
        es = [jnp.exp(l - top) for l in ls]
        inv = 1.0 / functools.reduce(jnp.add, es)
        ls[:] = [e * inv for e in es]
        return _token([_words(inv)])

    def mix(*groups):
        def weighted(c):
            acc = ls[0] * v_s[c, window(0), :]
            for w in range(1, _WINDOW):
                acc = acc + ls[w] * v_s[c, window(w), :]
            return acc

        return _token([y for c in groups for y in store(r0, c, weighted(c), weighted(c + 4))])

    return scores, softmax, mix


def _attention_halves(views, keep, dst, pos0):
    def store_upper(r0, c, a11, a12):
        keep[c, pl.ds(r0, 16), :] = a11
        keep[c + 4, pl.ds(r0, 16), :] = a12
        return [_words(a11), _words(a12)]

    def store_lower(r0, c, a21, a22):
        left = _strassen_left(keep[c, pl.ds(r0, 16), :], keep[c + 4, pl.ds(r0, 16), :], a21, a22)
        return _store_packed(dst, pl.ds(r0 // 2, 8), _block(c, 128), left)[1:2]

    return [_attention(*views[p], r0, None if p else pos0, store)
            for r0 in range(0, views[0][0].shape[0], 16) for p, store in enumerate((store_upper, store_lower))]


@jax.jit
def pallas_sequential_preLN__sliding_local_dilated__glu_gated_geglu__prompt_kernel(
    A_x: jax.Array,
    A_wqkv: jax.Array,
    A_wo: jax.Array,
    B_x: jax.Array,
    B_w_gate: jax.Array,
    B_w_up: jax.Array,
    B_w_down: jax.Array,
):
    del B_x
    B, S, D = A_x.shape
    F = B_w_gate.shape[1]
    assert (B, S, D) == (1, 2048, _HEADS * _HEAD_DIM) and F % 512 == 0
    T = 256
    n, hf, hd, qd = S // T, T // 2, D // 2, D // 4
    NQ = NK = NS = 4
    QC, TK = D // NQ, S // NS
    KR, AR = 96, 48

    def kernel(x_hbm, wqkv_hbm, wo_hbm, wg_hbm, wu_hbm, wd_hbm, out_hbm,
               x_s, w_in, wo_in, wg_in, wu_in, wd_in, wgu, wd, wk, wv, wo, wo_tmp,
               xn_s, xsum_s, wq, qraw_s, q_s, k_s, v_s, keep_s, o_s, ha_s, hb_s, hna_s, hnb_s, zero_s,
               xsem, wsem, fsem, osem):
        def x_copy(i):
            return [pltpu.make_async_copy(x_hbm.at[_block(i, T)], x_s.at[_block(i, T)], xsem.at[i])]

        def q_copy(j):
            at = lambda ref, p: ref.at[_block((2 + p) * NQ + j, hf // NQ)]
            return [pltpu.make_async_copy(a, b, xsem.at[n + j]) for a, b in (
                (at(x_hbm, 0), at(x_s, 0)), (at(x_hbm, 1), at(x_s, 1)),
                (wqkv_hbm.at[:, _block(j, QC)], w_in.at[:, _block(j, QC)]))]

        def kv_copy(j):
            at = lambda ref, p: ref.at[_block(p * NK + j, hd // NK), pl.ds(D, 2 * D)]
            return [pltpu.make_async_copy(at(wqkv_hbm, p), at(w_in, p), wsem.at[j]) for p in range(2)]

        def o_copy():
            return [pltpu.make_async_copy(wo_hbm, wo_in, wsem.at[NK])]

        def ffn_copy(i):
            return [pltpu.make_async_copy(w.at[:, _block(i, w.shape[1] // NS), :],
                                          dst.at[i % 2, :, pl.ds(0, w.shape[1] // NS), :], fsem.at[i % 2])
                    for w, dst in ((wg_hbm, wg_in), (wu_hbm, wu_in), (wd_hbm, wd_in))]

        def start(copies):
            for c in copies:
                c.start()

        def wait(copies):
            for c in copies:
                c.wait()

        def normalize(i, rows):
            at = lambda ref: ref.at[:, _block(i, hf // 2), :]
            src = [x_s.at[_block(2 * i + p, hf)] for p in range(2)]
            return [_bind(_normalize_input, src, at(xn_s), at(xsum_s), r0, rows) for r0 in range(0, hf, rows)]

        def normalized(i):
            return jnp.concatenate([xn_s[p, _block(i, hf // 2), :] for p in range(2)], axis=0)

        def first_q_step(j, _):
            pl.when(j + 2 < NQ)(lambda: start(q_copy(j + 2)))
            pl.when(j + 2 == NQ)(lambda: start(x_copy(2) + kv_copy(0)))
            wait(q_copy(j))
            rows = hf // NQ
            at = lambda ref: ref.at[:, _block(NQ + j, rows // 2), :]
            src = [x_s.at[_block((2 + p) * NQ + j, rows)] for p in range(2)]
            jobs = [_bind(_normalize_input, src, at(xn_s), at(xsum_s), r0, 16) for r0 in range(0, rows, 16)]
            wq[:, _block(j, QC)] = w = _words(w_in[:, _block(j, QC)])
            qraw_s[pl.ds(0, hf), _block(j, QC)] = _pack(_dot(normalized(0), w, zero_s[...], [jobs], 2))

        def q_step(i, _):
            pl.when(i < NK)(lambda: start(x_copy(i + 2) + kv_copy(i)))
            pl.when(i == NK - 1)(lambda: start(sum([x_copy(j) for j in range(NK + 2, n)], [])))
            pl.when(i == NK)(lambda: start(o_copy() + ffn_copy(0)))
            pl.when(i + 1 < n)(lambda: wait(x_copy(i + 1)))
            pl.when((i > 1) & (i < NK + 2))(lambda: wait(kv_copy(i - 2)))
            prepare = []
            for j, w in enumerate((wk, wv)):
                cols = _block(jnp.where(i > 1, j + 1, 0), D)
                src = [w_in.at[_block(p, hd), cols].at[_clamped(i - 2, KR, hd)] for p in range(2)]
                dst = w.at[:, _clamped(i - 2, KR // 2, hd // 2), :]
                prepare += [_prepare_kv_weight(src, dst, r0) for r0 in range(0, KR, 16)]
            queues = [_staggered(prepare), normalize(jnp.minimum(i + 1, n - 1), 16)]
            qraw_s[_block(i, hf), :] = _pack(_dot(normalized(i), wq[...], zero_s[...], queues, 2))

        def kv_step(i, _):
            pl.when(i + 1 < NS)(lambda: start(ffn_copy(i + 1)))
            wait(ffn_copy(i))

            def project(i_again, w, dst, t0):
                dst = dst.at[:, _block(i, TK, _HALO), :]
                rows, m = _block(i_again, TK // 4), {}
                for t, k in enumerate((2, 4, 1, 3, 0, 5, 6), t0):
                    a = (xsum_s[_STRASSEN_SUMS.index(k), rows, :] if k in _STRASSEN_SUMS
                         else xn_s[k - 2, rows, _block(k - 2, hd)])
                    m[k] = _dot(a, w[k], zero_s[...], [_share(q, t - a0, a1 - a0) for q, a0, a1 in queues if a0 <= t < a1],
                                0 if t else 1)
                    y = m[k][:16, 0 * 128:][:, :128]
                    if t in [3, 5, 7, 9]:
                        qraw_s[_block(S // 16 + (i >> 8), 8), _block(0, 128)] = _words(y[:8])
                    if t in [6]:
                        for ref in (wg_in, wu_in, wd_in):
                            ref.at[i >> 8, 0][pl.ds(ref.shape[2] - 16, 16), _block(0, 128)] = y.astype(_BF16)
                y = _strassen_upper(m) + _strassen_lower(m)
                for t in range(TK // T):
                    for p in range(2):
                        for c in range(8):
                            dst[c, pl.ds(_HALO + t * T + p * hf, hf), :] = (
                                y[2 * p + c // 4][t * hf:(t + 1) * hf, c % 4 * 128:(c % 4 + 1) * 128])

            prepare = []
            for src, dst, scale, shift in ((wg_in, wgu, 2, 0), (wu_in, wgu, 2, 128), (wd_in, wd, 1, 0)):
                size = src.shape[2] - 16
                prepare += [_bind(_prepare_ffn_weight, src.at[i % 2], dst.at[:, _block(i, size // 2), :],
                                  r0, c0, scale * c0 + shift, group)
                            for r0 in range(0, size, 16) for c0 in range(0, src.shape[3] // 4, 128)
                            for group in _HK_GROUPS]
            views = [[q_s.at[_block(p, hf)].at[_clamped(i - 1, AR, hf)]]
                     + [ref.at[:, _block(p, hf, _HALO), :].at[:, _clamped(i - 1, AR, hf, _HALO), :]
                        for ref in (k_s, v_s)] for p in range(2)]
            attend = _attention_halves(views, keep_s, o_s.at[:, _clamped(i - 1, AR // 2, hf // 2), :],
                                       jnp.clip((i - 1) * AR, 0, hf - AR))
            layout = [_prepare_q(qraw_s.at[_block(i, TK // 2)], q_s.at[_block(i, TK)], r0, 16)
                      for r0 in range(0, TK, 16)]
            queues = [(prepare, 0, 14), ([_chain(a, b) for a, b, _ in attend], 0, 6),
                      (_staggered(layout), 6 - 1, 14), (_prepare_out_weight(wo_in, wo_tmp, wo, i), 0, 7),
                      ([_bind(mix, 0, 1, 2, 3) for _, _, mix in attend], 8, 14)]
            project(i, wv, v_s, 0)
            for c in range(8):
                v_s[c, pl.ds(0, _HALO), :] = jnp.broadcast_to(v_s[c, pl.ds(_HALO, 1), :], (_HALO, 128))
            project(i + (i >> 8), wk, k_s, 7)

        def main_step(i, _):
            zero = zero_s[...]
            whole = lambda rows, use=0: _block(i >> (8 + use), rows)
            hs, moments = (ha_s, hb_s), {}

            def residual(p, blocks):
                for t, y in enumerate(blocks):
                    hs[p][:, _block(t, hd)] = x_s[_block(2 * i + p, hf), _block(t, hd)].astype(_F32) + y

            def norm(p, r0):
                y, moments[p, r0] = _layernorm(hs[p].at[whole(hf)][pl.ds(r0, 16), :])
                upper = _layernorm(hs[0].at[whole(hf, 1)][pl.ds(r0, 16), :], moments[0, r0])[0] if p else y
                blocks = [v[:, k * qd:(k + 1) * qd] for v in (upper, y) for k in range(4)]
                left = _sums(_HK_LEFT[_HK_EARLY:] if p else _HK_LEFT[:_HK_EARLY], blocks)
                return _token(_store_packed(hnb_s if p else hna_s, pl.ds(r0 // 2, 8), slice(None), left)[-3:])

            norms = [[_bind(norm, p, r0) for r0 in range(0, hf, 16)] for p in range(2)]
            m = {k: _dot(o_s[k], wo[k], zero) for k in (2, 4, 3, 0, 6)}
            residual(0, _strassen_upper(m))
            m[1] = _dot(o_s[1], wo[1], zero)
            m[5] = _dot(o_s[5], wo[5], zero, [norms[0][:4]])
            _chain(*norms[0][4:])()
            residual(1, _strassen_lower(m))

            j = jnp.minimum(i + 1, n - 1)
            views = [[q_s.at[_block(2 * j + p, hf)]]
                     + [ref.at[:, _block(2 * j + p, hf, _HALO), :] for ref in (k_s, v_s)] for p in range(2)]
            attend = [job for scores, softmax, mix in _attention_halves(views, keep_s, o_s, None)
                      for job in (scores, _chain(softmax, _bind(mix, 0, 1)), _bind(mix, 2, 3))]

            lead, tiles = 4, F // 512
            orders = [_HK_FIRST if u < lead else _HK_ORDER for u in range(tiles)]
            ups = [step[1:] for step in sorted(
                (t if u < lead and t < _HK_EARLY else t + 11 * u, u, k)
                for u, order in enumerate(orders) for t, k in enumerate(order))]
            steps = ups + list(_HK_ORDER)
            jobs = {}
            for queue, span in ((norms[1], steps[6:_HK_EARLY * lead]), (attend, steps[_HK_EARLY * lead:-3])):
                jobs.update({step: [_share(queue, t, len(span))] for t, step in enumerate(span)})
            up = {}
            for u, k in ups:
                a = hna_s.at[k] if k < _HK_EARLY else hnb_s.at[k - _HK_EARLY]
                up[u, k] = _dot(a[whole(hf // 2, u), :], wgu.at[k][:, _block(u, 256)], zero, jobs.get((u, k), ()))

            def activation(u):
                ready = [orders[u].index(k) for k in range(len(_HK))]
                gate_up = _sums(_HK_OUT, [up[u, k] for k in range(len(_HK))], ready)
                ready = [max(t for t, c in zip(ready, row) if c) for row in _HK_OUT]
                return _sums(_HK_LEFT, [_geglu(y[:, :128], y[:, 128:]) for y in gate_up], ready)

            left = [jnp.concatenate(v, axis=1) for v in zip(*[activation(u) for u in range(tiles)])]
            down = {k: _dot(left[k].astype(_BF16), wd.at[k][...], zero, jobs.get(k, ())) for k in _HK_ORDER}
            out = _sums(_HK_OUT, [down[k] for k in range(len(_HK))], [_HK_ORDER.index(k) for k in range(len(_HK))])

            for p, t0, nt in ((1, 0, 3), (0, 0, 2), (0, 2, 2), (1, 3, 1)):
                for t in range(t0, t0 + nt):
                    y = hs[p][whole(hf), _block(t, qd)] + out[4 * p + t]
                    x_s[_block(2 * i + p, hf), _block(t, qd)] = y.astype(_BF16)
                at = lambda ref: ref.at[_block(2 * i + p, hf), pl.ds(t0 * qd, nt * qd)]
                pltpu.make_async_copy(at(x_s), at(out_hbm), osem).start()

        start(x_copy(0) + q_copy(0) + q_copy(1))
        zero_s[...] = jnp.zeros(zero_s.shape, _I32)
        wo_tmp[...] = jnp.zeros(wo_tmp.shape, _F32)
        for p in range(2):
            k_s[:, pl.ds(p * hf, AR + _HALO), :] = jnp.zeros((8, AR + _HALO, 128), _F32)
            q_s[pl.ds(p * hf, AR), :] = jnp.zeros((AR, D), _BF16)
        wait(x_copy(0))
        _chain(*normalize(0, hf))()
        jax.lax.fori_loop(0, NQ, first_q_step, None)
        jax.lax.fori_loop(1, n, q_step, None)
        wait(o_copy())
        jax.lax.fori_loop(0, NS, kv_step, None)
        jax.lax.fori_loop(0, n, main_step, None)
        pltpu.make_async_copy(x_s, out_hbm, osem).wait()

    vmem, dma = pltpu.VMEM, pltpu.SemaphoreType.DMA
    in_hbm = pl.BlockSpec(memory_space=pl.ANY)
    row_blocks = lambda w: w.reshape(4, w.shape[0] // 4, w.shape[1])
    out = pl.pallas_call(
        kernel,
        out_shape=jax.ShapeDtypeStruct((S, D), A_x.dtype),
        in_specs=[in_hbm] * 6,
        out_specs=in_hbm,
        scratch_shapes=[
            vmem((S, D), _BF16), vmem((D, 3 * D), _BF16), vmem((D, D), _BF16),
            vmem((2, 4, qd // NS + 16, F), _BF16), vmem((2, 4, qd // NS + 16, F), _BF16),
            vmem((2, 4, F // 4 // NS + 16, D), _BF16),
            vmem((len(_HK), qd // 2, F // 2), _I32), vmem((len(_HK), F // 8, qd), _I32),
            vmem((7, hd // 2, hd), _I32), vmem((7, hd // 2, hd), _I32), vmem((7, hd // 2, hd), _I32),
            vmem((2, _HEADS * (_HEAD_DIM + 2), 128), _F32),
            vmem((2, S // 4, D), _I32), vmem((len(_STRASSEN_SUMS), S // 4, hd), _I32),
            vmem((D // 2, D), _I32), vmem((S // 2 + 8, D), _I32), vmem((S, D), _BF16),
            vmem((8, S + _HALO + 8, 128), _F32), vmem((8, S + _HALO + 8, 128), _F32),
            vmem((8, hf, 128), _F32), vmem((7, hf // 2, hd), _I32),
            vmem((hf, D), _F32), vmem((hf, D), _F32),
            vmem((_HK_EARLY, hf // 2, qd), _I32), vmem((len(_HK) - _HK_EARLY, hf // 2, qd), _I32),
            vmem((8, 128), _I32),
            dma((n + NQ,)), dma((NK + 1,)), dma((2,)), dma(()),
        ],
        compiler_params=pltpu.CompilerParams(
            vmem_limit_bytes=126 * 1024 * 1024,
            flags={"XLA_TPU_EVENLY_DISTRIBUTE_CRITICAL_NODES": True},
        ),
    )(A_x.reshape(S, D), A_wqkv, A_wo, row_blocks(B_w_gate), row_blocks(B_w_up), row_blocks(B_w_down))
    return out.reshape(B, S, D)
```

```python
import functools

import jax
import jax.experimental.pallas as pl
import jax.experimental.pallas.tpu as pltpu
import jax.numpy as jnp
import numpy as np

_HEADS, _HEAD_DIM, _WINDOW, _DILATION = 32, 32, 8, 2
_HALO = 16
_EPS = 1e-5
_F32, _BF16, _I32 = jnp.float32, jnp.bfloat16, jnp.int32
_bind = functools.partial


def _words(x):
    return pltpu.bitcast(x, _I32)


def _pack(x):
    return _words(x.astype(_BF16))


def _unpack(x):
    return pltpu.bitcast(x, _BF16)


def _block(i, size, extra=0):
    return pl.ds(i * size if isinstance(i, int) else pl.multiple_of(i * size, size), size + extra)


def _clamped(i, size, total, extra=0):
    start = jnp.clip(i * size, 0, total - size)
    return pl.ds(pl.multiple_of(start, 8 if size % 16 else 16), size + extra)


def _store_packed(dst, rows, cols, ys):
    ys = [_pack(y) for y in ys]
    for k, y in enumerate(ys):
        dst.at[k][rows, cols] = y
    return ys


def _token(parts):
    return functools.reduce(jnp.bitwise_or, [
        p[r:r + 8, c:c + 128] for p in parts
        for r in range(0, p.shape[0], 8) for c in range(0, p.shape[1], 128)])


def _dot(a, w, zero, queues=(), first=0):
    if any(queues):
        nt, nk = w.shape[1] // 128, pl.cdiv(w.shape[0], 256)
        due = {}
        for queue in queues:
            for j, job in enumerate(queue):
                slot = first + ((j + 1) * (nt * nk - first) - 1) // len(queue)
                due.setdefault(divmod(slot, nk), []).append(job())
        parts = []
        for k in range(nk):
            top = [w[k * 256:k * 256 + 8, t * 128:(t + 1) * 128] for t in range(nt)]
            top = [v | (_token(due[t, k]) & zero) if (t, k) in due else v for t, v in enumerate(top)]
            parts += [jnp.concatenate(top, axis=1), w[k * 256 + 8:(k + 1) * 256]]
        w = jnp.concatenate(parts, axis=0)
    return jnp.dot(a if a.dtype == _BF16 else _unpack(a), _unpack(w), preferred_element_type=_F32)


def _share(jobs, j, parts):
    return jobs[j * len(jobs) // parts:(j + 1) * len(jobs) // parts]


def _chain(*jobs):
    return lambda: [job() for job in jobs][-1]


def _staggered(chains):
    depth = len(chains[0])
    return [_bind(lambda jobs: _token([job() for job in jobs]),
                  [c[t - i] for i, c in enumerate(chains) if 0 <= t - i < depth])
            for t in range(len(chains) + depth - 1)]


def _strassen_left(a11, a12, a21, a22):
    return (a11 + a22, a21 + a22, a11, a22, a11 + a12, a21 - a11, a12 - a22)


def _strassen_right(b11, b12, b21, b22):
    return (b11 + b22, b11, b12 - b22, b21 - b11, b22, b11 + b12, b21 + b22)


def _strassen_upper(m):
    return (((m[3] - m[4]) + m[0]) + m[6], m[2] + m[4])


def _strassen_lower(m):
    return (m[1] + m[3], ((m[2] - m[1]) + m[0]) + m[5])


_STRASSEN_SUMS = (0, 1, 4, 5, 6)

_HK = [[[{"+": 1, ".": 0, "-": -1}[ch] for ch in part] for part in line.split()] for line in (
    "+....... +-......+....... +...-...",
    ".+...... ...++-.-.-...... .-......",
    "...+.... ...+.......-+-.- ...-...+",
    "+.-..... ........+....... -.+.....",
    ".+-..... .........+...... .-+..+-.",
    "..+-.... ...........+.... ..++....",
    "++.+.... ...+............ ++.+....",
    ".....+.. .+...--.....+-.. .....-..",
    "......+. ..+......++...+. ..-...+.",
    "+...+... +.+.-........... ....+...",
    "..+...+. ......+.+.+-.... ..+.....",
    "...+...+ ...+...-....+.+- .......-",
    "....++.. .+..........-... --..++..",
    "....+.-. ..+............. ....-.+.",
    "+.....+. ..+.....-....... ..+.-...",
    ".....+.- ............+-.. .-.+.+.-",
    "......+- ..............+. ......--",
    "...+..+. ...........+..+. ..+....+",
    "+...++.. .+..-........... ++..-...",
    ".+-...-. ......+..-...... ..+..+-.",
    "...+.-.+ ...+...-....-+.. .+.-...+",
    "....++.+ ............+... ....++.+",
    "...+--.. ...+........-... --.....-",
    "++..++.. ...+-........... --......",
    ".+-..+-. ......+......... .....-+.",
    ".+.-.+.- ...+...-........ .+.-....",
)]
_HK_LEFT, _HK_RIGHT = ([line[k] for line in _HK] for k in range(2))
_HK_OUT = [[line[2][o] for line in _HK] for o in range(8)]
_HK_EARLY = 7
_HK_FIRST = (4, 1, 6, 5, 0, 3, 2, 12, 22, 21, 19, 20, 15, 18, 25, 24, 23, 13, 7, 14, 9, 8, 16, 17, 10, 11)
_HK_ORDER = (15, 24, 22, 18, 19, 21, 6, 23, 4, 13, 12, 16, 8, 3, 0, 14, 9, 25, 7, 20, 1, 5, 2, 17, 10, 11)
_HK_GROUPS = ((2, 11, 15, 20, 21, 22, 25, 6), (8, 10, 13, 14, 16, 17, 19, 24, 3, 4, 5), (1, 7, 0, 9, 12, 18, 23))


def _sums(rows, xs, ready=None):
    xs, ready = list(xs), list(ready or range(len(xs)))
    rows = [{j: c for j, c in enumerate(row) if c} for row in rows]
    while True:
        count = {}
        for row in rows:
            for pair in [(a, b, row[a] * row[b]) for a in row for b in row if a < b]:
                count[pair] = count.get(pair, 0) + 1
        best = max(sorted(count), key=count.get, default=None)
        if best is None or count[best] < 2:
            break
        a, b, sign = best
        xs.append(xs[a] + xs[b] if sign > 0 else xs[a] - xs[b])
        ready.append(max(ready[a], ready[b]))
        for row in rows:
            if row.get(a, 0) * row.get(b, 0) == sign:
                row[len(xs) - 1] = row.pop(a)
                del row[b]
    out = []
    for row in rows:
        (j, sign), *rest = sorted(row.items(), key=lambda t: (ready[t[0]], t[0]))
        acc = xs[j]
        for j, c in rest:
            acc = acc + xs[j] if c == sign else acc - xs[j] if sign > 0 else xs[j] - acc
            sign = max(sign, c)
        out.append(acc if sign > 0 else -acc)
    return out


def _layernorm(x, moments=None):
    mean = moments[0] if moments else jnp.mean(x, axis=-1, keepdims=True)
    xc = x - mean
    scale = moments[1] if moments else jax.lax.rsqrt(jnp.mean(xc * xc, axis=-1, keepdims=True) + _EPS)
    return xc * scale, (mean, scale)


def _geglu(g, u):
    c = float(np.sqrt(2.0 / np.pi))
    th = jnp.tanh(g * (c + (c * 0.044715) * (g * g)))
    half = (0.5 * g) * u
    return half * th + half


def _normalize_input(src, plain, sums, r0, rows):
    hd = src[0].shape[1] // 2
    a, b = (_layernorm(ref[pl.ds(r0, rows), :].astype(_F32))[0] for ref in src)
    at = pl.ds(r0 // 2, rows // 2)
    _store_packed(plain, at, slice(None), (a, b))
    left = _strassen_left(a[:, :hd], a[:, hd:], b[:, :hd], b[:, hd:])
    return _token(_store_packed(sums, at, slice(None), [left[k] for k in _STRASSEN_SUMS])[1:3])


def _heads_minor(load, store):
    vs = []
    lanes = lambda: jax.lax.broadcasted_iota(_I32, vs[0].shape, 1)

    def skew():
        vs.extend(pltpu.roll(load(g), 4 * g, 1) if g else load(g) for g in range(8))
        return _token(vs[4:])

    def exchange():
        us = [vs[-j % 8] for j in range(8)]
        for b in (1, 2, 4):
            moved = (lanes() & (4 * b)) != 0
            us = [jnp.where(moved, us[(j - b) % 8], us[j]) for j in range(8)]
        vs[:] = [pltpu.roll(u, 128 - 4 * j, 1) if j else u for j, u in enumerate(us)]
        return _token(vs[4:])

    def shuffle():
        lane = lanes()
        idx = (lane & 3) * 32 + (lane & 28) + (lane >> 5)
        return store([jnp.take_along_axis(v, idx, axis=1, mode="promise_in_bounds") for v in vs])

    return [skew, exchange, shuffle]


def _prepare_q(src, dst, r0, rows):
    def store(vs):
        for j, v in enumerate(vs):
            dst[pl.ds(r0, rows), _block(j, 128)] = _unpack(v)
        return _token(vs[4:])

    return _heads_minor(lambda g: src[pl.ds(r0 // 2, rows // 2), _block(g, 128)], store)


def _prepare_kv_weight(src, dst, r0):
    def load(g):
        return jnp.concatenate([_words(ref[pl.ds(r0, 16), _block(g, 128)]) for ref in src], axis=0)

    def store(vs):
        vs = [_unpack(v).astype(_F32) for v in vs]
        return _token([_store_packed(
            dst, pl.ds(r0 // 2, 8), _block(j, 128),
            _strassen_right(vs[j][:16], vs[j + 4][:16], vs[j][16:], vs[j + 4][16:]))[0] for j in range(4)])

    return _heads_minor(load, store)


def _prepare_out_weight(src, tmp, dst, c):
    pitch = _HEAD_DIM + 1

    def spread(h0):
        ys = []
        for h in range(h0, h0 + 4):
            for k in range(2):
                ys.append(src[_block(h, _HEAD_DIM), _block(c + 4 * k, 128)].astype(_F32))
                tmp[k, pl.ds(h * pitch, _HEAD_DIM), :] = ys[-1]
        return _token([_words(y[:8]) for y in ys])

    def gather(d0):
        ys = []
        for d in range(d0, d0 + 2):
            b = [tmp[k, pl.ds(d + j * _HEAD_DIM // 2, _HEADS, stride=pitch), :] for j in range(2) for k in range(2)]
            ys.append(_store_packed(dst, _block(d, _HEADS // 2), _block(c, 128), _strassen_right(*b))[0])
        return _token(ys)

    return ([_bind(spread, h) for h in range(0, _HEADS, 4)]
            + [_bind(gather, d) for d in range(0, _HEAD_DIM // 2, 2)])


def _prepare_ffn_weight(src, dst, r0, c0, d0, group):
    quarter = src.shape[2] // 4
    b = [src.at[j // 4][pl.ds(r0, 16), pl.ds(j % 4 * quarter + c0, 128)].astype(_F32)
         if any(_HK_RIGHT[k][j] for k in group) else None for j in range(16)]
    ys = [_pack(y) for y in _sums([_HK_RIGHT[k] for k in group], b)]
    for k, y in zip(group, ys):
        dst.at[k][pl.ds(r0 // 2, 8), pl.ds(d0, 128)] = y
    return ys[0]


def _attention(q_s, k_s, v_s, r0, pos0, store):
    ls = []
    window = lambda w: pl.ds(_HALO + r0 - _DILATION * w, 16)

    def scores():
        q = [q_s[pl.ds(r0, 16), _block(c, 128)].astype(_F32) for c in range(8)]
        for w in range(_WINDOW):
            acc = q[0] * k_s[0, window(w), :]
            for c in range(1, 8):
                acc = acc + q[c] * k_s[c, window(w), :]
            ls.append(acc + pltpu.roll(acc, 64, 1))
        return _token([_words(l) for l in ls[-2:]])

    def softmax():
        for w in range(_WINDOW):
            l = (ls[w] + pltpu.roll(ls[w], 32, 1)) * (_HEAD_DIM ** -0.5)
            if pos0 is not None and r0 < _DILATION * w:
                pos = pos0 + r0 + jax.lax.broadcasted_iota(_I32, l.shape, 0)
                l = jnp.where(pos >= _DILATION * w, l, -1e9)
            ls[w] = l
        top = functools.reduce(jnp.maximum, ls)
        es = [jnp.exp(l - top) for l in ls]
        inv = 1.0 / functools.reduce(jnp.add, es)
        ls[:] = [e * inv for e in es]
        return _token([_words(inv)])

    def mix(*groups):
        def weighted(c):
            acc = ls[0] * v_s[c, window(0), :]
            for w in range(1, _WINDOW):
                acc = acc + ls[w] * v_s[c, window(w), :]
            return acc

        return _token([y for c in groups for y in store(r0, c, weighted(c), weighted(c + 4))])

    return scores, softmax, mix


def _attention_halves(views, keep, dst, pos0):
    def store_upper(r0, c, a11, a12):
        keep[c, pl.ds(r0, 16), :] = a11
        keep[c + 4, pl.ds(r0, 16), :] = a12
        return [_words(a11), _words(a12)]

    def store_lower(r0, c, a21, a22):
        left = _strassen_left(keep[c, pl.ds(r0, 16), :], keep[c + 4, pl.ds(r0, 16), :], a21, a22)
        return _store_packed(dst, pl.ds(r0 // 2, 8), _block(c, 128), left)[1:2]

    return [_attention(*views[p], r0, None if p else pos0, store)
            for r0 in range(0, views[0][0].shape[0], 16) for p, store in enumerate((store_upper, store_lower))]


@jax.jit
def pallas_sequential_preLN__sliding_local_dilated__glu_gated_geglu__prompt_kernel(
    A_x: jax.Array,
    A_wqkv: jax.Array,
    A_wo: jax.Array,
    B_x: jax.Array,
    B_w_gate: jax.Array,
    B_w_up: jax.Array,
    B_w_down: jax.Array,
):
    del B_x
    B, S, D = A_x.shape
    F = B_w_gate.shape[1]
    assert (B, S, D) == (1, 2048, _HEADS * _HEAD_DIM) and F % 512 == 0
    T = 256
    n, hf, hd, qd = S // T, T // 2, D // 2, D // 4
    NQ = NK = NS = 4
    QC, TK = D // NQ, S // NS
    KR, AR = 96, 48

    def kernel(x_hbm, wqkv_hbm, wo_hbm, wg_hbm, wu_hbm, wd_hbm, out_hbm,
               x_s, w_in, wo_in, wg_in, wu_in, wd_in, wgu, wd, wk, wv, wo, wo_tmp,
               xn_s, xsum_s, wq, qraw_s, q_s, k_s, v_s, keep_s, o_s, ha_s, hb_s, hna_s, hnb_s, zero_s,
               xsem, wsem, fsem, osem):
        def x_copy(i):
            return [pltpu.make_async_copy(x_hbm.at[_block(i, T)], x_s.at[_block(i, T)], xsem.at[i])]

        def q_copy(j):
            at = lambda ref, p: ref.at[_block((2 + p) * NQ + j, hf // NQ)]
            return [pltpu.make_async_copy(a, b, xsem.at[n + j]) for a, b in (
                (at(x_hbm, 0), at(x_s, 0)), (at(x_hbm, 1), at(x_s, 1)),
                (wqkv_hbm.at[:, _block(j, QC)], w_in.at[:, _block(j, QC)]))]

        def kv_copy(j):
            at = lambda ref, p: ref.at[_block(p * NK + j, hd // NK), pl.ds(D, 2 * D)]
            return [pltpu.make_async_copy(at(wqkv_hbm, p), at(w_in, p), wsem.at[j]) for p in range(2)]

        def o_copy():
            return [pltpu.make_async_copy(wo_hbm, wo_in, wsem.at[NK])]

        def ffn_copy(i):
            return [pltpu.make_async_copy(w.at[:, _block(i, w.shape[1] // NS), :],
                                          dst.at[i % 2, :, pl.ds(0, w.shape[1] // NS), :], fsem.at[i % 2])
                    for w, dst in ((wg_hbm, wg_in), (wu_hbm, wu_in), (wd_hbm, wd_in))]

        def start(copies):
            for c in copies:
                c.start()

        def wait(copies):
            for c in copies:
                c.wait()

        def normalize(i, rows):
            at = lambda ref: ref.at[:, _block(i, hf // 2), :]
            src = [x_s.at[_block(2 * i + p, hf)] for p in range(2)]
            return [_bind(_normalize_input, src, at(xn_s), at(xsum_s), r0, rows) for r0 in range(0, hf, rows)]

        def normalized(i):
            return jnp.concatenate([xn_s[p, _block(i, hf // 2), :] for p in range(2)], axis=0)

        def first_q_step(j, _):
            pl.when(j + 2 < NQ)(lambda: start(q_copy(j + 2)))
            pl.when(j + 2 == NQ)(lambda: start(x_copy(2) + kv_copy(0)))
            wait(q_copy(j))
            rows = hf // NQ
            at = lambda ref: ref.at[:, _block(NQ + j, rows // 2), :]
            src = [x_s.at[_block((2 + p) * NQ + j, rows)] for p in range(2)]
            jobs = [_bind(_normalize_input, src, at(xn_s), at(xsum_s), r0, 16) for r0 in range(0, rows, 16)]
            wq[:, _block(j, QC)] = w = _words(w_in[:, _block(j, QC)])
            qraw_s[pl.ds(0, hf), _block(j, QC)] = _pack(_dot(normalized(0), w, zero_s[...], [jobs], 2))

        def q_step(i, _):
            pl.when(i < NK)(lambda: start(x_copy(i + 2) + kv_copy(i)))
            pl.when(i == NK - 1)(lambda: start(sum([x_copy(j) for j in range(NK + 2, n)], [])))
            pl.when(i == NK)(lambda: start(o_copy() + ffn_copy(0)))
            pl.when(i + 1 < n)(lambda: wait(x_copy(i + 1)))
            pl.when((i > 1) & (i < NK + 2))(lambda: wait(kv_copy(i - 2)))
            prepare = []
            for j, w in enumerate((wk, wv)):
                cols = _block(jnp.where(i > 1, j + 1, 0), D)
                src = [w_in.at[_block(p, hd), cols].at[_clamped(i - 2, KR, hd)] for p in range(2)]
                dst = w.at[:, _clamped(i - 2, KR // 2, hd // 2), :]
                prepare += [_prepare_kv_weight(src, dst, r0) for r0 in range(0, KR, 16)]
            queues = [_staggered(prepare), normalize(jnp.minimum(i + 1, n - 1), 16)]
            qraw_s[_block(i, hf), :] = _pack(_dot(normalized(i), wq[...], zero_s[...], queues, 2))

        def kv_step(i, _):
            pl.when(i + 1 < NS)(lambda: start(ffn_copy(i + 1)))
            wait(ffn_copy(i))

            def project(i_again, w, dst, t0):
                dst = dst.at[:, _block(i, TK, _HALO), :]
                rows, m = _block(i_again, TK // 4), {}
                for t, k in enumerate((2, 4, 1, 3, 0, 5, 6), t0):
                    a = (xsum_s[_STRASSEN_SUMS.index(k), rows, :] if k in _STRASSEN_SUMS
                         else xn_s[k - 2, rows, _block(k - 2, hd)])
                    m[k] = _dot(a, w[k], zero_s[...], [_share(q, t - a0, a1 - a0) for q, a0, a1 in queues if a0 <= t < a1],
                                0 if t else 1)
                    y = m[k][:16, 1 * 128:][:, :128]
                    if t in [4, 6, 8, 10]:
                        qraw_s[_block(S // 16 + (i >> 8), 8), _block(0, 128)] = _words(y[:8])
                    if t in [5]:
                        for ref in (wg_in, wu_in, wd_in):
                            ref.at[i >> 8, 0][pl.ds(ref.shape[2] - 16, 16), _block(0, 128)] = y.astype(_BF16)
                y = _strassen_upper(m) + _strassen_lower(m)
                for t in range(TK // T):
                    for p in range(2):
                        for c in range(8):
                            dst[c, pl.ds(_HALO + t * T + p * hf, hf), :] = (
                                y[2 * p + c // 4][t * hf:(t + 1) * hf, c % 4 * 128:(c % 4 + 1) * 128])

            prepare = []
            for src, dst, scale, shift in ((wg_in, wgu, 2, 0), (wu_in, wgu, 2, 128), (wd_in, wd, 1, 0)):
                size = src.shape[2] - 16
                prepare += [_bind(_prepare_ffn_weight, src.at[i % 2], dst.at[:, _block(i, size // 2), :],
                                  r0, c0, scale * c0 + shift, group)
                            for r0 in range(0, size, 16) for c0 in range(0, src.shape[3] // 4, 128)
                            for group in _HK_GROUPS]
            views = [[q_s.at[_block(p, hf)].at[_clamped(i - 1, AR, hf)]]
                     + [ref.at[:, _block(p, hf, _HALO), :].at[:, _clamped(i - 1, AR, hf, _HALO), :]
                        for ref in (k_s, v_s)] for p in range(2)]
            attend = _attention_halves(views, keep_s, o_s.at[:, _clamped(i - 1, AR // 2, hf // 2), :],
                                       jnp.clip((i - 1) * AR, 0, hf - AR))
            layout = [_prepare_q(qraw_s.at[_block(i, TK // 2)], q_s.at[_block(i, TK)], r0, 32)
                      for r0 in range(0, TK, 32)]
            queues = [(prepare, 0, 14), ([_chain(a, b) for a, b, _ in attend], 0, 7),
                      (_staggered(layout), 7 - 1, 14), (_prepare_out_weight(wo_in, wo_tmp, wo, i), 0, 4),
                      ([_bind(mix, 0, 1, 2, 3) for _, _, mix in attend], 8, 14)]
            project(i, wv, v_s, 0)
            for c in range(8):
                v_s[c, pl.ds(0, _HALO), :] = jnp.broadcast_to(v_s[c, pl.ds(_HALO, 1), :], (_HALO, 128))
            project(i + (i >> 8), wk, k_s, 7)

        def main_step(i, _):
            zero = zero_s[...]
            whole = lambda rows, use=0: _block(i >> (8 + use), rows)
            hs, moments = (ha_s, hb_s), {}

            def residual(p, blocks):
                for t, y in enumerate(blocks):
                    hs[p][:, _block(t, hd)] = x_s[_block(2 * i + p, hf), _block(t, hd)].astype(_F32) + y

            def norm(p, r0):
                y, moments[p, r0] = _layernorm(hs[p].at[whole(hf)][pl.ds(r0, 16), :])
                upper = _layernorm(hs[0].at[whole(hf, 1)][pl.ds(r0, 16), :], moments[0, r0])[0] if p else y
                blocks = [v[:, k * qd:(k + 1) * qd] for v in (upper, y) for k in range(4)]
                left = _sums(_HK_LEFT[_HK_EARLY:] if p else _HK_LEFT[:_HK_EARLY], blocks)
                return _token(_store_packed(hnb_s if p else hna_s, pl.ds(r0 // 2, 8), slice(None), left)[-3:])

            norms = [[_bind(norm, p, r0) for r0 in range(0, hf, 16)] for p in range(2)]
            m = {k: _dot(o_s[k], wo[k], zero) for k in (2, 4, 3, 0, 6)}
            residual(0, _strassen_upper(m))
            m[1] = _dot(o_s[1], wo[1], zero)
            m[5] = _dot(o_s[5], wo[5], zero, [norms[0][:4]])
            _chain(*norms[0][4:])()
            residual(1, _strassen_lower(m))

            j = jnp.minimum(i + 1, n - 1)
            views = [[q_s.at[_block(2 * j + p, hf)]]
                     + [ref.at[:, _block(2 * j + p, hf, _HALO), :] for ref in (k_s, v_s)] for p in range(2)]
            attend = [job for scores, softmax, mix in _attention_halves(views, keep_s, o_s, None)
                      for job in (scores, _chain(softmax, _bind(mix, 0, 1)), _bind(mix, 2, 3))]

            lead, tiles = 4, F // 512
            orders = [_HK_FIRST if u < lead else _HK_ORDER for u in range(tiles)]
            ups = [step[1:] for step in sorted(
                (t if u < lead and t < _HK_EARLY else t + 11.5 * u, u, k)
                for u, order in enumerate(orders) for t, k in enumerate(order))]
            steps = ups + list(_HK_ORDER)
            jobs = {}
            for queue, span in ((norms[1], steps[8:_HK_EARLY * lead]), (attend, steps[_HK_EARLY * lead:-4])):
                jobs.update({step: [_share(queue, t, len(span))] for t, step in enumerate(span)})
            up = {}
            for u, k in ups:
                a = hna_s.at[k] if k < _HK_EARLY else hnb_s.at[k - _HK_EARLY]
                up[u, k] = _dot(a[whole(hf // 2, u), :], wgu.at[k][:, _block(u, 256)], zero, jobs.get((u, k), ()))

            def activation(u):
                ready = [orders[u].index(k) for k in range(len(_HK))]
                gate_up = _sums(_HK_OUT, [up[u, k] for k in range(len(_HK))], ready)
                ready = [max(t for t, c in zip(ready, row) if c) for row in _HK_OUT]
                return _sums(_HK_LEFT, [_geglu(y[:, :128], y[:, 128:]) for y in gate_up], ready)

            left = [jnp.concatenate(v, axis=1) for v in zip(*[activation(u) for u in range(tiles)])]
            down = {k: _dot(left[k].astype(_BF16), wd.at[k][...], zero, jobs.get(k, ())) for k in _HK_ORDER}
            out = _sums(_HK_OUT, [down[k] for k in range(len(_HK))], [_HK_ORDER.index(k) for k in range(len(_HK))])

            for p, t0, nt in ((1, 0, 3), (0, 0, 2), (0, 2, 2), (1, 3, 1)):
                for t in range(t0, t0 + nt):
                    y = hs[p][whole(hf), _block(t, qd)] + out[4 * p + t]
                    x_s[_block(2 * i + p, hf), _block(t, qd)] = y.astype(_BF16)
                at = lambda ref: ref.at[_block(2 * i + p, hf), pl.ds(t0 * qd, nt * qd)]
                pltpu.make_async_copy(at(x_s), at(out_hbm), osem).start()

        start(x_copy(0) + q_copy(0) + q_copy(1))
        zero_s[...] = jnp.zeros(zero_s.shape, _I32)
        wo_tmp[...] = jnp.zeros(wo_tmp.shape, _F32)
        for p in range(2):
            k_s[:, pl.ds(p * hf, AR + _HALO), :] = jnp.zeros((8, AR + _HALO, 128), _F32)
            q_s[pl.ds(p * hf, AR), :] = jnp.zeros((AR, D), _BF16)
        wait(x_copy(0))
        _chain(*normalize(0, hf))()
        jax.lax.fori_loop(0, NQ, first_q_step, None)
        jax.lax.fori_loop(1, n, q_step, None)
        wait(o_copy())
        jax.lax.fori_loop(0, NS, kv_step, None)
        jax.lax.fori_loop(0, n, main_step, None)
        pltpu.make_async_copy(x_s, out_hbm, osem).wait()

    vmem, dma = pltpu.VMEM, pltpu.SemaphoreType.DMA
    in_hbm = pl.BlockSpec(memory_space=pl.ANY)
    row_blocks = lambda w: w.reshape(4, w.shape[0] // 4, w.shape[1])
    out = pl.pallas_call(
        kernel,
        out_shape=jax.ShapeDtypeStruct((S, D), A_x.dtype),
        in_specs=[in_hbm] * 6,
        out_specs=in_hbm,
        scratch_shapes=[
            vmem((S, D), _BF16), vmem((D, 3 * D), _BF16), vmem((D, D), _BF16),
            vmem((2, 4, qd // NS + 16, F), _BF16), vmem((2, 4, qd // NS + 16, F), _BF16),
            vmem((2, 4, F // 4 // NS + 16, D), _BF16),
            vmem((len(_HK), qd // 2, F // 2), _I32), vmem((len(_HK), F // 8, qd), _I32),
            vmem((7, hd // 2, hd), _I32), vmem((7, hd // 2, hd), _I32), vmem((7, hd // 2, hd), _I32),
            vmem((2, _HEADS * (_HEAD_DIM + 2), 128), _F32),
            vmem((2, S // 4, D), _I32), vmem((len(_STRASSEN_SUMS), S // 4, hd), _I32),
            vmem((D // 2, D), _I32), vmem((S // 2 + 8, D), _I32), vmem((S, D), _BF16),
            vmem((8, S + _HALO + 8, 128), _F32), vmem((8, S + _HALO + 8, 128), _F32),
            vmem((8, hf, 128), _F32), vmem((7, hf // 2, hd), _I32),
            vmem((hf, D), _F32), vmem((hf, D), _F32),
            vmem((_HK_EARLY, hf // 2, qd), _I32), vmem((len(_HK) - _HK_EARLY, hf // 2, qd), _I32),
            vmem((8, 128), _I32),
            dma((n + NQ,)), dma((NK + 1,)), dma((2,)), dma(()),
        ],
        compiler_params=pltpu.CompilerParams(
            vmem_limit_bytes=126 * 1024 * 1024,
            flags={"XLA_TPU_EVENLY_DISTRIBUTE_CRITICAL_NODES": True, "XLA_TPU_RESCHEDULE_DMA_DONES": True},
        ),
    )(A_x.reshape(S, D), A_wqkv, A_wo, row_blocks(B_w_gate), row_blocks(B_w_up), row_blocks(B_w_down))
    return out.reshape(B, S, D)
```

```python
import functools

import jax
import jax.experimental.pallas as pl
import jax.experimental.pallas.tpu as pltpu
import jax.numpy as jnp
import numpy as np

_HEADS, _HEAD_DIM, _WINDOW, _DILATION = 32, 32, 8, 2
_HALO = 16
_EPS = 1e-5
_F32, _BF16, _I32 = jnp.float32, jnp.bfloat16, jnp.int32
_bind = functools.partial


def _words(x):
    return pltpu.bitcast(x, _I32)


def _pack(x):
    return _words(x.astype(_BF16))


def _unpack(x):
    return pltpu.bitcast(x, _BF16)


def _block(i, size, extra=0):
    return pl.ds(i * size if isinstance(i, int) else pl.multiple_of(i * size, size), size + extra)


def _clamped(i, size, total, extra=0):
    start = jnp.clip(i * size, 0, total - size)
    return pl.ds(pl.multiple_of(start, 8 if size % 16 else 16), size + extra)


def _store_packed(dst, rows, cols, ys):
    ys = [_pack(y) for y in ys]
    for k, y in enumerate(ys):
        dst.at[k][rows, cols] = y
    return ys


def _token(parts):
    return functools.reduce(jnp.bitwise_or, [
        p[r:r + 8, c:c + 128] for p in parts
        for r in range(0, p.shape[0], 8) for c in range(0, p.shape[1], 128)])


def _dot(a, w, zero, queues=(), first=0):
    if any(queues):
        nt, nk = w.shape[1] // 128, pl.cdiv(w.shape[0], 256)
        due = {}
        for queue in queues:
            for j, job in enumerate(queue):
                slot = first + ((j + 1) * (nt * nk - first) - 1) // len(queue)
                due.setdefault(divmod(slot, nk), []).append(job())
        parts = []
        for k in range(nk):
            top = [w[k * 256:k * 256 + 8, t * 128:(t + 1) * 128] for t in range(nt)]
            top = [v | (_token(due[t, k]) & zero) if (t, k) in due else v for t, v in enumerate(top)]
            parts += [jnp.concatenate(top, axis=1), w[k * 256 + 8:(k + 1) * 256]]
        w = jnp.concatenate(parts, axis=0)
    return jnp.dot(a if a.dtype == _BF16 else _unpack(a), _unpack(w), preferred_element_type=_F32)


def _share(jobs, j, parts):
    return jobs[j * len(jobs) // parts:(j + 1) * len(jobs) // parts]


def _chain(*jobs):
    return lambda: [job() for job in jobs][-1]


def _staggered(chains):
    depth = len(chains[0])
    return [_bind(lambda jobs: _token([job() for job in jobs]),
                  [c[t - i] for i, c in enumerate(chains) if 0 <= t - i < depth])
            for t in range(len(chains) + depth - 1)]


def _strassen_left(a11, a12, a21, a22):
    return (a11 + a22, a21 + a22, a11, a22, a11 + a12, a21 - a11, a12 - a22)


def _strassen_right(b11, b12, b21, b22):
    return (b11 + b22, b11, b12 - b22, b21 - b11, b22, b11 + b12, b21 + b22)


def _strassen_upper(m):
    return (((m[3] - m[4]) + m[0]) + m[6], m[2] + m[4])


def _strassen_lower(m):
    return (m[1] + m[3], ((m[2] - m[1]) + m[0]) + m[5])


_STRASSEN_SUMS = (0, 1, 4, 5, 6)

_HK = [[[{"+": 1, ".": 0, "-": -1}[ch] for ch in part] for part in line.split()] for line in (
    "+....... +-......+....... +...-...",
    ".+...... ...++-.-.-...... .-......",
    "...+.... ...+.......-+-.- ...-...+",
    "+.-..... ........+....... -.+.....",
    ".+-..... .........+...... .-+..+-.",
    "..+-.... ...........+.... ..++....",
    "++.+.... ...+............ ++.+....",
    ".....+.. .+...--.....+-.. .....-..",
    "......+. ..+......++...+. ..-...+.",
    "+...+... +.+.-........... ....+...",
    "..+...+. ......+.+.+-.... ..+.....",
    "...+...+ ...+...-....+.+- .......-",
    "....++.. .+..........-... --..++..",
    "....+.-. ..+............. ....-.+.",
    "+.....+. ..+.....-....... ..+.-...",
    ".....+.- ............+-.. .-.+.+.-",
    "......+- ..............+. ......--",
    "...+..+. ...........+..+. ..+....+",
    "+...++.. .+..-........... ++..-...",
    ".+-...-. ......+..-...... ..+..+-.",
    "...+.-.+ ...+...-....-+.. .+.-...+",
    "....++.+ ............+... ....++.+",
    "...+--.. ...+........-... --.....-",
    "++..++.. ...+-........... --......",
    ".+-..+-. ......+......... .....-+.",
    ".+.-.+.- ...+...-........ .+.-....",
)]
_HK_LEFT, _HK_RIGHT = ([line[k] for line in _HK] for k in range(2))
_HK_OUT = [[line[2][o] for line in _HK] for o in range(8)]
_HK_EARLY = 7
_HK_FIRST = (4, 1, 6, 5, 0, 3, 2, 12, 22, 21, 19, 20, 15, 18, 25, 24, 23, 13, 7, 14, 9, 8, 16, 17, 10, 11)
_HK_ORDER = (15, 24, 22, 18, 19, 21, 6, 23, 4, 13, 12, 16, 8, 3, 0, 14, 9, 25, 7, 20, 1, 5, 2, 17, 10, 11)
_HK_GROUPS = ((2, 11, 15, 20, 21, 22, 25, 6), (8, 10, 13, 14, 16, 17, 19, 24, 3, 4, 5), (1, 7, 0, 9, 12, 18, 23))


def _sums(rows, xs, ready=None):
    xs, ready = list(xs), list(ready or range(len(xs)))
    rows = [{j: c for j, c in enumerate(row) if c} for row in rows]
    while True:
        count = {}
        for row in rows:
            for pair in [(a, b, row[a] * row[b]) for a in row for b in row if a < b]:
                count[pair] = count.get(pair, 0) + 1
        best = max(sorted(count), key=count.get, default=None)
        if best is None or count[best] < 2:
            break
        a, b, sign = best
        xs.append(xs[a] + xs[b] if sign > 0 else xs[a] - xs[b])
        ready.append(max(ready[a], ready[b]))
        for row in rows:
            if row.get(a, 0) * row.get(b, 0) == sign:
                row[len(xs) - 1] = row.pop(a)
                del row[b]
    out = []
    for row in rows:
        (j, sign), *rest = sorted(row.items(), key=lambda t: (ready[t[0]], t[0]))
        acc = xs[j]
        for j, c in rest:
            acc = acc + xs[j] if c == sign else acc - xs[j] if sign > 0 else xs[j] - acc
            sign = max(sign, c)
        out.append(acc if sign > 0 else -acc)
    return out


def _layernorm(x, moments=None):
    mean = moments[0] if moments else jnp.mean(x, axis=-1, keepdims=True)
    xc = x - mean
    scale = moments[1] if moments else jax.lax.rsqrt(jnp.mean(xc * xc, axis=-1, keepdims=True) + _EPS)
    return xc * scale, (mean, scale)


def _geglu(g, u):
    c = float(np.sqrt(2.0 / np.pi))
    th = jnp.tanh(g * (c + (c * 0.044715) * (g * g)))
    half = (0.5 * g) * u
    return half * th + half


def _normalize_input(src, plain, sums, r0, rows):
    hd = src[0].shape[1] // 2
    a, b = (_layernorm(ref[pl.ds(r0, rows), :].astype(_F32))[0] for ref in src)
    at = pl.ds(r0 // 2, rows // 2)
    _store_packed(plain, at, slice(None), (a, b))
    left = _strassen_left(a[:, :hd], a[:, hd:], b[:, :hd], b[:, hd:])
    return _token(_store_packed(sums, at, slice(None), [left[k] for k in _STRASSEN_SUMS])[1:3])


def _heads_minor(load, store):
    vs = []
    lanes = lambda: jax.lax.broadcasted_iota(_I32, vs[0].shape, 1)

    def skew():
        vs.extend(pltpu.roll(load(g), 4 * g, 1) if g else load(g) for g in range(8))
        return _token(vs[4:])

    def exchange():
        us = [vs[-j % 8] for j in range(8)]
        for b in (1, 2, 4):
            moved = (lanes() & (4 * b)) != 0
            us = [jnp.where(moved, us[(j - b) % 8], us[j]) for j in range(8)]
        vs[:] = [pltpu.roll(u, 128 - 4 * j, 1) if j else u for j, u in enumerate(us)]
        return _token(vs[4:])

    def shuffle():
        lane = lanes()
        idx = (lane & 3) * 32 + (lane & 28) + (lane >> 5)
        return store([jnp.take_along_axis(v, idx, axis=1, mode="promise_in_bounds") for v in vs])

    return [skew, exchange, shuffle]


def _prepare_q(src, dst, r0, rows):
    def store(vs):
        for j, v in enumerate(vs):
            dst[pl.ds(r0, rows), _block(j, 128)] = _unpack(v)
        return _token(vs[4:])

    return _heads_minor(lambda g: src[pl.ds(r0 // 2, rows // 2), _block(g, 128)], store)


def _prepare_kv_weight(src, dst, r0):
    def load(g):
        return jnp.concatenate([_words(ref[pl.ds(r0, 16), _block(g, 128)]) for ref in src], axis=0)

    def store(vs):
        vs = [_unpack(v).astype(_F32) for v in vs]
        return _token([_store_packed(
            dst, pl.ds(r0 // 2, 8), _block(j, 128),
            _strassen_right(vs[j][:16], vs[j + 4][:16], vs[j][16:], vs[j + 4][16:]))[0] for j in range(4)])

    return _heads_minor(load, store)


def _prepare_out_weight(src, tmp, dst, c):
    pitch = _HEAD_DIM + 1

    def spread(h0):
        ys = []
        for h in range(h0, h0 + 4):
            for k in range(2):
                ys.append(src[_block(h, _HEAD_DIM), _block(c + 4 * k, 128)].astype(_F32))
                tmp[k, pl.ds(h * pitch, _HEAD_DIM), :] = ys[-1]
        return _token([_words(y[:8]) for y in ys])

    def gather(d0):
        ys = []
        for d in range(d0, d0 + 2):
            b = [tmp[k, pl.ds(d + j * _HEAD_DIM // 2, _HEADS, stride=pitch), :] for j in range(2) for k in range(2)]
            ys.append(_store_packed(dst, _block(d, _HEADS // 2), _block(c, 128), _strassen_right(*b))[0])
        return _token(ys)

    return ([_bind(spread, h) for h in range(0, _HEADS, 4)]
            + [_bind(gather, d) for d in range(0, _HEAD_DIM // 2, 2)])


def _prepare_ffn_weight(src, dst, r0, c0, d0, group):
    quarter = src.shape[2] // 4
    b = [src.at[j // 4][pl.ds(r0, 16), pl.ds(j % 4 * quarter + c0, 128)].astype(_F32)
         if any(_HK_RIGHT[k][j] for k in group) else None for j in range(16)]
    ys = [_pack(y) for y in _sums([_HK_RIGHT[k] for k in group], b)]
    for k, y in zip(group, ys):
        dst.at[k][pl.ds(r0 // 2, 8), pl.ds(d0, 128)] = y
    return ys[0]


def _attention(q_s, k_s, v_s, r0, pos0, store):
    ls = []
    window = lambda w: pl.ds(_HALO + r0 - _DILATION * w, 16)

    def scores():
        q = [q_s[pl.ds(r0, 16), _block(c, 128)].astype(_F32) for c in range(8)]
        for w in range(_WINDOW):
            acc = q[0] * k_s[0, window(w), :]
            for c in range(1, 8):
                acc = acc + q[c] * k_s[c, window(w), :]
            ls.append(acc + pltpu.roll(acc, 64, 1))
        return _token([_words(l) for l in ls[-2:]])

    def softmax():
        for w in range(_WINDOW):
            l = (ls[w] + pltpu.roll(ls[w], 32, 1)) * (_HEAD_DIM ** -0.5)
            if pos0 is not None and r0 < _DILATION * w:
                pos = pos0 + r0 + jax.lax.broadcasted_iota(_I32, l.shape, 0)
                l = jnp.where(pos >= _DILATION * w, l, -1e9)
            ls[w] = l
        top = functools.reduce(jnp.maximum, ls)
        es = [jnp.exp(l - top) for l in ls]
        inv = 1.0 / functools.reduce(jnp.add, es)
        ls[:] = [e * inv for e in es]
        return _token([_words(inv)])

    def mix(*groups):
        def weighted(c):
            acc = ls[0] * v_s[c, window(0), :]
            for w in range(1, _WINDOW):
                acc = acc + ls[w] * v_s[c, window(w), :]
            return acc

        return _token([y for c in groups for y in store(r0, c, weighted(c), weighted(c + 4))])

    return scores, softmax, mix


def _attention_halves(views, keep, dst, pos0):
    def store_upper(r0, c, a11, a12):
        keep[c, pl.ds(r0, 16), :] = a11
        keep[c + 4, pl.ds(r0, 16), :] = a12
        return [_words(a11), _words(a12)]

    def store_lower(r0, c, a21, a22):
        left = _strassen_left(keep[c, pl.ds(r0, 16), :], keep[c + 4, pl.ds(r0, 16), :], a21, a22)
        return _store_packed(dst, pl.ds(r0 // 2, 8), _block(c, 128), left)[1:2]

    return [_attention(*views[p], r0, None if p else pos0, store)
            for r0 in range(0, views[0][0].shape[0], 16) for p, store in enumerate((store_upper, store_lower))]


@jax.jit
def pallas_sequential_preLN__sliding_local_dilated__glu_gated_geglu__prompt_kernel(
    A_x: jax.Array,
    A_wqkv: jax.Array,
    A_wo: jax.Array,
    B_x: jax.Array,
    B_w_gate: jax.Array,
    B_w_up: jax.Array,
    B_w_down: jax.Array,
):
    del B_x
    B, S, D = A_x.shape
    F = B_w_gate.shape[1]
    assert (B, S, D) == (1, 2048, _HEADS * _HEAD_DIM) and F % 512 == 0
    T = 256
    n, hf, hd, qd = S // T, T // 2, D // 2, D // 4
    NQ = NK = NS = 4
    QC, TK = D // NQ, S // NS
    KR, AR = 96, 48

    def kernel(x_hbm, wqkv_hbm, wo_hbm, wg_hbm, wu_hbm, wd_hbm, out_hbm,
               x_s, w_in, wo_in, wg_in, wu_in, wd_in, wgu, wd, wk, wv, wo, wo_tmp,
               xn_s, xsum_s, wq, qraw_s, q_s, k_s, v_s, keep_s, o_s, ha_s, hb_s, hna_s, hnb_s, zero_s,
               xsem, wsem, fsem, osem):
        def x_copy(i):
            return [pltpu.make_async_copy(x_hbm.at[_block(i, T)], x_s.at[_block(i, T)], xsem.at[i])]

        def q_copy(j):
            at = lambda ref, p: ref.at[_block((2 + p) * NQ + j, hf // NQ)]
            return [pltpu.make_async_copy(a, b, xsem.at[n + j]) for a, b in (
                (at(x_hbm, 0), at(x_s, 0)), (at(x_hbm, 1), at(x_s, 1)),
                (wqkv_hbm.at[:, _block(j, QC)], w_in.at[:, _block(j, QC)]))]

        def kv_copy(j):
            at = lambda ref, p: ref.at[_block(p * NK + j, hd // NK), pl.ds(D, 2 * D)]
            return [pltpu.make_async_copy(at(wqkv_hbm, p), at(w_in, p), wsem.at[j]) for p in range(2)]

        def o_copy():
            return [pltpu.make_async_copy(wo_hbm, wo_in, wsem.at[NK])]

        def ffn_copy(i):
            return [pltpu.make_async_copy(w.at[:, _block(i, w.shape[1] // NS), :],
                                          dst.at[i % 2, :, pl.ds(0, w.shape[1] // NS), :], fsem.at[i % 2])
                    for w, dst in ((wg_hbm, wg_in), (wu_hbm, wu_in), (wd_hbm, wd_in))]

        def start(copies):
            for c in copies:
                c.start()

        def wait(copies):
            for c in copies:
                c.wait()

        def normalize(i, rows):
            at = lambda ref: ref.at[:, _block(i, hf // 2), :]
            src = [x_s.at[_block(2 * i + p, hf)] for p in range(2)]
            return [_bind(_normalize_input, src, at(xn_s), at(xsum_s), r0, rows) for r0 in range(0, hf, rows)]

        def normalized(i):
            return jnp.concatenate([xn_s[p, _block(i, hf // 2), :] for p in range(2)], axis=0)

        def first_q_step(j, _):
            pl.when(j + 2 < NQ)(lambda: start(q_copy(j + 2)))
            pl.when(j + 2 == NQ)(lambda: start(x_copy(2) + kv_copy(0)))
            wait(q_copy(j))
            rows = hf // NQ
            at = lambda ref: ref.at[:, _block(NQ + j, rows // 2), :]
            src = [x_s.at[_block((2 + p) * NQ + j, rows)] for p in range(2)]
            jobs = [_bind(_normalize_input, src, at(xn_s), at(xsum_s), r0, 16) for r0 in range(0, rows, 16)]
            wq[:, _block(j, QC)] = w = _words(w_in[:, _block(j, QC)])
            qraw_s[pl.ds(0, hf), _block(j, QC)] = _pack(_dot(normalized(0), w, zero_s[...], [jobs], 2))

        def q_step(i, _):
            pl.when(i < NK)(lambda: start(x_copy(i + 2) + kv_copy(i)))
            pl.when(i == NK - 1)(lambda: start(sum([x_copy(j) for j in range(NK + 2, n)], [])))
            pl.when(i == NK)(lambda: start(o_copy() + ffn_copy(0)))
            pl.when(i + 1 < n)(lambda: wait(x_copy(i + 1)))
            pl.when((i > 1) & (i < NK + 2))(lambda: wait(kv_copy(i - 2)))
            prepare = []
            for j, w in enumerate((wk, wv)):
                cols = _block(jnp.where(i > 1, j + 1, 0), D)
                src = [w_in.at[_block(p, hd), cols].at[_clamped(i - 2, KR, hd)] for p in range(2)]
                dst = w.at[:, _clamped(i - 2, KR // 2, hd // 2), :]
                prepare += [_prepare_kv_weight(src, dst, r0) for r0 in range(0, KR, 16)]
            queues = [_staggered(prepare), normalize(jnp.minimum(i + 1, n - 1), 16)]
            qraw_s[_block(i, hf), :] = _pack(_dot(normalized(i), wq[...], zero_s[...], queues, 2))

        def kv_step(i, _):
            pl.when(i + 1 < NS)(lambda: start(ffn_copy(i + 1)))
            wait(ffn_copy(i))

            def project(i_again, w, dst, t0):
                dst = dst.at[:, _block(i, TK, _HALO), :]
                rows, m = _block(i_again, TK // 4), {}
                for t, k in enumerate((2, 4, 1, 3, 0, 5, 6), t0):
                    a = (xsum_s[_STRASSEN_SUMS.index(k), rows, :] if k in _STRASSEN_SUMS
                         else xn_s[k - 2, rows, _block(k - 2, hd)])
                    m[k] = _dot(a, w[k], zero_s[...], [_share(q, t - a0, a1 - a0) for q, a0, a1 in queues if a0 <= t < a1],
                                0 if t else 1)
                    y = m[k][:16, 128:256]
                    if t in (4, 6, 8, 10):
                        qraw_s[_block(S // 16 + (i >> 8), 8), _block(0, 128)] = _words(y[:8])
                    if t == 5:
                        for ref in (wg_in, wu_in, wd_in):
                            ref.at[i >> 8, 0][pl.ds(ref.shape[2] - 16, 16), _block(0, 128)] = y.astype(_BF16)
                y = _strassen_upper(m) + _strassen_lower(m)
                for t in range(TK // T):
                    for p in range(2):
                        for c in range(8):
                            dst[c, pl.ds(_HALO + t * T + p * hf, hf), :] = (
                                y[2 * p + c // 4][t * hf:(t + 1) * hf, c % 4 * 128:(c % 4 + 1) * 128])

            prepare = []
            for src, dst, scale, shift in ((wg_in, wgu, 2, 0), (wu_in, wgu, 2, 128), (wd_in, wd, 1, 0)):
                size = src.shape[2] - 16
                prepare += [_bind(_prepare_ffn_weight, src.at[i % 2], dst.at[:, _block(i, size // 2), :],
                                  r0, c0, scale * c0 + shift, group)
                            for r0 in range(0, size, 16) for c0 in range(0, src.shape[3] // 4, 128)
                            for group in _HK_GROUPS]
            views = [[q_s.at[_block(p, hf)].at[_clamped(i - 1, AR, hf)]]
                     + [ref.at[:, _block(p, hf, _HALO), :].at[:, _clamped(i - 1, AR, hf, _HALO), :]
                        for ref in (k_s, v_s)] for p in range(2)]
            attend = _attention_halves(views, keep_s, o_s.at[:, _clamped(i - 1, AR // 2, hf // 2), :],
                                       jnp.clip((i - 1) * AR, 0, hf - AR))
            layout = [_prepare_q(qraw_s.at[_block(i, TK // 2)], q_s.at[_block(i, TK)], r0, 32)
                      for r0 in range(0, TK, 32)]
            queues = [(prepare, 0, 14), ([_chain(a, b) for a, b, _ in attend], 0, 7),
                      (_staggered(layout), 6, 14), (_prepare_out_weight(wo_in, wo_tmp, wo, i), 0, 4),
                      ([_bind(mix, 0, 1, 2, 3) for _, _, mix in attend], 8, 14)]
            project(i, wv, v_s, 0)
            for c in range(8):
                v_s[c, pl.ds(0, _HALO), :] = jnp.broadcast_to(v_s[c, pl.ds(_HALO, 1), :], (_HALO, 128))
            project(i + (i >> 8), wk, k_s, 7)

        def main_step(i, _):
            zero = zero_s[...]
            whole = lambda rows, use=0: _block(i >> (8 + use), rows)
            hs, moments = (ha_s, hb_s), {}

            def residual(p, blocks):
                for t, y in enumerate(blocks):
                    hs[p][:, _block(t, hd)] = x_s[_block(2 * i + p, hf), _block(t, hd)].astype(_F32) + y

            def norm(p, r0):
                y, moments[p, r0] = _layernorm(hs[p].at[whole(hf)][pl.ds(r0, 16), :])
                upper = _layernorm(hs[0].at[whole(hf, 1)][pl.ds(r0, 16), :], moments[0, r0])[0] if p else y
                blocks = [v[:, k * qd:(k + 1) * qd] for v in (upper, y) for k in range(4)]
                left = _sums(_HK_LEFT[_HK_EARLY:] if p else _HK_LEFT[:_HK_EARLY], blocks)
                return _token(_store_packed(hnb_s if p else hna_s, pl.ds(r0 // 2, 8), slice(None), left)[-3:])

            norms = [[_bind(norm, p, r0) for r0 in range(0, hf, 16)] for p in range(2)]
            m = {k: _dot(o_s[k], wo[k], zero) for k in (2, 4, 3, 0, 6)}
            residual(0, _strassen_upper(m))
            m[1] = _dot(o_s[1], wo[1], zero)
            m[5] = _dot(o_s[5], wo[5], zero, [norms[0][:4]])
            _chain(*norms[0][4:])()
            residual(1, _strassen_lower(m))

            j = jnp.minimum(i + 1, n - 1)
            views = [[q_s.at[_block(2 * j + p, hf)]]
                     + [ref.at[:, _block(2 * j + p, hf, _HALO), :] for ref in (k_s, v_s)] for p in range(2)]
            attend = [job for scores, softmax, mix in _attention_halves(views, keep_s, o_s, None)
                      for job in (scores, _chain(softmax, _bind(mix, 0, 1)), _bind(mix, 2, 3))]

            lead, tiles = 4, F // 512
            orders = [_HK_FIRST if u < lead else _HK_ORDER for u in range(tiles)]
            ups = [step[1:] for step in sorted(
                (t if u < lead and t < _HK_EARLY else t + 11.5 * u, u, k)
                for u, order in enumerate(orders) for t, k in enumerate(order))]
            steps = ups + list(_HK_ORDER)
            jobs = {}
            for queue, span in ((norms[1], steps[8:_HK_EARLY * lead]), (attend, steps[_HK_EARLY * lead:-4])):
                jobs.update({step: [_share(queue, t, len(span))] for t, step in enumerate(span)})
            up = {}
            for u, k in ups:
                a = hna_s.at[k] if k < _HK_EARLY else hnb_s.at[k - _HK_EARLY]
                up[u, k] = _dot(a[whole(hf // 2, u), :], wgu.at[k][:, _block(u, 256)], zero, jobs.get((u, k), ()))

            def activation(u):
                ready = [orders[u].index(k) for k in range(len(_HK))]
                gate_up = _sums(_HK_OUT, [up[u, k] for k in range(len(_HK))], ready)
                ready = [max(t for t, c in zip(ready, row) if c) for row in _HK_OUT]
                return _sums(_HK_LEFT, [_geglu(y[:, :128], y[:, 128:]) for y in gate_up], ready)

            left = [jnp.concatenate(v, axis=1) for v in zip(*[activation(u) for u in range(tiles)])]
            down = {k: _dot(left[k].astype(_BF16), wd.at[k][...], zero, jobs.get(k, ())) for k in _HK_ORDER}
            out = _sums(_HK_OUT, [down[k] for k in range(len(_HK))], [_HK_ORDER.index(k) for k in range(len(_HK))])

            for p, t0, nt in ((1, 0, 3), (0, 0, 2), (0, 2, 2), (1, 3, 1)):
                for t in range(t0, t0 + nt):
                    y = hs[p][whole(hf), _block(t, qd)] + out[4 * p + t]
                    x_s[_block(2 * i + p, hf), _block(t, qd)] = y.astype(_BF16)
                at = lambda ref: ref.at[_block(2 * i + p, hf), pl.ds(t0 * qd, nt * qd)]
                pltpu.make_async_copy(at(x_s), at(out_hbm), osem).start()

        start(x_copy(0) + q_copy(0) + q_copy(1))
        zero_s[...] = jnp.zeros(zero_s.shape, _I32)
        wo_tmp[...] = jnp.zeros(wo_tmp.shape, _F32)
        for p in range(2):
            k_s[:, pl.ds(p * hf, AR + _HALO), :] = jnp.zeros((8, AR + _HALO, 128), _F32)
            q_s[pl.ds(p * hf, AR), :] = jnp.zeros((AR, D), _BF16)
        wait(x_copy(0))
        _chain(*normalize(0, hf))()
        jax.lax.fori_loop(0, NQ, first_q_step, None)
        jax.lax.fori_loop(1, n, q_step, None)
        wait(o_copy())
        jax.lax.fori_loop(0, NS, kv_step, None)
        jax.lax.fori_loop(0, n, main_step, None)
        pltpu.make_async_copy(x_s, out_hbm, osem).wait()

    vmem, dma = pltpu.VMEM, pltpu.SemaphoreType.DMA
    in_hbm = pl.BlockSpec(memory_space=pl.ANY)
    row_blocks = lambda w: w.reshape(4, w.shape[0] // 4, w.shape[1])
    out = pl.pallas_call(
        kernel,
        out_shape=jax.ShapeDtypeStruct((S, D), A_x.dtype),
        in_specs=[in_hbm] * 6,
        out_specs=in_hbm,
        scratch_shapes=[
            vmem((S, D), _BF16), vmem((D, 3 * D), _BF16), vmem((D, D), _BF16),
            vmem((2, 4, qd // NS + 16, F), _BF16), vmem((2, 4, qd // NS + 16, F), _BF16),
            vmem((2, 4, F // 4 // NS + 16, D), _BF16),
            vmem((len(_HK), qd // 2, F // 2), _I32), vmem((len(_HK), F // 8, qd), _I32),
            vmem((7, hd // 2, hd), _I32), vmem((7, hd // 2, hd), _I32), vmem((7, hd // 2, hd), _I32),
            vmem((2, _HEADS * (_HEAD_DIM + 2), 128), _F32),
            vmem((2, S // 4, D), _I32), vmem((len(_STRASSEN_SUMS), S // 4, hd), _I32),
            vmem((D // 2, D), _I32), vmem((S // 2 + 8, D), _I32), vmem((S, D), _BF16),
            vmem((8, S + _HALO + 8, 128), _F32), vmem((8, S + _HALO + 8, 128), _F32),
            vmem((8, hf, 128), _F32), vmem((7, hf // 2, hd), _I32),
            vmem((hf, D), _F32), vmem((hf, D), _F32),
            vmem((_HK_EARLY, hf // 2, qd), _I32), vmem((len(_HK) - _HK_EARLY, hf // 2, qd), _I32),
            vmem((8, 128), _I32),
            dma((n + NQ,)), dma((NK + 1,)), dma((2,)), dma(()),
        ],
        compiler_params=pltpu.CompilerParams(
            vmem_limit_bytes=126 * 1024 * 1024,
            flags={"XLA_TPU_EVENLY_DISTRIBUTE_CRITICAL_NODES": True},
        ),
    )(A_x.reshape(S, D), A_wqkv, A_wo, row_blocks(B_w_gate), row_blocks(B_w_up), row_blocks(B_w_down))
    return out.reshape(B, S, D)
```

```python
import functools

import jax
import jax.experimental.pallas as pl
import jax.experimental.pallas.tpu as pltpu
import jax.numpy as jnp
import numpy as np

_HEADS, _HEAD_DIM, _WINDOW, _DILATION = 32, 32, 8, 2
_HALO = 16
_EPS = 1e-5
_F32, _BF16, _I32 = jnp.float32, jnp.bfloat16, jnp.int32
_bind = functools.partial


def _words(x):
    return pltpu.bitcast(x, _I32)


def _pack(x):
    return _words(x.astype(_BF16))


def _unpack(x):
    return pltpu.bitcast(x, _BF16)


def _block(i, size, extra=0):
    return pl.ds(i * size if isinstance(i, int) else pl.multiple_of(i * size, size), size + extra)


def _clamped(i, size, total, extra=0):
    start = jnp.clip(i * size, 0, total - size)
    return pl.ds(pl.multiple_of(start, 8 if size % 16 else 16), size + extra)


def _store_packed(dst, rows, cols, ys):
    ys = [_pack(y) for y in ys]
    for k, y in enumerate(ys):
        dst.at[k][rows, cols] = y
    return ys


def _token(parts):
    return functools.reduce(jnp.bitwise_or, [
        p[r:r + 8, c:c + 128] for p in parts
        for r in range(0, p.shape[0], 8) for c in range(0, p.shape[1], 128)])


def _dot(a, w, zero, queues=(), first=0):
    if any(queues):
        nt, nk = w.shape[1] // 128, pl.cdiv(w.shape[0], 256)
        due = {}
        for queue in queues:
            for j, job in enumerate(queue):
                slot = first + ((j + 1) * (nt * nk - first) - 1) // len(queue)
                due.setdefault(divmod(slot, nk), []).append(job())
        parts = []
        for k in range(nk):
            top = [w[k * 256:k * 256 + 8, t * 128:(t + 1) * 128] for t in range(nt)]
            top = [v | (_token(due[t, k]) & zero) if (t, k) in due else v for t, v in enumerate(top)]
            parts += [jnp.concatenate(top, axis=1), w[k * 256 + 8:(k + 1) * 256]]
        w = jnp.concatenate(parts, axis=0)
    return jnp.dot(a if a.dtype == _BF16 else _unpack(a), _unpack(w), preferred_element_type=_F32)


def _share(jobs, j, parts):
    return jobs[j * len(jobs) // parts:(j + 1) * len(jobs) // parts]


def _chain(*jobs):
    return lambda: [job() for job in jobs][-1]


def _staggered(chains):
    depth = len(chains[0])
    return [_bind(lambda jobs: _token([job() for job in jobs]),
                  [c[t - i] for i, c in enumerate(chains) if 0 <= t - i < depth])
            for t in range(len(chains) + depth - 1)]


def _strassen_left(a11, a12, a21, a22):
    return (a11 + a22, a21 + a22, a11, a22, a11 + a12, a21 - a11, a12 - a22)


def _strassen_right(b11, b12, b21, b22):
    return (b11 + b22, b11, b12 - b22, b21 - b11, b22, b11 + b12, b21 + b22)


def _strassen_upper(m):
    return (((m[3] - m[4]) + m[0]) + m[6], m[2] + m[4])


def _strassen_lower(m):
    return (m[1] + m[3], ((m[2] - m[1]) + m[0]) + m[5])


_STRASSEN_SUMS = (0, 1, 4, 5, 6)

_HK = [[[{"+": 1, ".": 0, "-": -1}[ch] for ch in part] for part in line.split()] for line in (
    "+....... +-......+....... +...-...",
    ".+...... ...++-.-.-...... .-......",
    "...+.... ...+.......-+-.- ...-...+",
    "+.-..... ........+....... -.+.....",
    ".+-..... .........+...... .-+..+-.",
    "..+-.... ...........+.... ..++....",
    "++.+.... ...+............ ++.+....",
    ".....+.. .+...--.....+-.. .....-..",
    "......+. ..+......++...+. ..-...+.",
    "+...+... +.+.-........... ....+...",
    "..+...+. ......+.+.+-.... ..+.....",
    "...+...+ ...+...-....+.+- .......-",
    "....++.. .+..........-... --..++..",
    "....+.-. ..+............. ....-.+.",
    "+.....+. ..+.....-....... ..+.-...",
    ".....+.- ............+-.. .-.+.+.-",
    "......+- ..............+. ......--",
    "...+..+. ...........+..+. ..+....+",
    "+...++.. .+..-........... ++..-...",
    ".+-...-. ......+..-...... ..+..+-.",
    "...+.-.+ ...+...-....-+.. .+.-...+",
    "....++.+ ............+... ....++.+",
    "...+--.. ...+........-... --.....-",
    "++..++.. ...+-........... --......",
    ".+-..+-. ......+......... .....-+.",
    ".+.-.+.- ...+...-........ .+.-....",
)]
_HK_LEFT, _HK_RIGHT = ([line[k] for line in _HK] for k in range(2))
_HK_OUT = [[line[2][o] for line in _HK] for o in range(8)]
_HK_EARLY = 7
_HK_FIRST = (4, 1, 6, 5, 0, 3, 2, 12, 22, 21, 19, 20, 15, 18, 25, 24, 23, 13, 7, 14, 9, 8, 16, 17, 10, 11)
_HK_ORDER = (15, 24, 22, 18, 19, 21, 6, 23, 4, 13, 12, 16, 8, 3, 0, 14, 9, 25, 7, 20, 1, 5, 2, 17, 10, 11)
_HK_GROUPS = ((2, 11, 15, 20, 21, 22, 25, 6), (8, 10, 13, 14, 16, 17, 19, 24, 3, 4, 5), (1, 7, 0, 9, 12, 18, 23))


def _sums(rows, xs, ready=None):
    xs, ready = list(xs), list(ready or range(len(xs)))
    rows = [{j: c for j, c in enumerate(row) if c} for row in rows]
    while True:
        count = {}
        for row in rows:
            for pair in [(a, b, row[a] * row[b]) for a in row for b in row if a < b]:
                count[pair] = count.get(pair, 0) + 1
        best = max(sorted(count), key=count.get, default=None)
        if best is None or count[best] < 2:
            break
        a, b, sign = best
        xs.append(xs[a] + xs[b] if sign > 0 else xs[a] - xs[b])
        ready.append(max(ready[a], ready[b]))
        for row in rows:
            if row.get(a, 0) * row.get(b, 0) == sign:
                row[len(xs) - 1] = row.pop(a)
                del row[b]
    out = []
    for row in rows:
        (j, sign), *rest = sorted(row.items(), key=lambda t: (ready[t[0]], t[0]))
        acc = xs[j]
        for j, c in rest:
            acc = acc + xs[j] if c == sign else acc - xs[j] if sign > 0 else xs[j] - acc
            sign = max(sign, c)
        out.append(acc if sign > 0 else -acc)
    return out


def _layernorm(x, moments=None):
    mean = moments[0] if moments else jnp.mean(x, axis=-1, keepdims=True)
    xc = x - mean
    scale = moments[1] if moments else jax.lax.rsqrt(jnp.mean(xc * xc, axis=-1, keepdims=True) + _EPS)
    return xc * scale, (mean, scale)


def _geglu(g, u):
    c = float(np.sqrt(2.0 / np.pi))
    th = jnp.tanh(g * (c + (c * 0.044715) * (g * g)))
    half = (0.5 * g) * u
    return half * th + half


def _normalize_input(src, plain, sums, r0, rows):
    hd = src[0].shape[1] // 2
    a, b = (_layernorm(ref[pl.ds(r0, rows), :].astype(_F32))[0] for ref in src)
    at = pl.ds(r0 // 2, rows // 2)
    _store_packed(plain, at, slice(None), (a, b))
    left = _strassen_left(a[:, :hd], a[:, hd:], b[:, :hd], b[:, hd:])
    return _token(_store_packed(sums, at, slice(None), [left[k] for k in _STRASSEN_SUMS])[1:3])


def _heads_minor(load, store):
    vs = []
    lanes = lambda: jax.lax.broadcasted_iota(_I32, vs[0].shape, 1)

    def skew():
        vs.extend(pltpu.roll(load(g), 4 * g, 1) if g else load(g) for g in range(8))
        return _token(vs[4:])

    def exchange():
        us = [vs[-j % 8] for j in range(8)]
        for b in (1, 2, 4):
            moved = (lanes() & (4 * b)) != 0
            us = [jnp.where(moved, us[(j - b) % 8], us[j]) for j in range(8)]
        vs[:] = [pltpu.roll(u, 128 - 4 * j, 1) if j else u for j, u in enumerate(us)]
        return _token(vs[4:])

    def shuffle():
        lane = lanes()
        idx = (lane & 3) * 32 + (lane & 28) + (lane >> 5)
        return store([jnp.take_along_axis(v, idx, axis=1, mode="promise_in_bounds") for v in vs])

    return [skew, exchange, shuffle]


def _prepare_q(src, dst, r0, rows):
    def store(vs):
        for j, v in enumerate(vs):
            dst[pl.ds(r0, rows), _block(j, 128)] = _unpack(v)
        return _token(vs[4:])

    return _heads_minor(lambda g: src[pl.ds(r0 // 2, rows // 2), _block(g, 128)], store)


def _prepare_kv_weight(src, dst):
    def load(g):
        return jnp.concatenate([_words(ref[:, _block(g, 128)]) for ref in src], axis=0)

    def store(vs):
        vs = [_unpack(v).astype(_F32) for v in vs]
        return _token([_store_packed(
            dst, slice(None), _block(j, 128),
            _strassen_right(vs[j][:16], vs[j + 4][:16], vs[j][16:], vs[j + 4][16:]))[0] for j in range(4)])

    return _heads_minor(load, store)


def _prepare_out_weight(src, tmp, dst, c):
    pitch = _HEAD_DIM + 1

    def spread(h0):
        ys = []
        for h in range(h0, h0 + 4):
            for k in range(2):
                ys.append(src[_block(h, _HEAD_DIM), _block(c + 4 * k, 128)].astype(_F32))
                tmp[k, pl.ds(h * pitch, _HEAD_DIM), :] = ys[-1]
        return _token([_words(y[:8]) for y in ys])

    def gather(d0):
        ys = []
        for d in range(d0, d0 + 2):
            b = [tmp[k, pl.ds(d + j * _HEAD_DIM // 2, _HEADS, stride=pitch), :] for j in range(2) for k in range(2)]
            ys.append(_store_packed(dst, _block(d, _HEADS // 2), _block(c, 128), _strassen_right(*b))[0])
        return _token(ys)

    return ([_bind(spread, h) for h in range(0, _HEADS, 4)]
            + [_bind(gather, d) for d in range(0, _HEAD_DIM // 2, 2)])


def _prepare_ffn_weight(src, dst, r0, c0, d0, group):
    quarter = src.shape[2] // 4
    b = [src.at[j // 4][pl.ds(r0, 16), pl.ds(j % 4 * quarter + c0, 128)].astype(_F32)
         if any(_HK_RIGHT[k][j] for k in group) else None for j in range(16)]
    ys = [_pack(y) for y in _sums([_HK_RIGHT[k] for k in group], b)]
    for k, y in zip(group, ys):
        dst.at[k][pl.ds(r0 // 2, 8), pl.ds(d0, 128)] = y
    return ys[0]


def _attention(q_s, k_s, v_s, r0, pos0, store):
    ls = []
    window = lambda w: pl.ds(_HALO + r0 - _DILATION * w, 16)

    def scores():
        q = [q_s[pl.ds(r0, 16), _block(c, 128)].astype(_F32) for c in range(8)]
        for w in range(_WINDOW):
            acc = q[0] * k_s[0, window(w), :]
            for c in range(1, 8):
                acc = acc + q[c] * k_s[c, window(w), :]
            ls.append(acc + pltpu.roll(acc, 64, 1))
        return _token([_words(l) for l in ls[-2:]])

    def softmax():
        for w in range(_WINDOW):
            l = (ls[w] + pltpu.roll(ls[w], 32, 1)) * (_HEAD_DIM ** -0.5)
            if pos0 is not None and r0 < _DILATION * w:
                pos = pos0 + r0 + jax.lax.broadcasted_iota(_I32, l.shape, 0)
                l = jnp.where(pos >= _DILATION * w, l, -1e9)
            ls[w] = l
        top = functools.reduce(jnp.maximum, ls)
        es = [jnp.exp(l - top) for l in ls]
        inv = 1.0 / functools.reduce(jnp.add, es)
        ls[:] = [e * inv for e in es]
        return _token([_words(inv)])

    def mix(*groups):
        def weighted(c):
            acc = ls[0] * v_s[c, window(0), :]
            for w in range(1, _WINDOW):
                acc = acc + ls[w] * v_s[c, window(w), :]
            return acc

        return _token([y for c in groups for y in store(r0, c, weighted(c), weighted(c + 4))])

    return scores, softmax, mix


def _attention_halves(views, keep, dst, pos0):
    def store_upper(r0, c, a11, a12):
        keep[c, pl.ds(r0, 16), :] = a11
        keep[c + 4, pl.ds(r0, 16), :] = a12
        return [_words(a11), _words(a12)]

    def store_lower(r0, c, a21, a22):
        left = _strassen_left(keep[c, pl.ds(r0, 16), :], keep[c + 4, pl.ds(r0, 16), :], a21, a22)
        return _store_packed(dst, pl.ds(r0 // 2, 8), _block(c, 128), left)[1:2]

    return [_attention(*views[p], r0, None if p else pos0, store)
            for r0 in range(0, views[0][0].shape[0], 16) for p, store in enumerate((store_upper, store_lower))]


@jax.jit
def pallas_sequential_preLN__sliding_local_dilated__glu_gated_geglu__prompt_kernel(
    A_x: jax.Array,
    A_wqkv: jax.Array,
    A_wo: jax.Array,
    B_x: jax.Array,
    B_w_gate: jax.Array,
    B_w_up: jax.Array,
    B_w_down: jax.Array,
):
    del B_x
    B, S, D = A_x.shape
    F = B_w_gate.shape[1]
    assert (B, S, D) == (1, 2048, _HEADS * _HEAD_DIM) and F % 512 == 0
    T = 256
    n, hf, hd, qd = S // T, T // 2, D // 2, D // 4
    NQ = NK = NS = 4
    QC, TK = D // NQ, S // NS
    KU, AR = 11, 48

    def kernel(x_hbm, wqkv_hbm, wo_hbm, wg_hbm, wu_hbm, wd_hbm, out_hbm,
               x_s, w_in, wo_in, wg_in, wu_in, wd_in, wgu, wd, wkv, wo, wo_tmp,
               xn_s, xsum_s, wq, qraw_s, q_s, k_s, v_s, keep_s, o_s, ha_s, hb_s, hna_s, hnb_s, zero_s,
               xsem, wsem, fsem, osem):
        def x_copy(i):
            return [pltpu.make_async_copy(x_hbm.at[_block(i, T)], x_s.at[_block(i, T)], xsem.at[i])]

        def q_copy(j):
            at = lambda ref, p: ref.at[_block((2 + p) * NQ + j, hf // NQ)]
            return [pltpu.make_async_copy(a, b, xsem.at[n + j]) for a, b in (
                (at(x_hbm, 0), at(x_s, 0)), (at(x_hbm, 1), at(x_s, 1)),
                (wqkv_hbm.at[:, _block(j, QC)], w_in.at[:, _block(j, QC)]))]

        def kv_copy(j):
            at = lambda ref, p: ref.at[_block(p * NK + j, hd // NK), pl.ds(D, 2 * D)]
            return [pltpu.make_async_copy(at(wqkv_hbm, p), at(w_in, p), wsem.at[j]) for p in range(2)]

        def o_copy():
            return [pltpu.make_async_copy(wo_hbm, wo_in, wsem.at[NK])]

        def ffn_copy(i):
            return [pltpu.make_async_copy(w.at[:, _block(i, w.shape[1] // NS), :],
                                          dst.at[i % 2, :, pl.ds(0, w.shape[1] // NS), :], fsem.at[i % 2])
                    for w, dst in ((wg_hbm, wg_in), (wu_hbm, wu_in), (wd_hbm, wd_in))]

        def start(copies):
            for c in copies:
                c.start()

        def wait(copies):
            for c in copies:
                c.wait()

        def normalize(i, rows):
            at = lambda ref: ref.at[:, _block(i, hf // 2), :]
            src = [x_s.at[_block(2 * i + p, hf)] for p in range(2)]
            return [_bind(_normalize_input, src, at(xn_s), at(xsum_s), r0, rows) for r0 in range(0, hf, rows)]

        def normalized(i):
            return jnp.concatenate([xn_s[p, _block(i, hf // 2), :] for p in range(2)], axis=0)

        def first_q_step(j, _):
            pl.when(j + 2 < NQ)(lambda: start(q_copy(j + 2)))
            pl.when(j + 2 == NQ)(lambda: start(x_copy(2) + kv_copy(0)))
            wait(q_copy(j))
            rows = hf // NQ
            at = lambda ref: ref.at[:, _block(NQ + j, rows // 2), :]
            src = [x_s.at[_block((2 + p) * NQ + j, rows)] for p in range(2)]
            jobs = [_bind(_normalize_input, src, at(xn_s), at(xsum_s), r0, 16) for r0 in range(0, rows, 16)]
            wq[:, _block(j, QC)] = w = _words(w_in[:, _block(j, QC)])
            qraw_s[pl.ds(0, hf), _block(j, QC)] = _pack(_dot(normalized(0), w, zero_s[...], [jobs], 2))

        def q_step(i, _):
            pl.when(i < NK)(lambda: start(x_copy(i + 2) + kv_copy(i)))
            pl.when(i == NK - 1)(lambda: start(sum([x_copy(j) for j in range(NK + 2, n)], [])))
            pl.when(i == NK)(lambda: start(o_copy() + ffn_copy(0)))
            pl.when(i + 1 < n)(lambda: wait(x_copy(i + 1)))
            pl.when((i > 1) & (i < NK + 2))(lambda: wait(kv_copy(i - 2)))
            prepare = []
            for t in range(KU):
                u = jnp.clip((i - 2) * KU, 0, hd // 8 - KU) + t
                cols = _block(jnp.where(i > 1, u % 2 + 1, 0), D)
                src = [w_in.at[_block(p * (hd // 16) + u // 2, 16), cols] for p in range(2)]
                prepare.append(_prepare_kv_weight(src, wkv.at[u % 2, :, _block(u // 2, 8), :]))
            queues = [_staggered(prepare), normalize(jnp.minimum(i + 1, n - 1), 16)]
            qraw_s[_block(i, hf), :] = _pack(_dot(normalized(i), wq[...], zero_s[...], queues, 3))

        def kv_step(i, _):
            pl.when(i + 1 < NS)(lambda: start(ffn_copy(i + 1)))
            wait(ffn_copy(i))

            def project(i_again, w, dst, t0):
                dst = dst.at[:, _block(i, TK, _HALO), :]
                rows, m = _block(i_again, TK // 4), {}
                for t, k in enumerate((2, 4, 1, 3, 0, 5, 6), t0):
                    a = (xsum_s[_STRASSEN_SUMS.index(k), rows, :] if k in _STRASSEN_SUMS
                         else xn_s[k - 2, rows, _block(k - 2, hd)])
                    m[k] = _dot(a, w[k], zero_s[...], [_share(q, t - a0, a1 - a0) for q, a0, a1 in queues if a0 <= t < a1],
                                0 if t else 1)
                    y = m[k][:16, 128:256]
                    if t in (4, 6, 8, 10):
                        qraw_s[_block(S // 16 + (i >> 8), 8), _block(0, 128)] = _words(y[:8])
                    if t == 5:
                        for ref in (wg_in, wu_in, wd_in):
                            ref.at[i % 2 + (i >> 8), 0][pl.ds(ref.shape[2] - 16, 16), _block(0, 128)] = y.astype(_BF16)
                y = _strassen_upper(m) + _strassen_lower(m)
                for t in range(TK // T):
                    for p in range(2):
                        for c in range(8):
                            dst[c, pl.ds(_HALO + t * T + p * hf, hf), :] = (
                                y[2 * p + c // 4][t * hf:(t + 1) * hf, c % 4 * 128:(c % 4 + 1) * 128])

            prepare = []
            for src, dst, scale, shift in ((wg_in, wgu, 2, 0), (wu_in, wgu, 2, 128), (wd_in, wd, 1, 0)):
                size = src.shape[2] - 16
                prepare += [_bind(_prepare_ffn_weight, src.at[i % 2], dst.at[:, _block(i, size // 2), :],
                                  r0, c0, scale * c0 + shift, group)
                            for r0 in range(0, size, 16) for c0 in range(0, src.shape[3] // 4, 128)
                            for group in _HK_GROUPS]
            views = [[q_s.at[_block(p, hf)].at[_clamped(i - 1, AR, hf)]]
                     + [ref.at[:, _block(p, hf, _HALO), :].at[:, _clamped(i - 1, AR, hf, _HALO), :]
                        for ref in (k_s, v_s)] for p in range(2)]
            attend = _attention_halves(views, keep_s, o_s.at[:, _clamped(i - 1, AR // 2, hf // 2), :],
                                       jnp.clip((i - 1) * AR, 0, hf - AR))
            layout = [_prepare_q(qraw_s.at[_block(i, TK // 2)], q_s.at[_block(i, TK)], r0, 32)
                      for r0 in range(0, TK, 32)]
            queues = [(prepare, 0, 14), ([_chain(a, b) for a, b, _ in attend], 0, 7),
                      (_staggered(layout), 6, 14), (_prepare_out_weight(wo_in, wo_tmp, wo, i), 0, 4),
                      ([_bind(mix, 0, 1, 2, 3) for _, _, mix in attend], 8, 14)]
            project(i, wkv.at[1], v_s, 0)
            for c in range(8):
                v_s[c, pl.ds(0, _HALO), :] = jnp.broadcast_to(v_s[c, pl.ds(_HALO, 1), :], (_HALO, 128))
            project(i + (i >> 8), wkv.at[0], k_s, 7)

        def main_step(i, _):
            zero = zero_s[...]
            whole = lambda rows, use=0: _block(i >> (8 + use), rows)
            hs, moments = (ha_s, hb_s), {}

            def residual(p, blocks):
                for t, y in enumerate(blocks):
                    hs[p][:, _block(t, hd)] = x_s[_block(2 * i + p, hf), _block(t, hd)].astype(_F32) + y

            def norm(p, r0):
                y, moments[p, r0] = _layernorm(hs[p].at[whole(hf)][pl.ds(r0, 16), :])
                upper = _layernorm(hs[0].at[whole(hf, 1)][pl.ds(r0, 16), :], moments[0, r0])[0] if p else y
                blocks = [v[:, k * qd:(k + 1) * qd] for v in (upper, y) for k in range(4)]
                left = _sums(_HK_LEFT[_HK_EARLY:] if p else _HK_LEFT[:_HK_EARLY], blocks)
                return _token(_store_packed(hnb_s if p else hna_s, pl.ds(r0 // 2, 8), slice(None), left)[-3:])

            norms = [[_bind(norm, p, r0) for r0 in range(0, hf, 16)] for p in range(2)]
            m = {k: _dot(o_s[k], wo[k], zero) for k in (2, 4, 3, 0, 6)}
            residual(0, _strassen_upper(m))
            m[1] = _dot(o_s[1], wo[1], zero)
            m[5] = _dot(o_s[5], wo[5], zero, [norms[0][:4]])
            _chain(*norms[0][4:])()
            residual(1, _strassen_lower(m))

            j = jnp.minimum(i + 1, n - 1)
            views = [[q_s.at[_block(2 * j + p, hf)]]
                     + [ref.at[:, _block(2 * j + p, hf, _HALO), :] for ref in (k_s, v_s)] for p in range(2)]
            attend = [job for scores, softmax, mix in _attention_halves(views, keep_s, o_s, None)
                      for job in (scores, _chain(softmax, _bind(mix, 0, 1)), _bind(mix, 2, 3))]

            lead, tiles = 4, F // 512
            orders = [_HK_FIRST if u < lead else _HK_ORDER for u in range(tiles)]
            ups = [step[1:] for step in sorted(
                (t if u < lead and t < _HK_EARLY else t + 11.5 * u, u, k)
                for u, order in enumerate(orders) for t, k in enumerate(order))]
            steps = ups + list(_HK_ORDER)
            jobs = {}
            for queue, span in ((norms[1], steps[8:_HK_EARLY * lead]), (attend, steps[_HK_EARLY * lead:-4])):
                jobs.update({step: [_share(queue, t, len(span))] for t, step in enumerate(span)})
            up = {}
            for u, k in ups:
                a = hna_s.at[k] if k < _HK_EARLY else hnb_s.at[k - _HK_EARLY]
                up[u, k] = _dot(a[whole(hf // 2, u), :], wgu.at[k][:, _block(u, 256)], zero, jobs.get((u, k), ()))

            def activation(u):
                ready = [orders[u].index(k) for k in range(len(_HK))]
                gate_up = _sums(_HK_OUT, [up[u, k] for k in range(len(_HK))], ready)
                ready = [max(t for t, c in zip(ready, row) if c) for row in _HK_OUT]
                return _sums(_HK_LEFT, [_geglu(y[:, :128], y[:, 128:]) for y in gate_up], ready)

            left = [jnp.concatenate(v, axis=1) for v in zip(*[activation(u) for u in range(tiles)])]
            down = {k: _dot(left[k].astype(_BF16), wd.at[k][...], zero, jobs.get(k, ())) for k in _HK_ORDER}
            out = _sums(_HK_OUT, [down[k] for k in range(len(_HK))], [_HK_ORDER.index(k) for k in range(len(_HK))])

            for p, t0, nt in ((1, 0, 3), (0, 0, 2), (0, 2, 2), (1, 3, 1)):
                for t in range(t0, t0 + nt):
                    y = hs[p][whole(hf), _block(t, qd)] + out[4 * p + t]
                    x_s[_block(2 * i + p, hf), _block(t, qd)] = y.astype(_BF16)
                at = lambda ref: ref.at[_block(2 * i + p, hf), pl.ds(t0 * qd, nt * qd)]
                pltpu.make_async_copy(at(x_s), at(out_hbm), osem).start()

        start(x_copy(0) + q_copy(0) + q_copy(1))
        zero_s[...] = jnp.zeros(zero_s.shape, _I32)
        wo_tmp[...] = jnp.zeros(wo_tmp.shape, _F32)
        for p in range(2):
            k_s[:, pl.ds(p * hf, AR + _HALO), :] = jnp.zeros((8, AR + _HALO, 128), _F32)
            q_s[pl.ds(p * hf, AR), :] = jnp.zeros((AR, D), _BF16)
        wait(x_copy(0))
        _chain(*normalize(0, hf))()
        jax.lax.fori_loop(0, NQ, first_q_step, None)
        jax.lax.fori_loop(1, n, q_step, None)
        wait(o_copy())
        jax.lax.fori_loop(0, NS, kv_step, None)
        jax.lax.fori_loop(0, n, main_step, None)
        pltpu.make_async_copy(x_s, out_hbm, osem).wait()

    vmem, dma = pltpu.VMEM, pltpu.SemaphoreType.DMA
    in_hbm = pl.BlockSpec(memory_space=pl.ANY)
    row_blocks = lambda w: w.reshape(4, w.shape[0] // 4, w.shape[1])
    out = pl.pallas_call(
        kernel,
        out_shape=jax.ShapeDtypeStruct((S, D), A_x.dtype),
        in_specs=[in_hbm] * 6,
        out_specs=in_hbm,
        scratch_shapes=[
            vmem((S, D), _BF16), vmem((D, 3 * D), _BF16), vmem((D, D), _BF16),
            vmem((2, 4, qd // NS + 16, F), _BF16), vmem((2, 4, qd // NS + 16, F), _BF16),
            vmem((2, 4, F // 4 // NS + 16, D), _BF16),
            vmem((len(_HK), qd // 2, F // 2), _I32), vmem((len(_HK), F // 8, qd), _I32),
            vmem((2, 7, hd // 2, hd), _I32), vmem((7, hd // 2, hd), _I32),
            vmem((2, _HEADS * (_HEAD_DIM + 2), 128), _F32),
            vmem((2, S // 4, D), _I32), vmem((len(_STRASSEN_SUMS), S // 4, hd), _I32),
            vmem((D // 2, D), _I32), vmem((S // 2 + 8, D), _I32), vmem((S, D), _BF16),
            vmem((8, S + _HALO + 8, 128), _F32), vmem((8, S + _HALO + 8, 128), _F32),
            vmem((8, hf, 128), _F32), vmem((7, hf // 2, hd), _I32),
            vmem((hf, D), _F32), vmem((hf, D), _F32),
            vmem((_HK_EARLY, hf // 2, qd), _I32), vmem((len(_HK) - _HK_EARLY, hf // 2, qd), _I32),
            vmem((8, 128), _I32),
            dma((n + NQ,)), dma((NK + 1,)), dma((2,)), dma(()),
        ],
        compiler_params=pltpu.CompilerParams(
            vmem_limit_bytes=126 * 1024 * 1024,
            flags={"XLA_TPU_EVENLY_DISTRIBUTE_CRITICAL_NODES": True},
        ),
    )(A_x.reshape(S, D), A_wqkv, A_wo, row_blocks(B_w_gate), row_blocks(B_w_up), row_blocks(B_w_down))
    return out.reshape(B, S, D)
```
